```python
import os as _os
_os.environ.setdefault("JAX_PLATFORMS", "cpu")
import jax
import jax.numpy as jnp

def _softmax(x, axis=-1):
    return jax.nn.softmax(x, axis=axis)
def _gelu(x):
    return jax.nn.gelu(x, approximate=True)
def _silu(x):
    return jax.nn.silu(x)
def _sigmoid(x):
    return jax.nn.sigmoid(x)
def _layernorm(x, axis=-1, eps=1e-5):
    m = jnp.mean(x, axis=axis, keepdims=True)
    v = jnp.var(x, axis=axis, keepdims=True)
    return (x - m) / jnp.sqrt(v + eps)
def _scatter_add(tgt, idx, src, axis=0):
    return tgt.at[idx].add(src)
def _segment_sum(src, seg, n):
    return jax.ops.segment_sum(src, seg, n)
class _Rng:
    def __init__(self, key):
        self._k = key
    def _next(self):
        self._k, sub = jax.random.split(self._k)
        return sub
    def normal(self, shape):
        return jax.random.normal(self._next(), shape, dtype=jnp.bfloat16)
    def randint(self, lo, hi, shape):
        return jax.random.randint(self._next(), shape, lo, hi, dtype=jnp.int32)
    def uniform(self, shape, lo=0.0, hi=1.0):
        return jax.random.uniform(self._next(), shape, jnp.bfloat16, lo, hi)
    def permutation(self, n):
        return jax.random.permutation(self._next(), n)


kernel_name = 'concat_heads__softmax_full_mha__softmax_full_mha__prompt'

def setup_inputs():
    _rng = _Rng(jax.random.key(int.from_bytes(__import__("os").urandom(4), "little")))
    _w = (lambda a: (lambda t: t.astype(jnp.bfloat16) if jnp.issubdtype(t.dtype, jnp.floating) else t)(jnp.asarray(a)))
    def _A_setup():
        B, S, D = 1, 2048, 512
        return {
            "x": _w((lambda *s: _rng.normal(s) * 0.2)(B, S, D)),
            "wqkv": _w((lambda *s: _rng.normal(s) * 0.2)(D, 3 * D)),
            "wo": _w((lambda *s: _rng.normal(s) * 0.05)(D, D)),
        }
    _A_in = _A_setup()

    def _B_setup():
        B, S, D = 1, 2048, 512
        return {
            "x": _w((lambda *s: _rng.normal(s) * 0.2)(B, S, D)),
            "wqkv": _w((lambda *s: _rng.normal(s) * 0.2)(D, 3 * D)),
            "wo": _w((lambda *s: _rng.normal(s) * 0.05)(D, D)),
        }
    _B_in = _B_setup()

    return {
        "A_x": _A_in["x"],
        "A_wqkv": _A_in["wqkv"],
        "A_wo": _A_in["wo"],
        "B_x": _B_in["x"],
        "B_wqkv": _B_in["wqkv"],
        "B_wo": _B_in["wo"],
    }

def reference(A_x, A_wqkv, A_wo, B_x, B_wqkv, B_wo):
    def _A_ref(x, wqkv, wo):
        B, S, D = x.shape
        H = 32; Dh = D // H
        qkv = (lambda x, *d: x.transpose(*d))((x @ wqkv).reshape(B, S, 3, H, Dh), 2, 0, 3, 1, 4)
        q, k, v = qkv[0], qkv[1], qkv[2]
        scale = Dh ** -0.5
        scores = jnp.einsum("bhqd,bhkd->bhqk", q, k) * scale
        p = _softmax(scores, axis=-1)
        o = jnp.einsum("bhqk,bhkd->bhqd", p, v)
        return (lambda x, *d: x.transpose(*d))(o, 0, 2, 1, 3).reshape(B, S, D) @ wo

    def _B_ref(x, wqkv, wo):
        B, S, D = x.shape
        H = 32; Dh = D // H
        qkv = (lambda x, *d: x.transpose(*d))((x @ wqkv).reshape(B, S, 3, H, Dh), 2, 0, 3, 1, 4)
        q, k, v = qkv[0], qkv[1], qkv[2]
        scale = Dh ** -0.5
        scores = jnp.einsum("bhqd,bhkd->bhqk", q, k) * scale
        p = _softmax(scores, axis=-1)
        o = jnp.einsum("bhqk,bhkd->bhqd", p, v)
        return (lambda x, *d: x.transpose(*d))(o, 0, 2, 1, 3).reshape(B, S, D) @ wo

    a = _A_ref(A_x, A_wqkv, A_wo)
    b = _B_ref(B_x, B_wqkv, B_wo)
    return jnp.concatenate([a, b], axis=-1)
```

```python
import math
import jax, jax.numpy as jnp
from jax import lax
from jax.experimental import pallas as pl
from jax.experimental.pallas import tpu as pltpu

S=2048; D=512; H=32; DH=16
TQ=512; CH=128
SK=3
D1=2; D2=2; D3=2
UPI=2
PR=512
NQ=S//TQ; NC=S//CH; NU=H*NQ
F32=jnp.float32; BF=jnp.bfloat16; U32=jnp.uint32
QSCALE = (DH ** -0.5) * math.log2(math.e)

def fold8(x, op):
    R = x.shape[0]
    acc = x[0:8]
    for i in range(1, R//8):
        acc = op(acc, x[i*8:(i+1)*8])
    return acc

def kern(ax, aw, ao, bx, bw, bo, out_hbm,
         x_b, w_b, wo_b, wt_s, k_s, qt_s, vt_s, ot_s, ob, s0, s1, w0, w1, m0, m1, l_c, o_c, isem, osem):
    b = pl.program_id(0)
    NXC = S // PR

    def in_copies(slot):
        x, w, wo = (ax, aw, ao) if slot == 0 else (bx, bw, bo)
        cps = [pltpu.make_async_copy(w, w_b.at[slot], isem.at[slot, 0])]
        for i in range(NXC):
            cps.append(pltpu.make_async_copy(x.at[0, pl.ds(i*PR, PR), :], x_b.at[slot, pl.ds(i*PR, PR), :], isem.at[slot, 1+i]))
        cps.append(pltpu.make_async_copy(wo, wo_b.at[slot], isem.at[slot, 1+NXC]))
        return cps

    @pl.when(b == 0)
    def _():
        for slot in range(2):
            for cp in in_copies(slot):
                cp.start()

    def wait_in(j):
        x, w, wo = ax, aw, ao
        if j == 0:
            pltpu.make_async_copy(w, w_b.at[b], isem.at[b, 0]).wait()
        elif j <= NXC:
            i = j-1
            pltpu.make_async_copy(x.at[0, pl.ds(i*PR, PR), :], x_b.at[b, pl.ds(i*PR, PR), :], isem.at[b, j]).wait()
        else:
            pltpu.make_async_copy(wo, wo_b.at[b], isem.at[b, j]).wait()

    wait_in(0)
    wt_s[0:D, :] = w_b[b, :, 0:D].T
    wt_s[D:2*D, :] = w_b[b, :, 2*D:3*D].T

    for i in range(NXC):
        wait_in(1+i)
        xc = x_b[b, pl.ds(i*PR, PR), :]
        kc = jnp.dot(xc, w_b[b, :, D:2*D], preferred_element_type=F32)
        k_s[pl.ds(i*PR//2, PR//2), :] = pltpu.bitcast(kc.astype(BF), U32)
        qv = lax.dot_general(wt_s[...], xc, (((1,), (1,)), ((), ())), preferred_element_type=F32)
        qt_s[:, pl.ds(i*PR, PR)] = pltpu.bitcast((qv[0:D] * QSCALE).astype(BF), U32)
        vt_s[:, pl.ds(i*PR, PR)] = pltpu.bitcast(qv[D:2*D].astype(BF), U32)

    sb = (s0, s1); wb = (w0, w1); mb = (m0, m1)

    def unit_idx(u):
        return u // NQ, u % NQ

    def make_w(u, w):
        h, qb = unit_idx(u)
        w[...] = jnp.zeros(w.shape, U32)
        r = pl.multiple_of(h*8, 8); c = pl.multiple_of(qb*TQ, TQ)
        wr = pl.multiple_of((h % 8)*8, 8)
        w[pl.ds(wr, 8), :] = qt_s[pl.ds(r, 8), pl.ds(c, TQ)]

    def a_chunk(u, c, w, sbuf, macc):
        h, qb = unit_idx(u)
        g = pl.multiple_of((h // 8)*128, 128)
        kk = pltpu.bitcast(k_s[pl.ds(c*CH//2, CH//2), pl.ds(g, 128)], BF)
        s = jnp.dot(kk, pltpu.bitcast(w[...], BF), preferred_element_type=F32)
        sbuf[pl.ds(c*CH, CH), :] = s
        mm = fold8(s, jnp.maximum)
        return mm if macc is None else jnp.maximum(macc, mm)

    def b_chunk(u, c, sbuf, m8, lacc, oacc):
        h, qb = unit_idx(u)
        r = pl.multiple_of(h*8, 8)
        s = sbuf[pl.ds(c*CH, CH), :]
        p = jnp.exp2(s.reshape(CH//8, 8, TQ) - m8[None]).reshape(CH, TQ)
        ll = fold8(p, jnp.add)
        vt = pltpu.bitcast(vt_s[pl.ds(r, 8), pl.ds(c*CH, CH)], BF)
        o = jnp.dot(vt, p.astype(BF), preferred_element_type=F32)
        return (ll if lacc is None else lacc + ll), (o if oacc is None else oacc + o)

    def finish(u, lacc, oacc):
        h, qb = unit_idx(u)
        l = jnp.sum(lacc, axis=0, keepdims=True)
        r = pl.multiple_of(h*DH, DH); c = pl.multiple_of(qb*TQ, TQ)
        ot_s[pl.ds(r, DH), pl.ds(c, TQ)] = oacc * (1.0/l)

    NEG = -jnp.inf
    def run_steps(ua0, n_units, do_a, b_first, b_last):
        hist_m = []; hist_l = []; hist_o = []
        macc = None; lacc = None; oacc = None; m8 = None
        for t in range(n_units*NC):
            ja, ca = divmod(t, NC)
            if do_a:
                ua = ua0 + ja
                par = ja % 2
                if ca == 0:
                    make_w(ua, wb[par]); macc = None
                macc = a_chunk(ua, ca, wb[par], sb[par], macc)
                hist_m.append(macc)
                if ca == NC-1:
                    mb[par][...] = jnp.broadcast_to(jnp.max(macc, axis=0, keepdims=True), (8, TQ))
            else:
                hist_m.append(None)
            tb = t - NC - SK
            jb, cb = divmod(tb, NC)
            if b_first <= t < b_last:
                ub = ua0 + jb
                par = jb % 2
                if cb == 0 or m8 is None:
                    m8 = mb[par][...]
                    if cb == 0:
                        lacc = None; oacc = None
                    else:
                        lacc = l_c[...]; oacc = o_c[...]
                mm = m8
                dep = None
                for hist, dd in ((hist_m, D1), (hist_l, D2-1), (hist_o, D3-1)):
                    if dd >= 0 and len(hist) > dd and hist[len(hist)-1-dd] is not None:
                        x = hist[len(hist)-1-dd][0:8]
                        dep = x if dep is None else jnp.minimum(dep, x)
                if dep is not None:
                    mm = jnp.maximum(m8, jnp.minimum(dep, NEG))
                lacc, oacc = b_chunk(ub, cb, sb[par], mm, lacc, oacc)
                hist_l.append(lacc); hist_o.append(oacc)
                if cb == NC-1:
                    finish(ub, lacc, oacc)
            else:
                hist_l.append(None); hist_o.append(None)
        if lacc is not None and do_a:
            l_c[...] = lacc; o_c[...] = oacc

    run_steps(0, UPI, True, NC+SK, UPI*NC)
    def body(i, carry):
        run_steps(UPI*i, UPI, True, 0, UPI*NC)
        return carry
    lax.fori_loop(1, NU//UPI, body, 0)
    run_steps(NU, 2, False, 0, NC+SK)

    wait_in(1+NXC)
    def out_copy(bb, i):
        return pltpu.make_async_copy(ob.at[pl.ds(i*PR, PR), :],
                                     out_hbm.at[0, pl.ds(i*PR, PR), pl.ds(pl.multiple_of(bb*D, D), D)], osem.at[i])
    @pl.when(b == 1)
    def _():
        for i in range(NXC):
            out_copy(0, i).wait()
    for i in range(NXC):
        oc = ot_s[:, pl.ds(i*PR, PR)].T.astype(BF)
        r = jnp.dot(oc, wo_b[b], preferred_element_type=F32)
        ob[pl.ds(i*PR, PR), :] = r.astype(BF)
        out_copy(b, i).start()
    @pl.when(b == 1)
    def _():
        for i in range(NXC):
            out_copy(1, i).wait()

@jax.jit
def pallas_concat_heads__softmax_full_mha__softmax_full_mha__prompt_kernel(A_x, A_wqkv, A_wo, B_x, B_wqkv, B_wo):
    ax, aw, ao, bx, bw, bo = A_x, A_wqkv, A_wo, B_x, B_wqkv, B_wo
    NXC = S // PR
    any_spec = pl.BlockSpec(memory_space=pl.ANY)
    return pl.pallas_call(kern, out_shape=jax.ShapeDtypeStruct((1, S, 2*D), BF),
        grid=(2,),
        in_specs=[any_spec]*6, out_specs=any_spec,
        scratch_shapes=[pltpu.VMEM((2,S,D),BF), pltpu.VMEM((2,D,3*D),BF), pltpu.VMEM((2,D,D),BF),
                        pltpu.VMEM((2*D,D),BF),
                        pltpu.VMEM((S//2,D),U32), pltpu.VMEM((D//2,S),U32), pltpu.VMEM((D//2,S),U32),
                        pltpu.VMEM((D,S),F32), pltpu.VMEM((S,D),BF),
                        pltpu.VMEM((S,TQ),F32), pltpu.VMEM((S,TQ),F32),
                        pltpu.VMEM((64,TQ),U32), pltpu.VMEM((64,TQ),U32),
                        pltpu.VMEM((8,TQ),F32), pltpu.VMEM((8,TQ),F32),
                        pltpu.VMEM((8,TQ),F32), pltpu.VMEM((DH,TQ),F32),
                        pltpu.SemaphoreType.DMA((2, NXC+2)), pltpu.SemaphoreType.DMA((NXC,))],
        compiler_params=pltpu.CompilerParams(vmem_limit_bytes=100*1024*1024, dimension_semantics=("arbitrary",)))(ax, aw, ao, bx, bw, bo)
```

```python
import functools, math
import jax, jax.numpy as jnp
from jax import lax
from jax.experimental import pallas as pl
from jax.experimental.pallas import tpu as pltpu

S=2048; D=512; H=32; DH=16
TQ=512; CH=128
SK=2; SPL=2; DL=6; LG=44
PR=512
CG=1; NG0=8; ROT=1; PS=8; PE=4
FORCE=0
PAT=[1]
NQ=S//TQ; NC=S//CH; NXC=S//PR
F32=jnp.float32; BF=jnp.bfloat16; U32=jnp.uint32
NV=[PAT[c % len(PAT)] for c in range(NC)]
OFF=[sum(NV[:c]) for c in range(NC)]
NVT=sum(NV)
NMB=8*NC-NVT
KBR = NVT*2*DH*8
QOFF = KBR
KOFF = QOFF + 256*8
SOFF = KOFF + 16*1024
PADOFF = SOFF + 16*NVT*8
OPQ = 1
NPAD = 4
TOTR = PADOFF + 8*NPAD + 8*0
NZ = 1024
QSCALE = (DH ** -0.5) * math.log2(math.e)
VBLOCKS = [(c, blk) for c in range(NC) for blk in range(NV[c])]
NPREP = NVT*32 + 256 + 1
SRCPOS = 20
SCORE_BOUND = 64.0
V_LO = 2.0 ** -30
V_HI = 2.0 ** 50

def kern(ax, aw, ao, bx, bw, bo, out_hbm,
         x_b, w_b, wo_b, wt_s, qt_s, vt_s, ot_s, ob, bufa, bufb, s_s, p_c, l_c, o_c, z_ref, isem, osem):
    b = pl.program_id(0)
    bufs = (bufa, bufb)

    def in_copies(slot):
        x, w, wo = (ax, aw, ao) if slot == 0 else (bx, bw, bo)
        cps = [pltpu.make_async_copy(w, w_b.at[slot], isem.at[slot, 0])]
        for i in range(NXC):
            cps.append(pltpu.make_async_copy(x.at[0, pl.ds(i*PR, PR), :], x_b.at[slot, pl.ds(i*PR, PR), :], isem.at[slot, 1+i]))
        cps.append(pltpu.make_async_copy(wo, wo_b.at[slot], isem.at[slot, 1+NXC]))
        return cps

    @pl.when(b == 0)
    def _():
        for slot in range(2):
            for cp in in_copies(slot):
                cp.start()
        def zz(j, c):
            z_ref[j] = 0
            return c
        lax.fori_loop(0, NZ, zz, 0)

    def wait_in(j):
        if j == 0:
            pltpu.make_async_copy(aw, w_b.at[b], isem.at[b, 0]).wait()
        elif j <= NXC:
            i = j-1
            pltpu.make_async_copy(ax.at[0, pl.ds(i*PR, PR), :], x_b.at[b, pl.ds(i*PR, PR), :], isem.at[b, j]).wait()
        else:
            pltpu.make_async_copy(ao, wo_b.at[b], isem.at[b, j]).wait()

    def ldk(hp, par, row, n=8):
        return bufs[1-par][pl.ds(pl.multiple_of(KOFF + hp*1024, 8) + row, n), :]

    def get_w(h, qb):
        r = pl.multiple_of(h*8, 8)
        return pltpu.bitcast(qt_s[pl.ds(r, 8), qb*TQ:(qb+1)*TQ], BF)

    def ld_src(hp, par, vb):
        return bufs[par][pl.ds(pl.multiple_of(SOFF + hp*NVT*8, 8) + vb*8, 8), :]

    def prep_kb_gen(src, par, vb):
        kk = pltpu.bitcast(src, BF).astype(F32)
        base = vb * 2 * DH * 8
        for d in range(DH):
            for gg in range(2):
                bufs[par][base + (gg*DH + d)*8: base + (gg*DH + d + 1)*8, :] = pltpu.bitcast(jnp.broadcast_to(kk[gg*8:(gg+1)*8, d:d+1], (8, 128)), U32)
                yield

    def prep_q_gen(hp, par, ct):
        r0 = pl.multiple_of((2*hp + par)*8, 8)
        wf = pltpu.bitcast(qt_s[pl.ds(r0, 8), ct*128:(ct+1)*128], BF).astype(F32)
        for d in range(DH):
            r = QOFF + (ct*16 + d)*8
            bufs[par][r:r+8, :] = pltpu.bitcast(jnp.broadcast_to(wf[d:d+1, :], (8,128)), U32)
            yield

    def prep_all(hp, par):
        nxt = ld_src(hp, par, 0)
        yield
        for x in range(max(16, NVT)):
            if x < 16: yield from prep_q_gen(hp, par, x)
            if x < NVT:
                cur = nxt
                g = prep_kb_gen(cur, par, x)
                for n in range(32):
                    if n == SRCPOS and x + 1 < NVT: nxt = ld_src(hp, par, x + 1)
                    next(g)
                    yield

    wait_in(0); wait_in(1)
    wt_s[0:D, :] = w_b[b, :, 0:D].T
    wt_s[D:2*D, :] = w_b[b, :, 2*D:3*D].T
    NT = (((1,), (1,)), ((), ()))
    kmax = None; qn2 = None; vmax = None
    for i in range(NXC):
        if i == 1:
            for j in range(2, NXC+1): wait_in(j)
        xc = x_b[b, pl.ds(i*PR, PR), :]
        kc = jnp.dot(xc, w_b[b, :, D:2*D], preferred_element_type=F32)
        ka = jnp.max(jnp.abs(kc).reshape(PR//8, 8, D), axis=0)
        kmax = ka if kmax is None else jnp.maximum(kmax, ka)
        kp = pltpu.bitcast(kc.astype(BF), U32)
        for h in range(H):
            g, r = divmod(h, 8)
            kr = kp[:, g*128:(g+1)*128]
            if r: kr = pltpu.roll(kr, 128 - DH*r, axis=1)
            ko = KOFF + (h//2)*1024 + i*(PR//2)
            bufs[1 - h % 2][ko: ko + PR//2, :] = kr
            for vb, (c, blk) in enumerate(VBLOCKS):
                if c // (PR//CH) == i:
                    row = (c % (PR//CH))*(CH//2) + (8 - NV[c] + blk)*8
                    so = SOFF + (h//2)*NVT*8 + vb*8
                    bufs[h % 2][so: so+8, :] = kr[row: row+8]
        q = lax.dot_general(wt_s[0:D, :], xc, NT, preferred_element_type=F32) * QSCALE
        qq = jnp.sum((q*q).reshape(H, DH, PR), axis=1)
        qn2 = qq if qn2 is None else jnp.maximum(qn2, qq)
        qt_s[:, pl.ds(i*PR, PR)] = pltpu.bitcast(q.astype(BF), U32)
    for i in range(NXC):
        xc = x_b[b, pl.ds(i*PR, PR), :]
        v = lax.dot_general(wt_s[D:2*D, :], xc, NT, preferred_element_type=F32)
        va = jnp.abs(v)
        va = jnp.maximum(jnp.maximum(va[:, 0:128], va[:, 128:256]), jnp.maximum(va[:, 256:384], va[:, 384:512]))
        va = jnp.max(va.reshape(H, DH, 128), axis=1)
        vmax = va if vmax is None else jnp.maximum(vmax, va)
        vt_s[:, pl.ds(i*PR, PR)] = pltpu.bitcast(v.astype(BF), U32)
    for _ in prep_all(0, 0): pass

    km = jnp.max(kmax, axis=0, keepdims=True)
    km = km * km
    kseg = jnp.concatenate([km[:, g*128:(g+1)*128] for g in range(4)], axis=0)
    for sh in (1, 2, 4, 8):
        kseg = kseg + pltpu.roll(kseg, sh, axis=1)
    kn2 = jnp.max(kseg)
    vh = jnp.max(vmax, axis=1, keepdims=True)
    safe = (jnp.max(qn2) * kn2 <= SCORE_BOUND * SCORE_BOUND) & (jnp.min(vh) >= V_LO) & (jnp.max(vh) <= V_HI)
    if FORCE == 1: safe = safe & (b < 0)

    def vpu_col(z0, par, qb, c, blk, j):
        accs = [None, None]
        buf = bufs[par]
        base = z0 + (OFF[c] + blk) * 2 * DH * 8
        for d in range(DH):
            kv = [pltpu.bitcast(buf[pl.ds(base + (gg*DH + d)*8, 8), :], F32) for gg in range(2)]
            qs = pltpu.bitcast(buf[pl.ds(z0 + QOFF + ((qb*4 + j)*16 + d)*8, 8), :], F32)
            for gg in range(2):
                t = kv[gg] * qs
                accs[gg] = t if accs[gg] is None else accs[gg] + t
        return jnp.concatenate(accs, axis=0)

    def pv_step(h, c, pb, oacc):
        r = pl.multiple_of(h*8, 8)
        vt = pltpu.bitcast(vt_s[pl.ds(r, 8), c*CH:(c+1)*CH], BF)
        o = jnp.dot(vt, pb, preferred_element_type=F32)
        return o if oacc is None else o + oacc

    def finish(h, qb, lacc, oacc):
        l = jnp.sum(lacc, axis=0, keepdims=True)
        r = pl.multiple_of(h*DH, DH)
        ot_s[pl.ds(r, DH), qb*TQ:(qb+1)*TQ] = oacc * (1.0/l)

    def head_block(hp, par):
        h = 2*hp + par
        hprev = (h + H - 1) % H
        NUI = NQ
        T = NUI*NC
        padrow = pl.multiple_of(PADOFF + z_ref[NZ-1], 8)
        pads = [pl.multiple_of(PADOFF + 8*x + z_ref[NZ-8-x], 8) for x in range(NPAD)]
        pbs = {t: {} for t in range(T)}
        laccs = {}; oaccs = {}
        vsteps = [(j, c, blk, col) for j in range(NUI) for (c, blk) in VBLOCKS for col in range(4)]
        NVS = len(vsteps) // NUI
        vdead = [(v * NMB) // NVS + DL for v in range(len(vsteps))]
        vnext = [0]; ng = [0]; nk = [0]; pend = []; lhist = []
        pgen = prep_all(hp, 1) if par == 0 else prep_all(jnp.minimum(hp+1, H//2-1), 0)
        def e_col(j, col, s):
            p = jnp.exp2(s)
            ll = p[0:8] + p[8:16]
            la = laccs.setdefault(j, [None]*4)
            la[col] = ll if la[col] is None else la[col] + ll
            lhist.append(la[col])
            return p, ll
        def share(x, tot, n, skip):
            if x < skip or x >= n: return 0
            return ((x-skip+1)*tot)//(n-skip) - ((x-skip)*tot)//(n-skip)
        def emit_vpu(upto_k=None, upto_t=None):
            while vnext[0] < len(vsteps):
                v = vnext[0]
                j, c, blk, col = vsteps[v]
                need = (upto_t is not None and j*NC + c <= upto_t) or (upto_k is not None and vdead[v] <= upto_k)
                if not need: break
                z0 = pl.multiple_of(z_ref[v], 8)
                pp, ll = e_col(j, col, vpu_col(z0, par, j, c, blk, col))
                pbs[j*NC + c].setdefault(8 - NV[c] + blk, {})[col] = pp
                if v >= NG0: pend.append(ll)
                vnext[0] += 1
        def qk_blocks(j, c, blks):
            ks = []
            for bb in blks:
                emit_vpu(upto_k=nk[0])
                if LG and len(lhist) > LG + 4: pend.append(lhist[-LG - (nk[0] % 4)])
                while pend:
                    bufs[1-par][pl.ds(pads[ng[0] % NPAD] if OPQ else padrow + 8*(ng[0] % NPAD), 8), :] = pltpu.bitcast(pend.pop(0), U32)
                    ng[0] += 1
                for _ in range(share(nk[0], NPREP, NQ*NMB - PE, PS)): next(pgen)
                ks.append(ldk(hp, par, c*CH//2 + bb*8))
                nk[0] += 1
            kk = pltpu.bitcast(jnp.concatenate(ks, axis=0), BF)[:, 0:DH]
            s = jnp.dot(kk, get_w(h, j), preferred_element_type=F32)
            return {bb: s[x*16:(x+1)*16] for x, bb in enumerate(blks)}
        def gather_p(tb):
            emit_vpu(upto_t=tb)
            pp = pbs.pop(tb)
            return jnp.concatenate([jnp.concatenate([pp[bb][col] for col in range(4)], axis=1) for bb in range(8)], axis=0).astype(BF)
        def do_pv(tb):
            if tb < 0:
                if not ROT: return
                c = NC + tb
                if tb == -SK: oaccs[-1] = o_c[...]
                oaccs[-1] = pv_step(hprev, c, pltpu.bitcast(p_c[(tb + SK)*CH//2:(tb + SK + 1)*CH//2, :], BF), oaccs[-1])
                if tb == -1:
                    finish(hprev, NQ-1, l_c[...], oaccs[-1])
                return
            j, c = divmod(tb, NC)
            oaccs[j] = pv_step(h, c, gather_p(tb), oaccs.get(j))
            if c == NC-1:
                finish(h, j, jnp.concatenate(laccs[j], axis=1), oaccs[j])
        for t in range(T):
            j, c = divmod(t, NC)
            mx = list(range(0, 8 - NV[c]))[::-1]
            for gi, g in enumerate([mx[:SPL], mx[SPL:]]):
                ss = qk_blocks(j, c, g)
                for bb in g:
                    pbs[t][bb] = {col: e_col(j, col, ss[bb][:, col*128:(col+1)*128])[0] for col in range(4)}
                if gi == 0 and t >= SK:
                    do_pv(t - SK)
                if gi == CG and t < SK:
                    do_pv(t - SK)
        if ROT:
            for x in range(SK):
                p_c[x*CH//2:(x+1)*CH//2, :] = pltpu.bitcast(gather_p(T - SK + x), U32)
            l_c[...] = jnp.concatenate(laccs[NUI-1], axis=1)
            o_c[...] = oaccs[NUI-1]
        else:
            for t in range(T, T + SK):
                do_pv(t - SK)

    @pl.when(safe)
    def _():
        if ROT:
            p_c[...] = jnp.zeros(p_c.shape, U32)
            l_c[...] = jnp.ones(l_c.shape, F32)
            o_c[...] = jnp.zeros(o_c.shape, F32)
        def fb(i, c):
            for par in range(2):
                @pl.when(z_ref[NZ-2-par] == 0)
                def _():
                    head_block(i, par)
            return c
        lax.fori_loop(0, H//2, fb, 0)
        if ROT:
            o = o_c[...]
            for x in range(SK):
                o = pv_step(H-1, NC - SK + x, pltpu.bitcast(p_c[x*CH//2:(x+1)*CH//2, :], BF), o)
            finish(H-1, NQ-1, l_c[...], o)

    def slow_body(hp, carry):
        SC = 256
        for par in range(2):
            h = 2*hp + par
            r8 = pl.multiple_of(h*8, 8)
            def unit(qb, c2):
                c0 = pl.multiple_of(qb*TQ, TQ)
                w = pltpu.bitcast(qt_s[pl.ds(r8, 8), pl.ds(c0, TQ)], BF)
                def p1(c, m):
                    ro = pl.multiple_of(c*(SC//2), 8)
                    kk = pltpu.bitcast(ldk(hp, par, ro, SC//2), BF)[:, 0:DH]
                    s = jnp.dot(kk, w, preferred_element_type=F32)
                    s_s[pl.ds(pl.multiple_of(c*SC, SC), SC), :] = s
                    return jnp.maximum(m, jnp.max(s, axis=0, keepdims=True))
                m = lax.fori_loop(0, S//SC, p1, jnp.full((1, TQ), -jnp.inf, F32))
                def p2(c, lo):
                    l, o = lo
                    co = pl.multiple_of(c*SC, SC)
                    p = jnp.exp2(s_s[pl.ds(co, SC), :] - m)
                    vt = pltpu.bitcast(vt_s[pl.ds(r8, 8), pl.ds(co, SC)], BF)
                    return (l + jnp.sum(p, axis=0, keepdims=True),
                            o + jnp.dot(vt, p.astype(BF), preferred_element_type=F32))
                l, o = lax.fori_loop(0, S//SC, p2, (jnp.zeros((1, TQ), F32), jnp.zeros((DH, TQ), F32)))
                ot_s[pl.ds(pl.multiple_of(h*DH, DH), DH), pl.ds(c0, TQ)] = o * (1.0/l)
                return c2
            lax.fori_loop(0, NQ, unit, 0)
        return carry

    @pl.when(jnp.logical_not(safe))
    def _():
        lax.fori_loop(0, H//2, slow_body, 0)

    wait_in(1+NXC)
    def out_copy(bb, i):
        return pltpu.make_async_copy(ob.at[pl.ds(i*PR, PR), :],
                                     out_hbm.at[0, pl.ds(i*PR, PR), pl.ds(pl.multiple_of(bb*D, D), D)], osem.at[i])
    @pl.when(b == 1)
    def _():
        for i in range(NXC):
            out_copy(0, i).wait()
    for i in range(NXC):
        oc = ot_s[:, pl.ds(i*PR, PR)].T.astype(BF)
        r = jnp.dot(oc, wo_b[b], preferred_element_type=F32)
        ob[pl.ds(i*PR, PR), :] = r.astype(BF)
        out_copy(b, i).start()
    @pl.when(b == 1)
    def _():
        for i in range(NXC):
            out_copy(1, i).wait()

@jax.jit
def pallas_concat_heads__softmax_full_mha__softmax_full_mha__prompt_kernel(A_x, A_wqkv, A_wo, B_x, B_wqkv, B_wo):
    ax, aw, ao, bx, bw, bo = A_x, A_wqkv, A_wo, B_x, B_wqkv, B_wo
    any_spec = pl.BlockSpec(memory_space=pl.ANY)
    return pl.pallas_call(kern, out_shape=jax.ShapeDtypeStruct((1, S, 2*D), BF),
        grid=(2,),
        in_specs=[any_spec]*6, out_specs=any_spec,
        scratch_shapes=[pltpu.VMEM((2,S,D),BF), pltpu.VMEM((2,D,3*D),BF), pltpu.VMEM((2,D,D),BF),
                        pltpu.VMEM((2*D,D),BF),
                        pltpu.VMEM((D//2,S),U32), pltpu.VMEM((D//2,S),U32),
                        pltpu.VMEM((D,S),F32), pltpu.VMEM((S,D),BF),
                        pltpu.VMEM((TOTR,128),U32), pltpu.VMEM((TOTR,128),U32),
                        pltpu.VMEM((S,TQ),F32),
                        pltpu.VMEM((SK*CH//2,TQ),U32), pltpu.VMEM((8,TQ),F32), pltpu.VMEM((DH,TQ),F32),
                        pltpu.SMEM((NZ,), jnp.int32),
                        pltpu.SemaphoreType.DMA((2, NXC+2)), pltpu.SemaphoreType.DMA((NXC,))],
        compiler_params=pltpu.CompilerParams(vmem_limit_bytes=100*1024*1024, dimension_semantics=("arbitrary",)))(ax, aw, ao, bx, bw, bo)
```

```python
import functools, math
import jax, jax.numpy as jnp
from jax import lax
from jax.experimental import pallas as pl
from jax.experimental.pallas import tpu as pltpu

S=2048; D=512; H=32; DH=16
TQ=512; CH=128
SK=2; SPL=2; DL=6; LG=48
PR=512
HPB=1; CG=1; NG0=0; PS=16; PE=12; VG=8
GP=[2,3]
DLT=24
FORCE=0; QRND=1
NQ=S//TQ; NC=S//CH; NXC=S//PR
F32=jnp.float32; BF=jnp.bfloat16; U32=jnp.uint32
NVG=[GP[c % len(GP)] for c in range(NC)]
GOFF=[sum(NVG[:c]) for c in range(NC)]
NGT=sum(NVG)
HALF=[c for c in range(NC) if NVG[c] % 2]
VB = 0
MXB = [x for x in range(7, -1, -1) if x != VB]
HB = MXB[SPL]
KBR = NGT*DH*8
SDL=80; RC=6; LS=10; LE=0
def kb_off(c, single): return (2*NC + HALF.index(c))*DH*8 if single else c*2*DH*8
def ks_off(c, single): return (2*NC + HALF.index(c))*8 if single else c*16
PITEMS=[(c, False) for c in range(NC)]
for _n, _c in enumerate(HALF): PITEMS.insert(_c + _n + 1, (_c, True))
KOFF = HPB*KBR
FOFF = KOFF + 16*1024
PADOFF = FOFF + 16*len(HALF)*8
NPAD = 4
TOTR = PADOFF + 8*NPAD
NSTEP = HPB*NQ*4*(NC + len(HALF))
NZ = NSTEP + NPAD + 2
QSCALE = (DH ** -0.5) * math.log2(math.e)
NPREP = HPB*len(PITEMS)*16
PORD = 4
SCORE_BOUND = 64.0
V_LO = 2.0 ** -30
V_HI = 2.0 ** 50
NG = H // HPB

def slots(c):
    return [('h', c) if (c in HALF and x == HB) else ('b', x) for x in MXB]

def timeline(T):
    ktime = []; pvtime = {}; now = 0
    for t in range(T):
        for n, sl_ in enumerate(slots(t % NC)):
            if n == SPL: pvtime[t - SK] = now; now += 16
            ktime.append(now); now += 8 if sl_[0] == 'h' else 16
    for t in range(T - SK, T): pvtime[t] = now + 128*(t - T + SK) + 32
    vs = []
    gap = NC*128 // max(len(HALF), 1) // 4
    for t in range(T):
        for col in range(4):
            vs.append((pvtime[t] - DLT - (3 - col)*32, t, col, False))
            if t % NC in HALF:
                vs.append((pvtime[t] - SDL - (3 - col)*gap, t, col, True))
    vs.sort()
    vsteps = [(t, col, single, sum(1 for k in ktime if k < tm)) for (tm, t, col, single) in vs]
    return ktime, vsteps

def kern(ax, aw, ao, bx, bw, bo, out_hbm,
         x_b, w_b, wo_b, wt_s, kp_s, qt_s, vt_s, qf_s, ks_s, ot_s, ls_s, ob, bufa, bufb, s_s, p_c, l_c, o_c, v_c, lv_c, z_ref, isem, osem):
    b = pl.program_id(0)
    bufs = (bufa, bufb)

    def in_copy(src3, slot, j):
        x, w, wo = src3
        if j < 3:
            c0 = (D, 0, 2*D)[j]
            return pltpu.make_async_copy(w.at[:, c0:c0+D], w_b.at[slot, :, c0:c0+D], isem.at[slot, j])
        if j < 3 + NXC:
            i = j - 3
            return pltpu.make_async_copy(x.at[0, pl.ds(i*PR, PR), :], x_b.at[slot, pl.ds(i*PR, PR), :], isem.at[slot, j])
        return pltpu.make_async_copy(wo, wo_b.at[slot], isem.at[slot, j])

    @pl.when(b == 0)
    def _():
        for slot, src3 in enumerate(((ax, aw, ao), (bx, bw, bo))):
            for j in (0, 3, 1, 2, 4, 5, 6, 7):
                in_copy(src3, slot, j).start()
        for j in range(NZ):
            z_ref[j] = 0

    def wait_in(j):
        in_copy((ax, aw, ao), b, j).wait()

    def hslot(gp, hh):
        return gp*HPB + hh

    def ldk(sl, par, row, n=8):
        return bufs[1-par][pl.ds(pl.multiple_of(KOFF + sl*1024, 8) + row, n), :]

    def get_w(h, cols):
        r = pl.multiple_of(h*8, 8)
        if cols[-1] - cols[0] + 1 == len(cols):
            return pltpu.bitcast(qt_s[pl.ds(r, 8), cols[0]*128:(cols[-1]+1)*128], BF)
        return pltpu.bitcast(jnp.concatenate([qt_s[pl.ds(r, 8), c*128:(c+1)*128] for c in cols], axis=1), BF)

    def prep_all(gp, par):
        for hh in range(HPB):
            h = (2*gp + par)*HPB + hh
            for i0 in range(0, len(PITEMS), PORD):
                for d in range(DH):
                    for (c, single) in PITEMS[i0:i0 + PORD]:
                        n = 8 if single else 16
                        col = ks_s[h, ks_off(c, single): ks_off(c, single) + n, :][:, d:d+1]
                        base = hh*KBR + kb_off(c, single) + d*n
                        bufs[par][base: base + n, :] = pltpu.bitcast(jnp.broadcast_to(col, (n, 128)), U32)
                        yield

    NT = (((1,), (1,)), ((), ()))
    stats = {}
    def upd(name, val):
        stats[name] = val if name not in stats else jnp.maximum(stats[name], val)
    def proj_k(i):
        xc = x_b[b, pl.ds(i*PR, PR), :]
        kc = jnp.dot(xc, w_b[b, :, D:2*D], preferred_element_type=F32)
        upd("k", jnp.max(jnp.abs(kc).reshape(PR//8, 8, D), axis=0))
        kp_s[i*(PR//2):(i+1)*(PR//2), :] = pltpu.bitcast(kc.astype(BF), U32)
    def spread_k(i):
        for h in range(H):
            g, r = divmod(h, 8)
            grp, hh = divmod(h, HPB)
            par = grp % 2; sl = hslot(grp // 2, hh)
            kr = kp_s[i*(PR//2):(i+1)*(PR//2), g*128:(g+1)*128]
            if r: kr = pltpu.roll(kr, 128 - DH*r, axis=1)
            ko = KOFF + sl*1024 + i*(PR//2)
            bufs[1 - par][ko: ko + PR//2, :] = kr
            for c in range(i*(PR//CH), (i+1)*(PR//CH)):
                r0 = (c % (PR//CH))*(CH//2)
                ks_s[h, ks_off(c, False): ks_off(c, False) + 16, :] = pltpu.bitcast(kr[r0 + VB*8: r0 + VB*8 + 8], BF).astype(F32)
                if c in HALF:
                    kf = pltpu.bitcast(kr[r0 + HB*8: r0 + HB*8 + 8], BF).astype(F32)
                    fo = FOFF + (sl*len(HALF) + HALF.index(c))*8
                    bufs[1 - par][fo: fo + 8, :] = pltpu.bitcast(kf[0:8], U32)
                    ks_s[h, ks_off(c, True): ks_off(c, True) + 8, :] = kf[8:16]
    def proj_q(i):
        xc = x_b[b, pl.ds(i*PR, PR), :]
        q = lax.dot_general(wt_s[0:D, :], xc, NT, preferred_element_type=F32) * QSCALE
        upd("q", jnp.sum((q*q).reshape(H, DH, PR), axis=1))
        qb16 = q.astype(BF)
        qt_s[:, pl.ds(i*PR, PR)] = pltpu.bitcast(qb16, U32)
        qf_s[:, :, pl.ds(i*PR, PR)] = (qb16.astype(F32) if QRND else q).reshape(H, DH, PR)
    def proj_v(i):
        xc = x_b[b, pl.ds(i*PR, PR), :]
        v = lax.dot_general(wt_s[D:2*D, :], xc, NT, preferred_element_type=F32)
        va = jnp.abs(v)
        va = jnp.maximum(jnp.maximum(va[:, 0:128], va[:, 128:256]), jnp.maximum(va[:, 256:384], va[:, 384:512]))
        upd("v", jnp.max(va.reshape(H, DH, 128), axis=1))
        vt_s[:, pl.ds(i*PR, PR)] = v

    wait_in(0); wait_in(3)
    proj_k(0)
    for j in (1, 2, 4, 5, 6): wait_in(j)
    wt_s[0:D, :] = w_b[b, :, 0:D].T
    wt_s[D:2*D, :] = w_b[b, :, 2*D:3*D].T
    for i in range(1, NXC):
        proj_k(i); spread_k(i-1)
    for i in range(NXC):
        proj_q(i)
        if i == 0: spread_k(NXC-1)
    for i in range(NXC): proj_v(i)
    for _ in prep_all(0, 0): pass

    km = jnp.max(stats["k"], axis=0, keepdims=True)
    km = km * km
    kseg = jnp.concatenate([km[:, g*128:(g+1)*128] for g in range(4)], axis=0)
    for sh in (1, 2, 4, 8):
        kseg = kseg + pltpu.roll(kseg, sh, axis=1)
    kn2 = jnp.max(kseg)
    vh = jnp.max(stats["v"], axis=1, keepdims=True)
    safe = (jnp.max(stats["q"]) * kn2 <= SCORE_BOUND * SCORE_BOUND) & (jnp.min(vh) >= V_LO) & (jnp.max(vh) <= V_HI)
    if FORCE == 1: safe = safe & (b < 0)

    def vpu_col(z, par, h, hh, ct, c, single):
        buf = bufs[par]
        z0 = pl.multiple_of(z, 8)
        n = 8 if single else 16
        acc = None
        for d in range(0, DH, VG):
            kv = pltpu.bitcast(buf[pl.ds(z0 + hh*KBR + kb_off(c, single) + d*n, VG*n), :], F32)
            for x in range(VG):
                qs = jnp.broadcast_to(qf_s[h + z, d+x:d+x+1, ct*128:(ct+1)*128], (n, 128))
                t = kv[x*n:(x+1)*n] * qs
                acc = t if acc is None else acc + t
        return acc

    def pv_step(h, c, pb, oacc):
        r = pl.multiple_of(h*DH, DH)
        o = jnp.dot(vt_s[pl.ds(r, DH), c*CH:(c+1)*CH].astype(pb.dtype), pb, preferred_element_type=F32)
        return o if oacc is None else o + oacc

    def finish(h, qb, lacc, oacc):
        ls_s[qb, pl.ds(h, 1), :] = jnp.sum(lacc, axis=0, keepdims=True)
        ot_s[h, :, qb*TQ:(qb+1)*TQ] = oacc

    def lead_gen(gp, par):
        h0 = (2*gp + par)*HPB
        lv = [jnp.zeros((8, 128), F32)]*4
        for v, (t, col, single, _) in enumerate(timeline(HPB*NQ*NC)[1][:RC]):
            p = jnp.exp2(vpu_col(z_ref[v], par, h0, 0, col, t, single))
            v_c[v*16: v*16 + p.shape[0], :] = p
            lv[col] = lv[col] + (p if single else p[0:8] + p[8:16])
            if v == RC-1: lv_c[...] = jnp.concatenate(lv, axis=1)
            yield

    def block(gp, par):
        h0 = (2*gp + par)*HPB
        hprev = (h0 + H - 1) % H
        NUI = HPB*NQ
        T = NUI*NC - 0
        pads = [pl.multiple_of(PADOFF + 8*x + z_ref[NSTEP + x], 8) for x in range(NPAD)]
        pbs = {t: {} for t in range(T)}
        allc = [0, 1, 2, 3]
        laccs = {}; oaccs = {}
        ktime, vsteps = timeline(T)
        vnext = [0]; ng = [0]; nk = [0]; pend = []; lhist = []
        pgen = prep_all(gp, 1) if par == 0 else prep_all(jnp.minimum(gp+1, NG//2-1), 0)
        lgen = lead_gen(gp, 1) if par == 0 else lead_gen(jnp.minimum(gp+1, NG//2-1), 0)
        def acc_l(j, col, x):
            la = laccs.setdefault(j, [None]*4)
            la[col] = x if la[col] is None else la[col] + x
            lhist.append(la[col])
        def e_blk(j, s, cols):
            p = jnp.exp2(s)
            ll = p[0:8]
            for x in range(1, s.shape[0]//8):
                ll = ll + p[x*8:(x+1)*8]
            for n, col in enumerate(cols):
                acc_l(j, col, ll[:, n*128:(n+1)*128] if len(cols) > 1 else ll)
            return p, ll
        def share(x, tot, n, skip):
            if x < skip or x >= n: return 0
            return ((x-skip+1)*tot)//(n-skip) - ((x-skip)*tot)//(n-skip)
        def emit_vpu(upto_k=None, upto_t=None):
            while vnext[0] < len(vsteps):
                v = vnext[0]
                t, col, single, dead = vsteps[v]
                if not ((upto_k is not None and dead <= upto_k) or (upto_t is not None and min(x[0] for x in vsteps[v:]) <= upto_t)): break
                j, c = divmod(t, NC)
                pp, ll = e_blk(j, vpu_col(z_ref[v], par, h0 + j // NQ, j // NQ, (j % NQ)*4 + col, c, single), [col])
                pbs[t].setdefault('s' if single else 'v', {})[col] = pp
                if v >= NG0: pend.append(ll)
                vnext[0] += 1
        if RC:
            lv0 = lv_c[...]
            laccs[0] = [lv0[:, col*128:(col+1)*128] for col in allc]
            for v, (t, col, single, _) in enumerate(vsteps[:RC]):
                assert t < NC
                pbs[t].setdefault('s' if single else 'v', {})[col] = v_c[v*16: v*16 + (8 if single else 16), :]
            vnext[0] = RC
        def gates():
            emit_vpu(upto_k=nk[0])
            if LG and len(lhist) > LG + 4: pend.append(lhist[-LG - (nk[0] % 4)])
            while pend:
                bufs[1-par][pl.ds(pads[ng[0] % NPAD], 8), :] = pltpu.bitcast(pend.pop(0), U32)
                ng[0] += 1
            for _ in range(share(nk[0], NPREP, len(ktime) - PE, PS)): next(pgen)
            for _ in range(share(nk[0], RC, len(ktime) - LE, len(ktime) - LS)): next(lgen)
            nk[0] += 1
        def qk(t, sls):
            j, c = divmod(t, NC)
            h = h0 + j // NQ; sl = hslot(gp, j // NQ)
            if sls and sls[0][0] == 'h':
                gates()
                kf = bufs[1-par][pl.ds(pl.multiple_of(FOFF + (sl*len(HALF) + HALF.index(c))*8, 8), 8), :]
                s = jnp.dot(pltpu.bitcast(kf, F32)[:, 0:DH], qf_s[h, :, (j % NQ)*TQ:(j % NQ + 1)*TQ], preferred_element_type=F32)
                pbs[t]['h'] = e_blk(j, s, allc)[0]
                sls = sls[1:]
            if not sls: return
            ks = []
            for _, bb in sls:
                gates()
                ks.append(ldk(sl, par, c*CH//2 + bb*8))
            kk = pltpu.bitcast(jnp.concatenate(ks, axis=0) if len(ks) > 1 else ks[0], BF)[:, 0:DH]
            s = jnp.dot(kk, get_w(h, [(j % NQ)*4 + col for col in allc]), preferred_element_type=F32)
            for x, (_, bb) in enumerate(sls):
                pbs[t][bb] = e_blk(j, s[x*16:(x+1)*16], allc)[0]
        def gather_p(tb):
            emit_vpu(upto_t=tb)
            pp = pbs.pop(tb)
            pv = jnp.concatenate([pp['v'][col] for col in allc], axis=1)
            rows = []
            for bb in range(8):
                rows += [pv] if bb == VB else [pp[bb]] if bb in pp else [pp['h'], jnp.concatenate([pp['s'][col] for col in allc], axis=1)]
            return jnp.concatenate(rows, axis=0)
        def do_pv(tb):
            if tb < 0:
                c = NC + tb
                if tb == -SK: oaccs[-1] = o_c[...]
                oaccs[-1] = pv_step(hprev, c, pltpu.bitcast(p_c[(tb + SK)*CH//2:(tb + SK + 1)*CH//2, :], BF), oaccs[-1])
                if tb == -1:
                    finish(hprev, NQ-1, l_c[...], oaccs[-1])
                return
            j, c = divmod(tb, NC)
            oaccs[j] = pv_step(h0 + j // NQ, c, gather_p(tb), oaccs.get(j))
            if c == NC-1:
                finish(h0 + j // NQ, j % NQ, jnp.concatenate(laccs[j], axis=1), oaccs[j])
        for t in range(T):
            sls = slots(t % NC)
            qk(t, sls[:SPL])
            if t >= SK or CG == 0: do_pv(t - SK)
            qk(t, sls[SPL:])
            if t < SK and CG == 1: do_pv(t - SK)
        for x in range(SK):
            p_c[x*CH//2:(x+1)*CH//2, :] = pltpu.bitcast(gather_p(T - SK + x).astype(BF), U32)
        l_c[...] = jnp.concatenate(laccs[NUI-1], axis=1)
        o_c[...] = oaccs[NUI-1]
        for _ in lgen: pass

    @pl.when(safe)
    def _():
        p_c[...] = jnp.zeros(p_c.shape, U32)
        l_c[...] = jnp.ones(l_c.shape, F32)
        o_c[...] = jnp.zeros(o_c.shape, F32)
        for _ in lead_gen(0, 0): pass
        def fb(i, c):
            for par in range(2):
                @pl.when(z_ref[NSTEP + NPAD + par] == 0)
                def _():
                    block(i, par)
            return c
        lax.fori_loop(0, NG//2, fb, 0)
        o = o_c[...]
        for x in range(SK):
            o = pv_step(H-1, NC - SK + x, pltpu.bitcast(p_c[x*CH//2:(x+1)*CH//2, :], BF), o)
        finish(H-1, NQ-1, l_c[...], o)

    def slow_body(gp, carry):
        SC = 256
        for par in range(2):
            def unit(u, c2):
                hh = u // NQ; qb = u % NQ
                h = (2*gp + par)*HPB + hh
                r8 = pl.multiple_of(h*8, 8)
                c0 = pl.multiple_of(qb*TQ, TQ)
                w = pltpu.bitcast(qt_s[pl.ds(r8, 8), pl.ds(c0, TQ)], BF)
                def p1(c, m):
                    ro = pl.multiple_of(c*(SC//2), 8)
                    kk = pltpu.bitcast(ldk(hslot(gp, hh), par, ro, SC//2), BF)[:, 0:DH]
                    s = jnp.dot(kk, w, preferred_element_type=F32)
                    s_s[pl.ds(pl.multiple_of(c*SC, SC), SC), :] = s
                    return jnp.maximum(m, jnp.max(s, axis=0, keepdims=True))
                m = lax.fori_loop(0, S//SC, p1, jnp.full((1, TQ), -jnp.inf, F32))
                def p2(c, lo):
                    l, o = lo
                    co = pl.multiple_of(c*SC, SC)
                    p = jnp.exp2(s_s[pl.ds(co, SC), :] - m)
                    vt = vt_s[pl.ds(pl.multiple_of(h*DH, DH), DH), pl.ds(co, SC)]
                    return (l + jnp.sum(p.reshape(SC//8, 8, TQ), axis=0),
                            o + jnp.dot(vt, p, preferred_element_type=F32))
                l, o = lax.fori_loop(0, S//SC, p2, (jnp.zeros((8, TQ), F32), jnp.zeros((DH, TQ), F32)))
                ot_s[h, :, pl.ds(c0, TQ)] = o
                ls_s[qb, pl.ds(h, 1), :] = jnp.sum(l, axis=0, keepdims=True)
                return c2
            lax.fori_loop(0, HPB*NQ, unit, 0)
        return carry

    @pl.when(jnp.logical_not(safe))
    def _():
        lax.fori_loop(0, NG//2, slow_body, 0)

    wait_in(3 + NXC)
    ls_s[...] = 1.0 / ls_s[...]
    def out_copy(bb, i):
        return pltpu.make_async_copy(ob.at[pl.ds(i*PR, PR), :],
                                     out_hbm.at[0, pl.ds(i*PR, PR), pl.ds(pl.multiple_of(bb*D, D), D)], osem.at[i])
    @pl.when(b == 1)
    def _():
        for i in range(NXC):
            out_copy(0, i).wait()
    for i in range(NXC):
        oc = jnp.concatenate([ot_s[h, :, pl.ds(i*PR, PR)] * jnp.broadcast_to(ls_s[i, h:h+1, :], (DH, PR)) for h in range(H)], axis=0)
        oc = oc.T.astype(BF)
        r = jnp.dot(oc, wo_b[b], preferred_element_type=F32)
        ob[pl.ds(i*PR, PR), :] = r.astype(BF)
        out_copy(b, i).start()
    @pl.when(b == 1)
    def _():
        for i in range(NXC):
            out_copy(1, i).wait()

@jax.jit
def pallas_concat_heads__softmax_full_mha__softmax_full_mha__prompt_kernel(A_x, A_wqkv, A_wo, B_x, B_wqkv, B_wo):
    ax, aw, ao, bx, bw, bo = A_x, A_wqkv, A_wo, B_x, B_wqkv, B_wo
    any_spec = pl.BlockSpec(memory_space=pl.ANY)
    return pl.pallas_call(kern, out_shape=jax.ShapeDtypeStruct((1, S, 2*D), BF),
        grid=(2,),
        in_specs=[any_spec]*6, out_specs=any_spec,
        scratch_shapes=[pltpu.VMEM((2,S,D),BF), pltpu.VMEM((2,D,3*D),BF), pltpu.VMEM((2,D,D),BF),
                        pltpu.VMEM((2*D,D),BF),
                        pltpu.VMEM((S//2,D),U32), pltpu.VMEM((D//2,S),U32), pltpu.VMEM((D,S),F32),
                        pltpu.VMEM((H,DH,S),F32), pltpu.VMEM((H,NGT*8,128),F32),
                        pltpu.VMEM((H,DH,S),F32), pltpu.VMEM((NQ,H,TQ),F32), pltpu.VMEM((S,D),BF),
                        pltpu.VMEM((TOTR,128),U32), pltpu.VMEM((TOTR,128),U32),
                        pltpu.VMEM((S,TQ),F32),
                        pltpu.VMEM((SK*CH//2,TQ),U32), pltpu.VMEM((8,TQ),F32), pltpu.VMEM((DH,TQ),F32),
                        pltpu.VMEM((max(RC,1)*16,128),F32), pltpu.VMEM((8,TQ),F32),
                        pltpu.SMEM((NZ,), jnp.int32),
                        pltpu.SemaphoreType.DMA((2, NXC+4)), pltpu.SemaphoreType.DMA((NXC,))],
        compiler_params=pltpu.CompilerParams(vmem_limit_bytes=100*1024*1024, dimension_semantics=("arbitrary",)))(ax, aw, ao, bx, bw, bo)
```

```python
import functools
import math

import jax
import jax.numpy as jnp
from jax import lax
from jax.experimental import pallas as pl
from jax.experimental.pallas import tpu as pltpu

S = 2048; D = 512; H = 32; DH = 16
TQ = 512
CH = 128
PR = 512
NQ = S // TQ; NC = S // CH; NXC = S // PR
F32 = jnp.float32; BF = jnp.bfloat16; U32 = jnp.uint32

QSCALE = (DH ** -0.5) * math.log2(math.e)
SCORE_BOUND = 64.0
V_LO = 2.0 ** -30
V_HI = 2.0 ** 50

SK = 2
SPL = 2
LG = 48
PS = 8; PE = 12
VG = 4; PORD = 4
NG0 = 0
DLT = 24; SDL = 80; SO = (80, 16)
RC = 4; LS = 8
CP = (5, 5)
XC = 4
HALF = [c for c in range(NC) if c % 2]
VB = 0
MXB = [x for x in range(7, -1, -1) if x != VB]
HB = MXB[SPL]
NGT = 2 * NC + len(HALF)
KBR = NGT * DH * 8
PITEMS = [(c, False) for c in range(NC)]
for _n, _c in enumerate(HALF):
    PITEMS.insert(_c + _n + 1, (_c, True))
NPREP = len(PITEMS) * DH
NPH = 3
BLOCKS = ((0, 1), (2,))
NIT = -(-H // NPH)
KOFF = KBR
FOFF = KOFF + NIT * (S // 2)
XOFF = FOFF + NIT * len(HALF) * 8
XFO = XOFF + NIT * XC * (CH // 2)
PADOFF = XFO + NIT * XC * 8
NPAD = 4
TOTR = PADOFF + 8 * NPAD
NSTEP = 2 * NQ * 4 * (NC + len(HALF))
NZ = NSTEP + NPAD
OCH = ((0, 128), (128, 384), (512, 512), (1024, 512), (1536, 384), (1920, 128))
COLS = (0, 1, 2, 3)


def kb_off(c, single):
    return (2 * NC + HALF.index(c)) * DH * 8 if single else c * 2 * DH * 8


def ks_off(c, single):
    return (2 * NC + HALF.index(c)) * 8 if single else c * 16


def slots(c):
    return [('h', c) if (c in HALF and x == HB) else ('b', x) for x in MXB]


def timeline(T):
    ktime = []; pvtime = {}; now = 0
    for t in range(T):
        for n, sl in enumerate(slots(t % NC)):
            if n == SPL:
                pvtime[t - SK] = now; now += 16
            ktime.append(now); now += 8 if sl[0] == 'h' else 16
    for t in range(T - SK, T):
        pvtime[t] = now + 128 * (t - T + SK) + 32
    vs = [(pvtime[t] - DLT - (3 - col) * 32, t, col, False) for t in range(T) for col in COLS]
    free = sorted(pvtime[t] - o for t in range(-SK, T) for o in SO)
    for t in range(T - 1, -1, -1):
        if t % NC in HALF:
            for col in reversed(COLS):
                tm = [x for x in free if x <= pvtime[t] - SDL][-1]
                free.remove(tm)
                vs.append((tm, t, col, True))
    vs.sort()
    return len(ktime), [(t, col, single, sum(1 for k in ktime if k < tm)) for (tm, t, col, single) in vs]


def share(x, tot, n, skip):
    if x < skip or x >= n:
        return 0
    return ((x - skip + 1) * tot) // (n - skip) - ((x - skip) * tot) // (n - skip)


def _kernel(ax, aw, ao, bx, bw, bo, out_hbm,
            x_b, w_b, wo_b, wt_s, kp_s, qt_s, vt_s, qf_s, ks_s, ot_s, ls_s, ob, bufa, bufb, bufc,
            s_s, p_c, l_c, o_c, v_c, lv_c, vm_s, z_ref, isem, osem):
    b = pl.program_id(0)
    bufs = (bufa, bufb, bufc)

    def kbuf(ph):
        return bufs[(ph + 2) % NPH]

    def in_refs(src3, slot, j):
        x, w, wo = src3
        if j < 3:
            c0 = (D, 0, 2 * D)[j]
            return w.at[:, c0:c0 + D], w_b.at[slot, :, c0:c0 + D]
        if j < 3 + NXC:
            i = j - 3
            return x.at[0, i * PR:(i + 1) * PR, :], x_b.at[slot, i * PR:(i + 1) * PR, :]
        return wo, wo_b.at[slot]

    @pl.when(b == 0)
    def _():
        for slot, src3 in enumerate(((ax, aw, ao), (bx, bw, bo))):
            for j in (0, 3, 4, 5, 6, 1, 2, 7):
                src, dst = in_refs(src3, slot, j)
                pltpu.make_async_copy(src, dst, isem.at[slot, j]).start()
        for j in range(NZ):
            z_ref[j] = 0

    def wait_in(j):
        dst = in_refs((ax, aw, ao), b, j)[1]
        pltpu.make_async_copy(dst, dst, isem.at[b, j]).wait()

    def ldk(it, ph, row, n=8):
        return kbuf(ph)[pl.ds(pl.multiple_of(KOFF + it * (S // 2), 8) + row, n), :]

    def prep_gen(h, ph):
        for i0 in range(0, len(PITEMS), PORD):
            for d in range(DH):
                for (c, single) in PITEMS[i0:i0 + PORD]:
                    n = 8 if single else 16
                    col = ks_s[h, ks_off(c, single): ks_off(c, single) + n, :][:, d:d + 1]
                    base = kb_off(c, single) + d * n
                    bufs[ph][base: base + n, :] = pltpu.bitcast(jnp.broadcast_to(col, (n, 128)), U32)
                    yield

    nt_dims = (((1,), (1,)), ((), ()))
    stats = {}

    def upd(name, val):
        stats[name] = val if name not in stats else jnp.maximum(stats[name], val)

    def proj_k(i):
        xc = x_b[b, pl.ds(i * PR, PR), :]
        kc = jnp.dot(xc, w_b[b, :, D:2 * D], preferred_element_type=F32)
        upd("k", jnp.max(jnp.abs(kc).reshape(PR // 8, 8, D), axis=0))
        kp_s[i * (PR // 2):(i + 1) * (PR // 2), :] = pltpu.bitcast(kc.astype(BF), U32)

    def spread_k(i):
        for h in range(H):
            g, r = divmod(h, 8)
            it, ph = divmod(h, NPH)
            kr = kp_s[i * (PR // 2):(i + 1) * (PR // 2), g * 128:(g + 1) * 128]
            if r:
                kr = pltpu.roll(kr, 128 - DH * r, axis=1)
            ko = KOFF + it * (S // 2) + i * (PR // 2)
            kbuf(ph)[ko: ko + PR // 2, :] = kr
            if ph == 1 and i == 0:
                xo = XOFF + it * XC * (CH // 2)
                kbuf(0)[xo: xo + XC * (CH // 2), :] = kr[0: XC * (CH // 2)]
            for c in range(i * (PR // CH), (i + 1) * (PR // CH)):
                r0 = (c % (PR // CH)) * (CH // 2)
                ks_s[h, ks_off(c, False): ks_off(c, False) + 16, :] = (
                    pltpu.bitcast(kr[r0 + VB * 8: r0 + VB * 8 + 8], BF).astype(F32))
                if c in HALF:
                    kf = pltpu.bitcast(kr[r0 + HB * 8: r0 + HB * 8 + 8], BF).astype(F32)
                    fo = FOFF + (it * len(HALF) + HALF.index(c)) * 8
                    kbuf(ph)[fo: fo + 8, :] = pltpu.bitcast(kf[0:8], U32)
                    if ph == 1 and c < XC:
                        xf = XFO + (it * XC + c) * 8
                        kbuf(0)[xf: xf + 8, :] = pltpu.bitcast(kf[0:8], U32)
                    ks_s[h, ks_off(c, True): ks_off(c, True) + 8, :] = kf[8:16]

    def proj_q(i):
        xc = x_b[b, pl.ds(i * PR, PR), :]
        q = lax.dot_general(wt_s[0:D, :], xc, nt_dims, preferred_element_type=F32) * QSCALE
        upd("q", jnp.sum((q * q).reshape(H, DH, PR), axis=1))
        qt_s[:, pl.ds(i * PR, PR)] = pltpu.bitcast(q.astype(BF), U32)
        qf_s[:, :, pl.ds(i * PR, PR)] = q.reshape(H, DH, PR)

    def proj_v(i):
        xc = x_b[b, pl.ds(i * PR, PR), :]
        v = lax.dot_general(wt_s[D:2 * D, :], xc, nt_dims, preferred_element_type=F32)
        va = jnp.abs(v)
        va = jnp.maximum(jnp.maximum(va[:, 0:128], va[:, 128:256]),
                         jnp.maximum(va[:, 256:384], va[:, 384:512]))
        va = jnp.max(va.reshape(H, 2, 8, 128), axis=1)
        vm_s[...] = va if i == 0 else jnp.maximum(vm_s[...], va)
        vt_s[:, pl.ds(i * PR, PR)] = v

    wait_in(0); wait_in(3)
    proj_k(0)
    wait_in(4); wait_in(5)
    proj_k(1)
    spread_k(0)
    proj_k(2)
    wait_in(6); wait_in(1); wait_in(2)
    wt_s[0:D, :] = w_b[b, :, 0:D].T
    wt_s[D:2 * D, :] = w_b[b, :, 2 * D:3 * D].T
    proj_k(3)
    spread_k(1)
    for i in range(NXC):
        proj_q(i)
        if i < 2:
            spread_k(2 + i)
    for i in range(NXC):
        proj_v(i)

    km = jnp.max(stats["k"], axis=0, keepdims=True)
    km = km * km
    kseg = jnp.concatenate([km[:, g * 128:(g + 1) * 128] for g in range(4)], axis=0)
    for sh in (1, 2, 4, 8):
        kseg = kseg + pltpu.roll(kseg, sh, axis=1)
    safe_qk = jnp.max(stats["q"]) * jnp.max(kseg) <= SCORE_BOUND * SCORE_BOUND

    def vpu_col(z, ph, h, ct, c, single):
        z0 = pl.multiple_of(z, 8)
        n = 8 if single else 16
        acc = None
        for d in range(0, DH, VG):
            kv = pltpu.bitcast(bufs[ph][pl.ds(z0 + kb_off(c, single) + d * n, VG * n), :], F32)
            for x in range(VG):
                qs = jnp.broadcast_to(qf_s[h + z, d + x:d + x + 1, ct * 128:(ct + 1) * 128], (n, 128))
                t = kv[x * n:(x + 1) * n] * qs
                acc = t if acc is None else acc + t
        return acc

    def pv_step(h, c, pb, oacc):
        r = pl.multiple_of(h * DH, DH)
        o = jnp.dot(vt_s[pl.ds(r, DH), c * CH:(c + 1) * CH].astype(pb.dtype), pb,
                    preferred_element_type=F32)
        return o if oacc is None else o + oacc

    def carried_p(x):
        return pltpu.bitcast(p_c[x * CH // 2:(x + 1) * CH // 2, :], BF)

    def finish(h, qb, lacc, oacc):
        ls_s[qb, pl.ds(h, 1), :] = jnp.sum(lacc, axis=0, keepdims=True)
        ot_s[h, :, qb * TQ:(qb + 1) * TQ] = oacc

    lead = [x[:3] for x in timeline(NQ * NC)[1][:RC]]

    def lead_gen(h, ph):
        lv = [jnp.zeros((8, 128), F32)] * 4
        for v, (t, col, single) in enumerate(lead):
            p = jnp.exp2(vpu_col(z_ref[v], ph, h, col, t, single))
            v_c[v * 16: v * 16 + p.shape[0], :] = p
            lv[col] = lv[col] + (p if single else p[0:8] + p[8:16])
            if v == RC - 1:
                lv_c[...] = jnp.concatenate(lv, axis=1)
            yield

    def block(it, phs):
        h0 = it * NPH + phs[0]
        hprev = (h0 + H - 1) % H
        nui = len(phs) * NQ
        T = nui * NC
        pads = [pl.multiple_of(PADOFF + 8 * x + z_ref[NSTEP + x], 8) for x in range(NPAD)]
        pbs = {t: {} for t in range(T)}
        laccs = {}; oaccs = {}
        nkt, vsteps = timeline(T)
        assert [x[:3] for x in vsteps[:RC]] == lead
        vnext = [RC]; ng = [0]; nk = [0]; pend = []; lhist = []
        pgen = [prep_gen(jnp.minimum(h0 + n + 2, H - 1), (ph + 2) % NPH) for n, ph in enumerate(phs)]
        phn = (phs[-1] + 1) % NPH
        lgen = lead_gen(jnp.minimum(h0 + len(phs), H - 1), phn)
        kph = nkt // len(phs)

        def e_blk(j, s, cols):
            p = jnp.exp2(s)
            ll = p[0:8]
            for x in range(1, s.shape[0] // 8):
                ll = ll + p[x * 8:(x + 1) * 8]
            la = laccs.setdefault(j, [None] * 4)
            for n, col in enumerate(cols):
                x = ll[:, n * 128:(n + 1) * 128] if len(cols) > 1 else ll
                la[col] = x if la[col] is None else la[col] + x
                lhist.append(la[col])
            return p, ll

        def emit_vpu(upto_k=None, upto_t=None):
            while vnext[0] < len(vsteps):
                v = vnext[0]
                t, col, single, dead = vsteps[v]
                if not ((upto_k is not None and dead <= upto_k)
                        or (upto_t is not None and min(x[0] for x in vsteps[v:]) <= upto_t)):
                    break
                j, c = divmod(t, NC)
                s = vpu_col(z_ref[v], phs[j // NQ], h0 + j // NQ, (j % NQ) * 4 + col, c, single)
                pp, ll = e_blk(j, s, [col])
                pbs[t].setdefault('s' if single else 'v', {})[col] = pp
                if v >= NG0:
                    pend.append(ll)
                vnext[0] += 1

        lv0 = lv_c[...]
        laccs[0] = [lv0[:, col * 128:(col + 1) * 128] for col in COLS]
        for v, (t, col, single) in enumerate(lead):
            pbs[t].setdefault('s' if single else 'v', {})[col] = v_c[v * 16: v * 16 + (8 if single else 16), :]

        def gates():
            n, kx = divmod(nk[0], kph)
            gb = kbuf(phs[n - 1]) if (n >= 1 and kx < XC * 7) else kbuf(phs[n])
            emit_vpu(upto_k=nk[0])
            if len(lhist) > LG + 4:
                pend.append(lhist[-LG - (nk[0] % 4)])
            while pend:
                gb[pl.ds(pads[ng[0] % NPAD], 8), :] = pltpu.bitcast(pend.pop(0), U32)
                ng[0] += 1
            for _ in range(share(kx, NPREP, kph - PE, max(PS, XC * 7) if n >= 1 else PS)):
                next(pgen[n])
            for _ in range(share(nk[0], RC, nkt, nkt - LS)):
                bufs[phn][pl.ds(pads[ng[0] % NPAD], 8), :] = pltpu.bitcast(lhist[-LG - (nk[0] % 4)], U32)
                next(lgen)
            nk[0] += 1

        def qk(t, sls):
            j, c = divmod(t, NC)
            h = h0 + j // NQ; ph = phs[j // NQ]; qb = j % NQ
            dup = (j == NQ and c < XC)
            hpos = [x for x, y in enumerate(sls) if y[0] == 'h']
            if hpos and hpos[0] > 0:
                qk(t, sls[:hpos[0]]); qk(t, sls[hpos[0]:])
                return
            if hpos:
                gates()
                if dup:
                    kf = kbuf(ph - 1)[pl.ds(pl.multiple_of(XFO + (it * XC + c) * 8, 8), 8), :]
                else:
                    fo = FOFF + (it * len(HALF) + HALF.index(c)) * 8
                    kf = kbuf(ph)[pl.ds(pl.multiple_of(fo, 8), 8), :]
                s = jnp.dot(pltpu.bitcast(kf, F32)[:, 0:DH], qf_s[h, :, qb * TQ:(qb + 1) * TQ],
                            preferred_element_type=F32)
                pbs[t]['h'] = e_blk(j, s, COLS)[0]
                sls = sls[1:]
            if not sls:
                return
            ks = []
            for _, bb in sls:
                gates()
                row = c * CH // 2 + bb * 8
                if dup:
                    ks.append(kbuf(ph - 1)[pl.ds(pl.multiple_of(XOFF + it * XC * (CH // 2), 8) + row, 8), :])
                else:
                    ks.append(ldk(it, ph, row))
            kk = pltpu.bitcast(jnp.concatenate(ks, axis=0) if len(ks) > 1 else ks[0], BF)[:, 0:DH]
            w = pltpu.bitcast(qt_s[pl.ds(pl.multiple_of(h * 8, 8), 8), qb * TQ:(qb + 1) * TQ], BF)
            s = jnp.dot(kk, w, preferred_element_type=F32)
            for x, (_, bb) in enumerate(sls):
                pbs[t][bb] = e_blk(j, s[x * 16:(x + 1) * 16], COLS)[0]

        def gather_p(tb):
            emit_vpu(upto_t=tb)
            pp = pbs.pop(tb)
            pv = jnp.concatenate([pp['v'][col] for col in COLS], axis=1)
            rows = []
            for bb in range(8):
                if bb == VB:
                    rows.append(pv)
                elif bb in pp:
                    rows.append(pp[bb])
                else:
                    rows += [pp['h'], jnp.concatenate([pp['s'][col] for col in COLS], axis=1)]
            return jnp.concatenate(rows, axis=0)

        def do_pv(tb):
            if tb < 0:
                if tb == -SK:
                    oaccs[-1] = o_c[...]
                oaccs[-1] = pv_step(hprev, NC + tb, carried_p(tb + SK), oaccs[-1])
                if tb == -1:
                    finish(hprev, NQ - 1, l_c[...], oaccs[-1])
                return
            j, c = divmod(tb, NC)
            oaccs[j] = pv_step(h0 + j // NQ, c, gather_p(tb), oaccs.get(j))
            if c == NC - 1:
                finish(h0 + j // NQ, j % NQ, jnp.concatenate(laccs[j], axis=1), oaccs[j])

        for t in range(T):
            sls = slots(t % NC)
            cut = SPL if t >= SK else CP[t]
            qk(t, sls[:cut])
            do_pv(t - SK)
            qk(t, sls[cut:])
        for x in range(SK):
            p_c[x * CH // 2:(x + 1) * CH // 2, :] = pltpu.bitcast(gather_p(T - SK + x).astype(BF), U32)
        l_c[...] = jnp.concatenate(laccs[nui - 1], axis=1)
        o_c[...] = oaccs[nui - 1]

    for hh in range(2):
        for _ in prep_gen(hh, hh):
            pass
    p_c[...] = jnp.zeros(p_c.shape, U32)
    l_c[...] = jnp.ones(l_c.shape, F32)
    o_c[...] = jnp.zeros(o_c.shape, F32)
    for _ in lead_gen(0, 0):
        pass

    @pl.when(safe_qk)
    def _():
        def body(i, c):
            block(i, BLOCKS[0])
            pl.when(i * NPH + BLOCKS[1][0] < H)(functools.partial(block, i, BLOCKS[1]))
            return c
        lax.fori_loop(0, NIT, body, 0)

    o = o_c[...]
    for x in range(SK):
        o = pv_step(H - 1, NC - SK + x, carried_p(x), o)
    finish(H - 1, NQ - 1, l_c[...], o)
    vh = jnp.max(jnp.max(vm_s[...], axis=1), axis=1, keepdims=True)
    safe = safe_qk & (jnp.min(vh) >= V_LO) & (jnp.max(vh) <= V_HI)

    def slow_body(it, carry):
        sc = 256
        for ph in range(NPH):
            h = it * NPH + ph

            def unit(qb, c2):
                c0 = pl.multiple_of(qb * TQ, TQ)
                w = pltpu.bitcast(qt_s[pl.ds(pl.multiple_of(h * 8, 8), 8), pl.ds(c0, TQ)], BF)

                def p1(c, m):
                    ro = pl.multiple_of(c * (sc // 2), 8)
                    kk = pltpu.bitcast(ldk(it, ph, ro, sc // 2), BF)[:, 0:DH]
                    s = jnp.dot(kk, w, preferred_element_type=F32)
                    s_s[pl.ds(pl.multiple_of(c * sc, sc), sc), :] = s
                    return jnp.maximum(m, jnp.max(s, axis=0, keepdims=True))
                m = lax.fori_loop(0, S // sc, p1, jnp.full((1, TQ), -jnp.inf, F32))

                def p2(c, lo):
                    l, o = lo
                    co = pl.multiple_of(c * sc, sc)
                    p = jnp.exp2(s_s[pl.ds(co, sc), :] - m)
                    vt = vt_s[pl.ds(pl.multiple_of(h * DH, DH), DH), pl.ds(co, sc)]
                    return (l + jnp.sum(p.reshape(sc // 8, 8, TQ), axis=0),
                            o + jnp.dot(vt, p, preferred_element_type=F32))
                l, o = lax.fori_loop(0, S // sc, p2,
                                     (jnp.zeros((8, TQ), F32), jnp.zeros((DH, TQ), F32)))
                ot_s[h, :, pl.ds(c0, TQ)] = o
                ls_s[qb, pl.ds(h, 1), :] = jnp.sum(l, axis=0, keepdims=True)
                return c2
            lax.fori_loop(0, jnp.where(h < H, NQ, 0), unit, 0)
        return carry

    @pl.when(jnp.logical_not(safe))
    def _():
        lax.fori_loop(0, NIT, slow_body, 0)

    wait_in(3 + NXC)

    def out_copy(bb, n):
        r0, nr = OCH[n]
        return pltpu.make_async_copy(
            ob.at[r0:r0 + nr, :],
            out_hbm.at[0, r0:r0 + nr, pl.ds(pl.multiple_of(bb * D, D), D)], osem.at[n])

    @pl.when(b == 1)
    def _():
        for n in range(len(OCH)):
            out_copy(0, n).wait()

    for n, (r0, nr) in enumerate(OCH):
        qb, c0 = divmod(r0, TQ)
        inv = 1.0 / ls_s[qb, :, c0:c0 + nr]
        oc = (ot_s[:, :, r0:r0 + nr] * inv.reshape(H, 1, nr)).reshape(D, nr).T.astype(BF)
        r = jnp.dot(oc, wo_b[b], preferred_element_type=F32)
        ob[r0:r0 + nr, :] = r.astype(BF)
        out_copy(b, n).start()

    @pl.when(b == 1)
    def _():
        for n in range(len(OCH)):
            out_copy(1, n).wait()


@jax.jit
def pallas_concat_heads__softmax_full_mha__softmax_full_mha__prompt_kernel(
    A_x: jax.Array,
    A_wqkv: jax.Array,
    A_wo: jax.Array,
    B_x: jax.Array,
    B_wqkv: jax.Array,
    B_wo: jax.Array,
):
    any_spec = pl.BlockSpec(memory_space=pl.ANY)
    vm = pltpu.VMEM
    return pl.pallas_call(
        _kernel,
        out_shape=jax.ShapeDtypeStruct((1, S, 2 * D), BF),
        grid=(2,),
        in_specs=[any_spec] * 6,
        out_specs=any_spec,
        scratch_shapes=[
            vm((2, S, D), BF), vm((2, D, 3 * D), BF), vm((2, D, D), BF),
            vm((2 * D, D), BF),
            vm((S // 2, D), U32), vm((D // 2, S), U32), vm((D, S), F32),
            vm((H, DH, S), F32), vm((H, NGT * 8, 128), F32),
            vm((H, DH, S), F32), vm((NQ, H, TQ), F32), vm((S, D), BF),
            vm((TOTR, 128), U32), vm((TOTR, 128), U32), vm((TOTR, 128), U32),
            vm((S, TQ), F32),
            vm((SK * CH // 2, TQ), U32), vm((8, TQ), F32), vm((DH, TQ), F32),
            vm((RC * 16, 128), F32), vm((8, TQ), F32), vm((H, 8, 128), F32),
            pltpu.SMEM((NZ,), jnp.int32),
            pltpu.SemaphoreType.DMA((2, NXC + 4)), pltpu.SemaphoreType.DMA((len(OCH),)),
        ],
        compiler_params=pltpu.CompilerParams(
            vmem_limit_bytes=100 * 1024 * 1024, dimension_semantics=("arbitrary",)),
    )(A_x, A_wqkv, A_wo, B_x, B_wqkv, B_wo)
```

```python
import functools
import math

import jax
import jax.numpy as jnp
from jax import lax
from jax.experimental import pallas as pl
from jax.experimental.pallas import tpu as pltpu

S = 2048; D = 512; H = 32; DH = 16
TQ = 512
CH = 128
PR = 512
NQ = S // TQ; NC = S // CH; NXC = S // PR
F32 = jnp.float32; BF = jnp.bfloat16; U32 = jnp.uint32

QSCALE = (DH ** -0.5) * math.log2(math.e)
SCORE_BOUND = 64.0
V_LO = 2.0 ** -30
V_HI = 2.0 ** 50

SK = 2
SPL = 2
LG = 47
PS = 8; PE = 12
VG = 3; PORD = 4
NG0 = 0
DLT = 24; SDL = 80; SO = (80, 16)
RC = 4; LS = 8
CP = (5, 5)
XC = 4
HALF = [c for c in range(NC) if c % 2]
VB = 0
MXB = [x for x in range(7, -1, -1) if x != VB]
HB = MXB[SPL]
NGT = 2 * NC + len(HALF)
KBR = NGT * DH * 8
PITEMS = [(c, False) for c in range(NC)]
for _n, _c in enumerate(HALF):
    PITEMS.insert(_c + _n + 1, (_c, True))
NPREP = len(PITEMS) * DH
NPH = 3
BLOCKS = ((0, 1), (2,))
NIT = -(-H // NPH)
KOFF = KBR
FOFF = KOFF + NIT * (S // 2)
XOFF = FOFF + NIT * len(HALF) * 8
XFO = XOFF + NIT * XC * (CH // 2)
PADOFF = XFO + NIT * XC * 8
NPAD = 4
TOTR = PADOFF + 32 * NPAD
assert all(x % 32 == 0 for x in (KOFF, FOFF, XOFF, XFO, PADOFF, TOTR))
NSTEP = 2 * NQ * 4 * (NC + len(HALF))
NZ = NSTEP + NPAD
OCH = ((0, 128), (128, 384), (512, 512), (1024, 512), (1536, 384), (1920, 128))
COLS = (0, 1, 2, 3)


def kb_off(c, single):
    return (2 * NC + HALF.index(c)) * DH * 8 if single else c * 2 * DH * 8


def ks_off(c, single):
    return (2 * NC + HALF.index(c)) * 8 if single else c * 16


def slots(c):
    return [('h', c) if (c in HALF and x == HB) else ('b', x) for x in MXB]


def timeline(T):
    ktime = []; pvtime = {}; now = 0
    for t in range(T):
        for n, sl in enumerate(slots(t % NC)):
            if n == SPL:
                pvtime[t - SK] = now; now += 16
            ktime.append(now); now += 8 if sl[0] == 'h' else 16
    for t in range(T - SK, T):
        pvtime[t] = now + 128 * (t - T + SK) + 32
    vs = [(pvtime[t] - DLT - (3 - col) * 32, t, col, False) for t in range(T) for col in COLS]
    free = sorted(pvtime[t] - o for t in range(-SK, T) for o in SO)
    for t in range(T - 1, -1, -1):
        if t % NC in HALF:
            for col in reversed(COLS):
                tm = [x for x in free if x <= pvtime[t] - SDL][-1]
                free.remove(tm)
                vs.append((tm, t, col, True))
    vs.sort()
    return len(ktime), [(t, col, single, sum(1 for k in ktime if k < tm)) for (tm, t, col, single) in vs]


def share(x, tot, n, skip):
    if x < skip or x >= n:
        return 0
    return ((x - skip + 1) * tot) // (n - skip) - ((x - skip) * tot) // (n - skip)


def _kernel(ax, aw, ao, bx, bw, bo, out_hbm,
            x_b, w_b, wo_b, wt_s, kp_s, qt_s, vt_s, qf_s, ks_s, ot_s, ls_s, ob, bufa, bufb, bufc,
            s_s, p_c, l_c, o_c, v_c, lv_c, vm_s, z_ref, isem, osem):
    b = pl.program_id(0)
    bufs = (bufa, bufb, bufc)

    def kbuf(ph):
        return bufs[(ph + 2) % NPH]

    def in_refs(src3, slot, j):
        x, w, wo = src3
        if j < 3:
            c0 = (D, 0, 2 * D)[j]
            return w.at[:, c0:c0 + D], w_b.at[slot, :, c0:c0 + D]
        if j < 3 + NXC:
            i = j - 3
            return x.at[0, i * PR:(i + 1) * PR, :], x_b.at[slot, i * PR:(i + 1) * PR, :]
        return wo, wo_b.at[slot]

    @pl.when(b == 0)
    def _():
        for slot, src3 in enumerate(((ax, aw, ao), (bx, bw, bo))):
            for j in (0, 3, 4, 5, 6, 1, 2, 7):
                src, dst = in_refs(src3, slot, j)
                pltpu.make_async_copy(src, dst, isem.at[slot, j]).start()
        for j in range(NZ):
            z_ref[j] = 0

    def wait_in(j):
        dst = in_refs((ax, aw, ao), b, j)[1]
        pltpu.make_async_copy(dst, dst, isem.at[b, j]).wait()

    def ldk(it, ph, row, n=8):
        return kbuf(ph)[pl.ds(pl.multiple_of(KOFF + it * (S // 2), 8) + row, n), :]

    def prep_gen(h, ph):
        for i0 in range(0, len(PITEMS), PORD):
            for d in range(DH):
                for (c, single) in PITEMS[i0:i0 + PORD]:
                    n = 8 if single else 16
                    col = ks_s[h, ks_off(c, single): ks_off(c, single) + n, :][:, d:d + 1]
                    base = kb_off(c, single) + d * n
                    bufs[ph][base: base + n, :] = pltpu.bitcast(jnp.broadcast_to(col, (n, 128)), U32)
                    yield

    nt_dims = (((1,), (1,)), ((), ()))
    stats = {}

    def upd(name, val):
        stats[name] = val if name not in stats else jnp.maximum(stats[name], val)

    def proj_k(i):
        xc = x_b[b, pl.ds(i * PR, PR), :]
        kc = jnp.dot(xc, w_b[b, :, D:2 * D], preferred_element_type=F32)
        upd("k", jnp.max(jnp.abs(kc).reshape(PR // 8, 8, D), axis=0))
        kp_s[i * (PR // 2):(i + 1) * (PR // 2), :] = pltpu.bitcast(kc.astype(BF), U32)

    def spread_k(i):
        for h in range(H):
            g, r = divmod(h, 8)
            it, ph = divmod(h, NPH)
            kr = kp_s[i * (PR // 2):(i + 1) * (PR // 2), g * 128:(g + 1) * 128]
            if r:
                kr = pltpu.roll(kr, 128 - DH * r, axis=1)
            ko = KOFF + it * (S // 2) + i * (PR // 2)
            kbuf(ph)[ko: ko + PR // 2, :] = kr
            if ph == 1 and i == 0:
                xo = XOFF + it * XC * (CH // 2)
                kbuf(0)[xo: xo + XC * (CH // 2), :] = kr[0: XC * (CH // 2)]
            for c in range(i * (PR // CH), (i + 1) * (PR // CH)):
                r0 = (c % (PR // CH)) * (CH // 2)
                ks_s[h, ks_off(c, False): ks_off(c, False) + 16, :] = (
                    pltpu.bitcast(kr[r0 + VB * 8: r0 + VB * 8 + 8], BF).astype(F32))
                if c in HALF:
                    kf = pltpu.bitcast(kr[r0 + HB * 8: r0 + HB * 8 + 8], BF).astype(F32)
                    fo = FOFF + (it * len(HALF) + HALF.index(c)) * 8
                    kbuf(ph)[fo: fo + 8, :] = pltpu.bitcast(kf[0:8], U32)
                    if ph == 1 and c < XC:
                        xf = XFO + (it * XC + c) * 8
                        kbuf(0)[xf: xf + 8, :] = pltpu.bitcast(kf[0:8], U32)
                    ks_s[h, ks_off(c, True): ks_off(c, True) + 8, :] = kf[8:16]

    def proj_q(i):
        xc = x_b[b, pl.ds(i * PR, PR), :]
        q = lax.dot_general(wt_s[0:D, :], xc, nt_dims, preferred_element_type=F32) * QSCALE
        upd("q", jnp.sum((q * q).reshape(H, DH, PR), axis=1))
        qt_s[:, pl.ds(i * PR, PR)] = pltpu.bitcast(q.astype(BF), U32)
        qf_s[:, :, pl.ds(i * PR, PR)] = q.reshape(H, DH, PR)

    def proj_v(i):
        xc = x_b[b, pl.ds(i * PR, PR), :]
        v = lax.dot_general(wt_s[D:2 * D, :], xc, nt_dims, preferred_element_type=F32)
        va = jnp.abs(v)
        va = jnp.maximum(jnp.maximum(va[:, 0:128], va[:, 128:256]),
                         jnp.maximum(va[:, 256:384], va[:, 384:512]))
        va = jnp.max(va.reshape(H, 2, 8, 128), axis=1)
        vm_s[...] = va if i == 0 else jnp.maximum(vm_s[...], va)
        vt_s[:, pl.ds(i * PR, PR)] = v

    wait_in(0); wait_in(3)
    proj_k(0)
    wait_in(4); wait_in(5)
    proj_k(1)
    spread_k(0)
    proj_k(2)
    wait_in(6); wait_in(1); wait_in(2)
    wt_s[0:D, :] = w_b[b, :, 0:D].T
    wt_s[D:2 * D, :] = w_b[b, :, 2 * D:3 * D].T
    proj_k(3)
    spread_k(1)
    for i in range(NXC):
        proj_q(i)
        if i < 2:
            spread_k(2 + i)
    for i in range(NXC):
        proj_v(i)

    km = jnp.max(stats["k"], axis=0, keepdims=True)
    km = km * km
    kseg = jnp.concatenate([km[:, g * 128:(g + 1) * 128] for g in range(4)], axis=0)
    for sh in (1, 2, 4, 8):
        kseg = kseg + pltpu.roll(kseg, sh, axis=1)
    safe_qk = jnp.max(stats["q"]) * jnp.max(kseg) <= SCORE_BOUND * SCORE_BOUND

    def vpu_col(z, ph, h, ct, c, single):
        z0 = pl.multiple_of(z, 8)
        ngrp = 1 if single else 2
        slabs = {}

        def kvreg(e):
            g = e // VG
            if g not in slabs:
                cnt = min(VG, DH * ngrp - g * VG)
                rows = pl.ds(z0 + kb_off(c, single) + g * VG * 8, cnt * 8)
                slabs[g] = pltpu.bitcast(bufs[ph][rows, :], F32)
            return slabs[g][(e % VG) * 8:(e % VG + 1) * 8]

        accs = [None] * ngrp
        for d in range(DH):
            qs = jnp.broadcast_to(qf_s[h + z, d:d + 1, ct * 128:(ct + 1) * 128], (8, 128))
            for g in range(ngrp):
                t = kvreg(d * ngrp + g) * qs
                accs[g] = t if accs[g] is None else accs[g] + t
        return accs[0] if single else jnp.concatenate(accs, axis=0)

    def pv_step(h, c, pb, oacc):
        r = pl.multiple_of(h * DH, DH)
        o = jnp.dot(vt_s[pl.ds(r, DH), c * CH:(c + 1) * CH].astype(pb.dtype), pb,
                    preferred_element_type=F32)
        return o if oacc is None else o + oacc

    def carried_p(x):
        return pltpu.bitcast(p_c[x * CH // 2:(x + 1) * CH // 2, :], BF)

    def finish(h, qb, lacc, oacc):
        ls_s[qb, pl.ds(h, 1), :] = jnp.sum(lacc, axis=0, keepdims=True)
        ot_s[h, :, qb * TQ:(qb + 1) * TQ] = oacc

    lead = [x[:3] for x in timeline(NQ * NC)[1][:RC]]

    def lead_gen(h, ph):
        lv = [jnp.zeros((8, 128), F32)] * 4
        for v, (t, col, single) in enumerate(lead):
            p = jnp.exp2(vpu_col(z_ref[v], ph, h, col, t, single))
            v_c[v * 16: v * 16 + p.shape[0], :] = p
            lv[col] = lv[col] + (p if single else p[0:8] + p[8:16])
            if v == RC - 1:
                lv_c[...] = jnp.concatenate(lv, axis=1)
            yield

    def block(it, phs):
        h0 = it * NPH + phs[0]
        hprev = (h0 + H - 1) % H
        nui = len(phs) * NQ
        T = nui * NC
        pads = [pl.multiple_of(PADOFF + 32 * x + z_ref[NSTEP + x], 8) for x in range(NPAD)]
        pbs = {t: {} for t in range(T)}
        laccs = {}; oaccs = {}
        nkt, vsteps = timeline(T)
        assert [x[:3] for x in vsteps[:RC]] == lead
        vnext = [RC]; ng = [0]; nk = [0]; pend = []; lhist = []
        pgen = [prep_gen(jnp.minimum(h0 + n + 2, H - 1), (ph + 2) % NPH) for n, ph in enumerate(phs)]
        phn = (phs[-1] + 1) % NPH
        lgen = lead_gen(jnp.minimum(h0 + len(phs), H - 1), phn)
        kph = nkt // len(phs)

        def e_blk(j, s, cols):
            p = jnp.exp2(s)
            ll = p[0:8]
            for x in range(1, s.shape[0] // 8):
                ll = ll + p[x * 8:(x + 1) * 8]
            la = laccs.setdefault(j, [None] * 4)
            for n, col in enumerate(cols):
                x = ll[:, n * 128:(n + 1) * 128] if len(cols) > 1 else ll
                la[col] = x if la[col] is None else la[col] + x
                lhist.append(la[col])
            return p, ll

        def emit_vpu(upto_k=None, upto_t=None):
            while vnext[0] < len(vsteps):
                v = vnext[0]
                t, col, single, dead = vsteps[v]
                if not ((upto_k is not None and dead <= upto_k)
                        or (upto_t is not None and min(x[0] for x in vsteps[v:]) <= upto_t)):
                    break
                j, c = divmod(t, NC)
                s = vpu_col(z_ref[v], phs[j // NQ], h0 + j // NQ, (j % NQ) * 4 + col, c, single)
                pp, ll = e_blk(j, s, [col])
                pbs[t].setdefault('s' if single else 'v', {})[col] = pp
                if v >= NG0:
                    pend.append(ll)
                vnext[0] += 1

        lv0 = lv_c[...]
        laccs[0] = [lv0[:, col * 128:(col + 1) * 128] for col in COLS]
        for v, (t, col, single) in enumerate(lead):
            pbs[t].setdefault('s' if single else 'v', {})[col] = v_c[v * 16: v * 16 + (8 if single else 16), :]

        def gates():
            n, kx = divmod(nk[0], kph)
            gb = kbuf(phs[n - 1]) if (n >= 1 and kx < XC * 7) else kbuf(phs[n])
            emit_vpu(upto_k=nk[0])
            if len(lhist) > LG + 4:
                pend.append(lhist[-LG - (nk[0] % 4)])
            while pend:
                gb[pl.ds(pads[ng[0] % NPAD], 8), :] = pltpu.bitcast(pend.pop(0), U32)
                ng[0] += 1
            for _ in range(share(kx, NPREP, kph - PE, max(PS, XC * 7) if n >= 1 else PS)):
                next(pgen[n])
            for _ in range(share(nk[0], RC, nkt, nkt - LS)):
                bufs[phn][pl.ds(pads[ng[0] % NPAD], 8), :] = pltpu.bitcast(lhist[-LG - (nk[0] % 4)], U32)
                next(lgen)
            nk[0] += 1

        def qk(t, sls):
            j, c = divmod(t, NC)
            h = h0 + j // NQ; ph = phs[j // NQ]; qb = j % NQ
            dup = (j == NQ and c < XC)
            hpos = [x for x, y in enumerate(sls) if y[0] == 'h']
            if hpos and hpos[0] > 0:
                qk(t, sls[:hpos[0]]); qk(t, sls[hpos[0]:])
                return
            if hpos:
                gates()
                if dup:
                    kf = kbuf(ph - 1)[pl.ds(pl.multiple_of(XFO + it * XC * 8, 8) + c * 8, 8), :]
                else:
                    fo = pl.multiple_of(FOFF + it * len(HALF) * 8, 8) + HALF.index(c) * 8
                    kf = kbuf(ph)[pl.ds(fo, 8), :]
                s = jnp.dot(pltpu.bitcast(kf, F32)[:, 0:DH], qf_s[h, :, qb * TQ:(qb + 1) * TQ],
                            preferred_element_type=F32)
                pbs[t]['h'] = e_blk(j, s, COLS)[0]
                sls = sls[1:]
            if not sls:
                return
            ks = []
            for _, bb in sls:
                gates()
                row = c * CH // 2 + bb * 8
                if dup:
                    ks.append(kbuf(ph - 1)[pl.ds(pl.multiple_of(XOFF + it * XC * (CH // 2), 8) + row, 8), :])
                else:
                    ks.append(ldk(it, ph, row))
            kk = pltpu.bitcast(jnp.concatenate(ks, axis=0) if len(ks) > 1 else ks[0], BF)[:, 0:DH]
            w = pltpu.bitcast(qt_s[pl.ds(pl.multiple_of(h * 8, 8), 8), qb * TQ:(qb + 1) * TQ], BF)
            s = jnp.dot(kk, w, preferred_element_type=F32)
            for x, (_, bb) in enumerate(sls):
                pbs[t][bb] = e_blk(j, s[x * 16:(x + 1) * 16], COLS)[0]

        def gather_p(tb):
            emit_vpu(upto_t=tb)
            pp = pbs.pop(tb)
            pv = jnp.concatenate([pp['v'][col] for col in COLS], axis=1)
            rows = []
            for bb in range(8):
                if bb == VB:
                    rows.append(pv)
                elif bb in pp:
                    rows.append(pp[bb])
                else:
                    rows += [pp['h'], jnp.concatenate([pp['s'][col] for col in COLS], axis=1)]
            return jnp.concatenate(rows, axis=0)

        def do_pv(tb):
            if tb < 0:
                if tb == -SK:
                    oaccs[-1] = o_c[...]
                oaccs[-1] = pv_step(hprev, NC + tb, carried_p(tb + SK), oaccs[-1])
                if tb == -1:
                    finish(hprev, NQ - 1, l_c[...], oaccs[-1])
                return
            j, c = divmod(tb, NC)
            oaccs[j] = pv_step(h0 + j // NQ, c, gather_p(tb), oaccs.get(j))
            if c == NC - 1:
                finish(h0 + j // NQ, j % NQ, jnp.concatenate(laccs[j], axis=1), oaccs[j])

        for t in range(T):
            sls = slots(t % NC)
            cut = SPL if t >= SK else CP[t]
            qk(t, sls[:cut])
            do_pv(t - SK)
            qk(t, sls[cut:])
        for x in range(SK):
            p_c[x * CH // 2:(x + 1) * CH // 2, :] = pltpu.bitcast(gather_p(T - SK + x).astype(BF), U32)
        l_c[...] = jnp.concatenate(laccs[nui - 1], axis=1)
        o_c[...] = oaccs[nui - 1]

    for hh in range(2):
        for _ in prep_gen(hh, hh):
            pass
    p_c[...] = jnp.zeros(p_c.shape, U32)
    l_c[...] = jnp.ones(l_c.shape, F32)
    o_c[...] = jnp.zeros(o_c.shape, F32)
    for _ in lead_gen(0, 0):
        pass

    @pl.when(safe_qk)
    def _():
        def body(i, c):
            block(i, BLOCKS[0])
            pl.when(i * NPH + BLOCKS[1][0] < H)(functools.partial(block, i, BLOCKS[1]))
            return c
        lax.fori_loop(0, NIT, body, 0)

    o = o_c[...]
    for x in range(SK):
        o = pv_step(H - 1, NC - SK + x, carried_p(x), o)
    finish(H - 1, NQ - 1, l_c[...], o)
    vh = jnp.max(jnp.max(vm_s[...], axis=1), axis=1, keepdims=True)
    safe = safe_qk & (jnp.min(vh) >= V_LO) & (jnp.max(vh) <= V_HI)

    def slow_body(it, carry):
        sc = 256
        for ph in range(NPH):
            h = it * NPH + ph

            def unit(qb, c2):
                c0 = pl.multiple_of(qb * TQ, TQ)
                w = pltpu.bitcast(qt_s[pl.ds(pl.multiple_of(h * 8, 8), 8), pl.ds(c0, TQ)], BF)

                def p1(c, m):
                    ro = pl.multiple_of(c * (sc // 2), 8)
                    kk = pltpu.bitcast(ldk(it, ph, ro, sc // 2), BF)[:, 0:DH]
                    s = jnp.dot(kk, w, preferred_element_type=F32)
                    s_s[pl.ds(pl.multiple_of(c * sc, sc), sc), :] = s
                    return jnp.maximum(m, jnp.max(s, axis=0, keepdims=True))
                m = lax.fori_loop(0, S // sc, p1, jnp.full((1, TQ), -jnp.inf, F32))

                def p2(c, lo):
                    l, o = lo
                    co = pl.multiple_of(c * sc, sc)
                    p = jnp.exp2(s_s[pl.ds(co, sc), :] - m)
                    vt = vt_s[pl.ds(pl.multiple_of(h * DH, DH), DH), pl.ds(co, sc)]
                    return (l + jnp.sum(p.reshape(sc // 8, 8, TQ), axis=0),
                            o + jnp.dot(vt, p, preferred_element_type=F32))
                l, o = lax.fori_loop(0, S // sc, p2,
                                     (jnp.zeros((8, TQ), F32), jnp.zeros((DH, TQ), F32)))
                ot_s[h, :, pl.ds(c0, TQ)] = o
                ls_s[qb, pl.ds(h, 1), :] = jnp.sum(l, axis=0, keepdims=True)
                return c2
            lax.fori_loop(0, jnp.where(h < H, NQ, 0), unit, 0)
        return carry

    @pl.when(jnp.logical_not(safe))
    def _():
        lax.fori_loop(0, NIT, slow_body, 0)

    wait_in(3 + NXC)

    def out_copy(bb, n):
        r0, nr = OCH[n]
        return pltpu.make_async_copy(
            ob.at[r0:r0 + nr, :],
            out_hbm.at[0, r0:r0 + nr, pl.ds(pl.multiple_of(bb * D, D), D)], osem.at[n])

    @pl.when(b == 1)
    def _():
        for n in range(len(OCH)):
            out_copy(0, n).wait()

    for n, (r0, nr) in enumerate(OCH):
        qb, c0 = divmod(r0, TQ)
        inv = 1.0 / ls_s[qb, :, c0:c0 + nr]
        oc = (ot_s[:, :, r0:r0 + nr] * inv.reshape(H, 1, nr)).reshape(D, nr).T.astype(BF)
        r = jnp.dot(oc, wo_b[b], preferred_element_type=F32)
        ob[r0:r0 + nr, :] = r.astype(BF)
        out_copy(b, n).start()

    @pl.when(b == 1)
    def _():
        for n in range(len(OCH)):
            out_copy(1, n).wait()


@jax.jit
def pallas_concat_heads__softmax_full_mha__softmax_full_mha__prompt_kernel(
    A_x: jax.Array,
    A_wqkv: jax.Array,
    A_wo: jax.Array,
    B_x: jax.Array,
    B_wqkv: jax.Array,
    B_wo: jax.Array,
):
    any_spec = pl.BlockSpec(memory_space=pl.ANY)
    vm = pltpu.VMEM
    return pl.pallas_call(
        _kernel,
        out_shape=jax.ShapeDtypeStruct((1, S, 2 * D), BF),
        grid=(2,),
        in_specs=[any_spec] * 6,
        out_specs=any_spec,
        scratch_shapes=[
            vm((2, S, D), BF), vm((2, D, 3 * D), BF), vm((2, D, D), BF),
            vm((2 * D, D), BF),
            vm((S // 2, D), U32), vm((D // 2, S), U32), vm((D, S), F32),
            vm((H, DH, S), F32), vm((H, NGT * 8, 128), F32),
            vm((H, DH, S), F32), vm((NQ, H, TQ), F32), vm((S, D), BF),
            vm((TOTR, 128), U32), vm((TOTR, 128), U32), vm((TOTR, 128), U32),
            vm((S, TQ), F32),
            vm((SK * CH // 2, TQ), U32), vm((8, TQ), F32), vm((DH, TQ), F32),
            vm((RC * 16, 128), F32), vm((8, TQ), F32), vm((H, 8, 128), F32),
            pltpu.SMEM((NZ,), jnp.int32),
            pltpu.SemaphoreType.DMA((2, NXC + 4)), pltpu.SemaphoreType.DMA((len(OCH),)),
        ],
        compiler_params=pltpu.CompilerParams(
            vmem_limit_bytes=100 * 1024 * 1024, dimension_semantics=("arbitrary",)),
    )(A_x, A_wqkv, A_wo, B_x, B_wqkv, B_wo)
```

```python
import functools
import math

import jax
import jax.numpy as jnp
from jax import lax
from jax.experimental import pallas as pl
from jax.experimental.pallas import tpu as pltpu

S = 2048; D = 512; H = 32; DH = 16
TQ = 512
CH = 128
PR = 512
NQ = S // TQ; NC = S // CH; NXC = S // PR
F32 = jnp.float32; BF = jnp.bfloat16; U32 = jnp.uint32

QSCALE = (DH ** -0.5) * math.log2(math.e)
SCORE_BOUND = 64.0
V_LO = 2.0 ** -30
V_HI = 2.0 ** 50

SK = 2
SPL = 2
LG = 49
PS = 16; PE = 12
VG = 3; PORD = 4
NG0 = 0
DLT = 24; SDL = 80; SO = (80, 16)
RC = 4; LS = 8
CP = (3, 6)
XC = 4
HALF = [c for c in range(NC) if c % 2]
VB = 0
MXB = [x for x in range(7, -1, -1) if x != VB]
HB = MXB[SPL]
NGT = 2 * NC + len(HALF)
KBR = NGT * DH * 8
PITEMS = [(c, False) for c in range(NC)]
for _n, _c in enumerate(HALF):
    PITEMS.insert(_c + _n + 1, (_c, True))
NPREP = len(PITEMS) * DH
NPH = 3
BLOCKS = ((0, 1), (2,))
NIT = -(-H // NPH)
KOFF = KBR
FOFF = KOFF + NIT * (S // 2)
XOFF = FOFF + NIT * len(HALF) * 8
XFO = XOFF + NIT * XC * (CH // 2)
PADOFF = XFO + NIT * XC * 8
NPAD = 4
TOTR = PADOFF + 32 * NPAD
assert all(x % 32 == 0 for x in (KOFF, FOFF, XOFF, XFO, PADOFF, TOTR))
NSTEP = 2 * NQ * 4 * (NC + len(HALF))
NZ = NSTEP + NPAD
OCH = ((0, 128), (128, 384), (512, 512), (1024, 512), (1536, 384), (1920, 128))
COLS = (0, 1, 2, 3)


def kb_off(c, single):
    return (2 * NC + HALF.index(c)) * DH * 8 if single else c * 2 * DH * 8


def ks_off(c, single):
    return (2 * NC + HALF.index(c)) * 8 if single else c * 16


def slots(c):
    return [('h', c) if (c in HALF and x == HB) else ('b', x) for x in MXB]


def timeline(T):
    ktime = []; pvtime = {}; now = 0
    for t in range(T):
        for n, sl in enumerate(slots(t % NC)):
            if n == SPL:
                pvtime[t - SK] = now; now += 16
            ktime.append(now); now += 8 if sl[0] == 'h' else 16
    for t in range(T - SK, T):
        pvtime[t] = now + 128 * (t - T + SK) + 32
    vs = [(pvtime[t] - DLT - (3 - col) * 32, t, col, False) for t in range(T) for col in COLS]
    free = sorted(pvtime[t] - o for t in range(-SK, T) for o in SO)
    for t in range(T - 1, -1, -1):
        if t % NC in HALF:
            for col in reversed(COLS):
                tm = [x for x in free if x <= pvtime[t] - SDL][-1]
                free.remove(tm)
                vs.append((tm, t, col, True))
    vs.sort()
    return len(ktime), [(t, col, single, sum(1 for k in ktime if k < tm)) for (tm, t, col, single) in vs]


def share(x, tot, n, skip):
    if x < skip or x >= n:
        return 0
    return ((x - skip + 1) * tot) // (n - skip) - ((x - skip) * tot) // (n - skip)


def _kernel(ax, aw, ao, bx, bw, bo, out_hbm,
            x_b, w_b, wo_b, wt_s, kp_s, qt_s, vt_s, qf_s, ks_s, ot_s, ls_s, ob, bufa, bufb, bufc,
            s_s, p_c, l_c, o_c, v_c, lv_c, vm_s, z_ref, isem, osem):
    b = pl.program_id(0)
    bufs = (bufa, bufb, bufc)

    def kbuf(ph):
        return bufs[(ph + 2) % NPH]

    def in_refs(src3, slot, j):
        x, w, wo = src3
        if j < 3:
            c0 = (D, 0, 2 * D)[j]
            return w.at[:, c0:c0 + D], w_b.at[slot, :, c0:c0 + D]
        if j < 3 + NXC:
            i = j - 3
            return x.at[0, i * PR:(i + 1) * PR, :], x_b.at[slot, i * PR:(i + 1) * PR, :]
        return wo, wo_b.at[slot]

    @pl.when(b == 0)
    def _():
        for slot, src3 in enumerate(((ax, aw, ao), (bx, bw, bo))):
            for j in (0, 3, 4, 5, 6, 1, 2, 7):
                src, dst = in_refs(src3, slot, j)
                pltpu.make_async_copy(src, dst, isem.at[slot, j]).start()
        for j in range(NZ):
            z_ref[j] = 0

    def wait_in(j):
        dst = in_refs((ax, aw, ao), b, j)[1]
        pltpu.make_async_copy(dst, dst, isem.at[b, j]).wait()

    def ldk(it, ph, row, n=8):
        return kbuf(ph)[pl.ds(pl.multiple_of(KOFF + it * (S // 2), 8) + row, n), :]

    def prep_gen(h, ph):
        for i0 in range(0, len(PITEMS), PORD):
            for d in range(DH):
                for (c, single) in PITEMS[i0:i0 + PORD]:
                    n = 8 if single else 16
                    col = ks_s[h, ks_off(c, single): ks_off(c, single) + n, :][:, d:d + 1]
                    base = kb_off(c, single) + d * n
                    bufs[ph][base: base + n, :] = pltpu.bitcast(jnp.broadcast_to(col, (n, 128)), U32)
                    yield

    nt_dims = (((1,), (1,)), ((), ()))
    stats = {}

    def upd(name, val):
        stats[name] = val if name not in stats else jnp.maximum(stats[name], val)

    def proj_k(i):
        xc = x_b[b, pl.ds(i * PR, PR), :]
        kc = jnp.dot(xc, w_b[b, :, D:2 * D], preferred_element_type=F32)
        upd("k", jnp.max(jnp.abs(kc).reshape(PR // 8, 8, D), axis=0))
        kp_s[i * (PR // 2):(i + 1) * (PR // 2), :] = pltpu.bitcast(kc.astype(BF), U32)

    def spread_k(i):
        for h in range(H):
            g, r = divmod(h, 8)
            it, ph = divmod(h, NPH)
            kr = kp_s[i * (PR // 2):(i + 1) * (PR // 2), g * 128:(g + 1) * 128]
            if r:
                kr = pltpu.roll(kr, 128 - DH * r, axis=1)
            ko = KOFF + it * (S // 2) + i * (PR // 2)
            kbuf(ph)[ko: ko + PR // 2, :] = kr
            if ph == 1 and i == 0:
                xo = XOFF + it * XC * (CH // 2)
                kbuf(0)[xo: xo + XC * (CH // 2), :] = kr[0: XC * (CH // 2)]
            for c in range(i * (PR // CH), (i + 1) * (PR // CH)):
                r0 = (c % (PR // CH)) * (CH // 2)
                ks_s[h, ks_off(c, False): ks_off(c, False) + 16, :] = (
                    pltpu.bitcast(kr[r0 + VB * 8: r0 + VB * 8 + 8], BF).astype(F32))
                if c in HALF:
                    kf = pltpu.bitcast(kr[r0 + HB * 8: r0 + HB * 8 + 8], BF).astype(F32)
                    fo = FOFF + (it * len(HALF) + HALF.index(c)) * 8
                    kbuf(ph)[fo: fo + 8, :] = pltpu.bitcast(kf[0:8], U32)
                    if ph == 1 and c < XC:
                        xf = XFO + (it * XC + c) * 8
                        kbuf(0)[xf: xf + 8, :] = pltpu.bitcast(kf[0:8], U32)
                    ks_s[h, ks_off(c, True): ks_off(c, True) + 8, :] = kf[8:16]

    def proj_q(i):
        xc = x_b[b, pl.ds(i * PR, PR), :]
        q = lax.dot_general(wt_s[0:D, :], xc, nt_dims, preferred_element_type=F32) * QSCALE
        upd("q", jnp.sum((q * q).reshape(H, DH, PR), axis=1))
        qt_s[:, pl.ds(i * PR, PR)] = pltpu.bitcast(q.astype(BF), U32)
        qf_s[:, :, pl.ds(i * PR, PR)] = q.reshape(H, DH, PR)

    def proj_v(i):
        xc = x_b[b, pl.ds(i * PR, PR), :]
        v = lax.dot_general(wt_s[D:2 * D, :], xc, nt_dims, preferred_element_type=F32)
        va = jnp.abs(v)
        va = jnp.maximum(jnp.maximum(va[:, 0:128], va[:, 128:256]),
                         jnp.maximum(va[:, 256:384], va[:, 384:512]))
        va = jnp.max(va.reshape(H, 2, 8, 128), axis=1)
        vm_s[...] = va if i == 0 else jnp.maximum(vm_s[...], va)
        vt_s[:, pl.ds(i * PR, PR)] = v

    wait_in(0); wait_in(3)
    proj_k(0)
    wait_in(4); wait_in(5)
    proj_k(1)
    spread_k(0)
    proj_k(2)
    wait_in(6); wait_in(1); wait_in(2)
    wt_s[0:D, :] = w_b[b, :, 0:D].T
    wt_s[D:2 * D, :] = w_b[b, :, 2 * D:3 * D].T
    proj_k(3)
    spread_k(1)
    for i in range(NXC):
        proj_q(i)
        if i < 2:
            spread_k(2 + i)
    for i in range(NXC):
        proj_v(i)

    km = jnp.max(stats["k"], axis=0, keepdims=True)
    km = km * km
    kseg = jnp.concatenate([km[:, g * 128:(g + 1) * 128] for g in range(4)], axis=0)
    for sh in (1, 2, 4, 8):
        kseg = kseg + pltpu.roll(kseg, sh, axis=1)
    safe_qk = jnp.max(stats["q"]) * jnp.max(kseg) <= SCORE_BOUND * SCORE_BOUND

    def vpu_col(z, ph, h, ct, c, single):
        z0 = pl.multiple_of(z, 8)
        ngrp = 1 if single else 2
        slabs = {}

        def kvreg(e):
            g = e // VG
            if g not in slabs:
                cnt = min(VG, DH * ngrp - g * VG)
                rows = pl.ds(z0 + kb_off(c, single) + g * VG * 8, cnt * 8)
                slabs[g] = pltpu.bitcast(bufs[ph][rows, :], F32)
            return slabs[g][(e % VG) * 8:(e % VG + 1) * 8]

        accs = [None] * ngrp
        for d in range(DH):
            qs = jnp.broadcast_to(qf_s[h + z, d:d + 1, ct * 128:(ct + 1) * 128], (8, 128))
            for g in range(ngrp):
                t = kvreg(d * ngrp + g) * qs
                accs[g] = t if accs[g] is None else accs[g] + t
        return accs[0] if single else jnp.concatenate(accs, axis=0)

    def pv_step(h, c, pb, oacc):
        r = pl.multiple_of(h * DH, DH)
        o = jnp.dot(vt_s[pl.ds(r, DH), c * CH:(c + 1) * CH].astype(pb.dtype), pb,
                    preferred_element_type=F32)
        return o if oacc is None else o + oacc

    def carried_p(x):
        return pltpu.bitcast(p_c[x * CH // 2:(x + 1) * CH // 2, :], BF)

    def finish(h, qb, lacc, oacc):
        ls_s[qb, pl.ds(h, 1), :] = jnp.sum(lacc, axis=0, keepdims=True)
        ot_s[h, :, qb * TQ:(qb + 1) * TQ] = oacc

    lead = [x[:3] for x in timeline(NQ * NC)[1][:RC]]

    def lead_gen(h, ph):
        lv = [jnp.zeros((8, 128), F32)] * 4
        for v, (t, col, single) in enumerate(lead):
            p = jnp.exp2(vpu_col(z_ref[v], ph, h, col, t, single))
            v_c[v * 16: v * 16 + p.shape[0], :] = p
            lv[col] = lv[col] + (p if single else p[0:8] + p[8:16])
            if v == RC - 1:
                lv_c[...] = jnp.concatenate(lv, axis=1)
            yield

    def block(it, phs):
        h0 = it * NPH + phs[0]
        hprev = (h0 + H - 1) % H
        nui = len(phs) * NQ
        T = nui * NC
        pads = [pl.multiple_of(PADOFF + 32 * x + z_ref[NSTEP + x], 8) for x in range(NPAD)]
        pbs = {t: {} for t in range(T)}
        laccs = {}; oaccs = {}
        nkt, vsteps = timeline(T)
        assert [x[:3] for x in vsteps[:RC]] == lead
        vnext = [RC]; ng = [0]; nk = [0]; pend = []; lhist = []
        pgen = [prep_gen(jnp.minimum(h0 + n + 2, H - 1), (ph + 2) % NPH) for n, ph in enumerate(phs)]
        phn = (phs[-1] + 1) % NPH
        lgen = lead_gen(jnp.minimum(h0 + len(phs), H - 1), phn)
        kph = nkt // len(phs)

        def e_blk(j, s, cols):
            p = jnp.exp2(s)
            ll = p[0:8]
            for x in range(1, s.shape[0] // 8):
                ll = ll + p[x * 8:(x + 1) * 8]
            la = laccs.setdefault(j, [None] * 4)
            for n, col in enumerate(cols):
                x = ll[:, n * 128:(n + 1) * 128] if len(cols) > 1 else ll
                la[col] = x if la[col] is None else la[col] + x
                lhist.append(la[col])
            return p, ll

        def emit_vpu(upto_k=None, upto_t=None):
            while vnext[0] < len(vsteps):
                v = vnext[0]
                t, col, single, dead = vsteps[v]
                if not ((upto_k is not None and dead <= upto_k)
                        or (upto_t is not None and min(x[0] for x in vsteps[v:]) <= upto_t)):
                    break
                j, c = divmod(t, NC)
                s = vpu_col(z_ref[v], phs[j // NQ], h0 + j // NQ, (j % NQ) * 4 + col, c, single)
                pp, ll = e_blk(j, s, [col])
                pbs[t].setdefault('s' if single else 'v', {})[col] = pp
                if v >= NG0:
                    pend.append(ll)
                vnext[0] += 1

        lv0 = lv_c[...]
        laccs[0] = [lv0[:, col * 128:(col + 1) * 128] for col in COLS]
        for v, (t, col, single) in enumerate(lead):
            pbs[t].setdefault('s' if single else 'v', {})[col] = v_c[v * 16: v * 16 + (8 if single else 16), :]

        def gates():
            n, kx = divmod(nk[0], kph)
            gb = kbuf(phs[n - 1]) if (n >= 1 and kx < XC * 7) else kbuf(phs[n])
            emit_vpu(upto_k=nk[0])
            if len(lhist) > LG + 4:
                pend.append(lhist[-LG])
            while pend:
                gb[pl.ds(pads[ng[0] % NPAD], 8), :] = pltpu.bitcast(pend.pop(0), U32)
                ng[0] += 1
            for _ in range(share(kx, NPREP, kph - PE, max(PS, XC * 7) if n >= 1 else PS)):
                next(pgen[n])
            for _ in range(share(nk[0], RC, nkt, nkt - LS)):
                bufs[phn][pl.ds(pads[ng[0] % NPAD], 8), :] = pltpu.bitcast(lhist[-LG - (nk[0] % 4)], U32)
                next(lgen)
            nk[0] += 1

        def qk(t, sls):
            j, c = divmod(t, NC)
            h = h0 + j // NQ; ph = phs[j // NQ]; qb = j % NQ
            dup = (j == NQ and c < XC)
            hpos = [x for x, y in enumerate(sls) if y[0] == 'h']
            if hpos and hpos[0] > 0:
                qk(t, sls[:hpos[0]]); qk(t, sls[hpos[0]:])
                return
            if hpos:
                gates()
                if dup:
                    kf = kbuf(ph - 1)[pl.ds(pl.multiple_of(XFO + it * XC * 8, 8) + c * 8, 8), :]
                else:
                    fo = pl.multiple_of(FOFF + it * len(HALF) * 8, 8) + HALF.index(c) * 8
                    kf = kbuf(ph)[pl.ds(fo, 8), :]
                s = jnp.dot(pltpu.bitcast(kf, F32)[:, 0:DH], qf_s[h, :, qb * TQ:(qb + 1) * TQ],
                            preferred_element_type=F32)
                pbs[t]['h'] = e_blk(j, s, COLS)[0]
                sls = sls[1:]
            if not sls:
                return
            ks = []
            for _, bb in sls:
                gates()
                row = c * CH // 2 + bb * 8
                if dup:
                    ks.append(kbuf(ph - 1)[pl.ds(pl.multiple_of(XOFF + it * XC * (CH // 2), 8) + row, 8), :])
                else:
                    ks.append(ldk(it, ph, row))
            kk = pltpu.bitcast(jnp.concatenate(ks, axis=0) if len(ks) > 1 else ks[0], BF)[:, 0:DH]
            w = pltpu.bitcast(qt_s[pl.ds(pl.multiple_of(h * 8, 8), 8), qb * TQ:(qb + 1) * TQ], BF)
            s = jnp.dot(kk, w, preferred_element_type=F32)
            for x, (_, bb) in enumerate(sls):
                pbs[t][bb] = e_blk(j, s[x * 16:(x + 1) * 16], COLS)[0]

        def gather_p(tb):
            emit_vpu(upto_t=tb)
            pp = pbs.pop(tb)
            pv = jnp.concatenate([pp['v'][col] for col in COLS], axis=1)
            rows = []
            for bb in range(8):
                if bb == VB:
                    rows.append(pv)
                elif bb in pp:
                    rows.append(pp[bb])
                else:
                    rows += [pp['h'], jnp.concatenate([pp['s'][col] for col in COLS], axis=1)]
            return jnp.concatenate(rows, axis=0)

        def do_pv(tb):
            if tb < 0:
                if tb == -SK:
                    oaccs[-1] = o_c[...]
                oaccs[-1] = pv_step(hprev, NC + tb, carried_p(tb + SK), oaccs[-1])
                if tb == -1:
                    finish(hprev, NQ - 1, l_c[...], oaccs[-1])
                return
            j, c = divmod(tb, NC)
            oaccs[j] = pv_step(h0 + j // NQ, c, gather_p(tb), oaccs.get(j))
            if c == NC - 1:
                finish(h0 + j // NQ, j % NQ, jnp.concatenate(laccs[j], axis=1), oaccs[j])

        for t in range(T):
            sls = slots(t % NC)
            if t == 0:
                cuts = [(CP[x], x - SK) for x in range(SK)]
            else:
                cuts = [(SPL, t - SK)] if t >= SK else []
            pos = 0
            for cut, tb in cuts:
                qk(t, sls[pos:cut])
                do_pv(tb)
                pos = cut
            qk(t, sls[pos:])
        for x in range(SK):
            p_c[x * CH // 2:(x + 1) * CH // 2, :] = pltpu.bitcast(gather_p(T - SK + x).astype(BF), U32)
        l_c[...] = jnp.concatenate(laccs[nui - 1], axis=1)
        o_c[...] = oaccs[nui - 1]

    for hh in range(2):
        for _ in prep_gen(hh, hh):
            pass
    p_c[...] = jnp.zeros(p_c.shape, U32)
    l_c[...] = jnp.ones(l_c.shape, F32)
    o_c[...] = jnp.zeros(o_c.shape, F32)
    for _ in lead_gen(0, 0):
        pass

    @pl.when(safe_qk)
    def _():
        def body(i, c):
            block(i, BLOCKS[0])
            pl.when(i * NPH + BLOCKS[1][0] < H)(functools.partial(block, i, BLOCKS[1]))
            return c
        lax.fori_loop(0, NIT, body, 0)

    o = o_c[...]
    for x in range(SK):
        o = pv_step(H - 1, NC - SK + x, carried_p(x), o)
    finish(H - 1, NQ - 1, l_c[...], o)
    vh = jnp.max(jnp.max(vm_s[...], axis=1), axis=1, keepdims=True)
    safe = safe_qk & (jnp.min(vh) >= V_LO) & (jnp.max(vh) <= V_HI)

    def slow_body(it, carry):
        sc = 256
        for ph in range(NPH):
            h = it * NPH + ph

            def unit(qb, c2):
                c0 = pl.multiple_of(qb * TQ, TQ)
                w = pltpu.bitcast(qt_s[pl.ds(pl.multiple_of(h * 8, 8), 8), pl.ds(c0, TQ)], BF)

                def p1(c, m):
                    ro = pl.multiple_of(c * (sc // 2), 8)
                    kk = pltpu.bitcast(ldk(it, ph, ro, sc // 2), BF)[:, 0:DH]
                    s = jnp.dot(kk, w, preferred_element_type=F32)
                    s_s[pl.ds(pl.multiple_of(c * sc, sc), sc), :] = s
                    return jnp.maximum(m, jnp.max(s, axis=0, keepdims=True))
                m = lax.fori_loop(0, S // sc, p1, jnp.full((1, TQ), -jnp.inf, F32))

                def p2(c, lo):
                    l, o = lo
                    co = pl.multiple_of(c * sc, sc)
                    p = jnp.exp2(s_s[pl.ds(co, sc), :] - m)
                    vt = vt_s[pl.ds(pl.multiple_of(h * DH, DH), DH), pl.ds(co, sc)]
                    return (l + jnp.sum(p.reshape(sc // 8, 8, TQ), axis=0),
                            o + jnp.dot(vt, p, preferred_element_type=F32))
                l, o = lax.fori_loop(0, S // sc, p2,
                                     (jnp.zeros((8, TQ), F32), jnp.zeros((DH, TQ), F32)))
                ot_s[h, :, pl.ds(c0, TQ)] = o
                ls_s[qb, pl.ds(h, 1), :] = jnp.sum(l, axis=0, keepdims=True)
                return c2
            lax.fori_loop(0, jnp.where(h < H, NQ, 0), unit, 0)
        return carry

    @pl.when(jnp.logical_not(safe))
    def _():
        lax.fori_loop(0, NIT, slow_body, 0)

    wait_in(3 + NXC)

    def out_copy(bb, n):
        r0, nr = OCH[n]
        return pltpu.make_async_copy(
            ob.at[r0:r0 + nr, :],
            out_hbm.at[0, r0:r0 + nr, pl.ds(pl.multiple_of(bb * D, D), D)], osem.at[n])

    @pl.when(b == 1)
    def _():
        for n in range(len(OCH)):
            out_copy(0, n).wait()

    for n, (r0, nr) in enumerate(OCH):
        qb, c0 = divmod(r0, TQ)
        inv = 1.0 / ls_s[qb, :, c0:c0 + nr]
        oc = (ot_s[:, :, r0:r0 + nr] * inv.reshape(H, 1, nr)).reshape(D, nr).T.astype(BF)
        r = jnp.dot(oc, wo_b[b], preferred_element_type=F32)
        ob[r0:r0 + nr, :] = r.astype(BF)
        out_copy(b, n).start()

    @pl.when(b == 1)
    def _():
        for n in range(len(OCH)):
            out_copy(1, n).wait()


@jax.jit
def pallas_concat_heads__softmax_full_mha__softmax_full_mha__prompt_kernel(
    A_x: jax.Array,
    A_wqkv: jax.Array,
    A_wo: jax.Array,
    B_x: jax.Array,
    B_wqkv: jax.Array,
    B_wo: jax.Array,
):
    any_spec = pl.BlockSpec(memory_space=pl.ANY)
    vm = pltpu.VMEM
    return pl.pallas_call(
        _kernel,
        out_shape=jax.ShapeDtypeStruct((1, S, 2 * D), BF),
        grid=(2,),
        in_specs=[any_spec] * 6,
        out_specs=any_spec,
        scratch_shapes=[
            vm((2, S, D), BF), vm((2, D, 3 * D), BF), vm((2, D, D), BF),
            vm((2 * D, D), BF),
            vm((S // 2, D), U32), vm((D // 2, S), U32), vm((D, S), F32),
            vm((H, DH, S), F32), vm((H, NGT * 8, 128), F32),
            vm((H, DH, S), F32), vm((NQ, H, TQ), F32), vm((S, D), BF),
            vm((TOTR, 128), U32), vm((TOTR, 128), U32), vm((TOTR, 128), U32),
            vm((S, TQ), F32),
            vm((SK * CH // 2, TQ), U32), vm((8, TQ), F32), vm((DH, TQ), F32),
            vm((RC * 16, 128), F32), vm((8, TQ), F32), vm((H, 8, 128), F32),
            pltpu.SMEM((NZ,), jnp.int32),
            pltpu.SemaphoreType.DMA((2, NXC + 4)), pltpu.SemaphoreType.DMA((len(OCH),)),
        ],
        compiler_params=pltpu.CompilerParams(
            vmem_limit_bytes=100 * 1024 * 1024, dimension_semantics=("arbitrary",)),
    )(A_x, A_wqkv, A_wo, B_x, B_wqkv, B_wo)
```

```python
import functools
import math

import jax
import jax.numpy as jnp
from jax import lax
from jax.experimental import pallas as pl
from jax.experimental.pallas import tpu as pltpu

S = 2048; D = 512; H = 32; DH = 16
TQ = 512
CH = 128
PR = 512
NQ = S // TQ; NC = S // CH; NXC = S // PR
F32 = jnp.float32; BF = jnp.bfloat16; U32 = jnp.uint32

QSCALE = (DH ** -0.5) * math.log2(math.e)
SCORE_BOUND = 64.0
V_LO = 2.0 ** -30
V_HI = 2.0 ** 50

SK = 2
SPL = 2
LG = 49
PS = 16; PE = 12
VG = 3; PORD = 4
NG0 = 0
DLT = 24; SDL = 80; SO = (80, 16)
RC = 4; LS = 8
CP = (3, 6)
XC = 4
HALF = [c for c in range(NC) if c % 2]
XCH = 6
HM = sorted(HALF + [XCH])
HST = -(-len(HM) // 4) * 4
XW = 2
VB = 0
MXB = [x for x in range(7, -1, -1) if x != VB]
HB = MXB[SPL]
NGT = 2 * NC + len(HALF)
KBR = NGT * DH * 8
PITEMS = [(c, False) for c in range(NC)]
for _n, _c in enumerate(HALF):
    PITEMS.insert(_c + _n + 1, (_c, True))
NPREP = len(PITEMS) * DH
NPH = 3
BLOCKS = ((0, 1), (2,))
NIT = -(-H // NPH)
KOFF = KBR
FOFF = KOFF + NIT * (S // 2)
XOFF = FOFF + NIT * HST * 8
XFO = XOFF + NIT * XC * (CH // 2)
PADOFF = XFO + NIT * XC * 8
NPAD = 4
TOTR = PADOFF + 32 * NPAD
assert all(x % 32 == 0 for x in (KOFF, FOFF, XOFF, XFO, PADOFF, TOTR))
NSTEP = 2 * NQ * 4 * (NC + len(HALF))
NZ = NSTEP + NPAD
OCH = ((0, 128), (128, 384), (512, 512), (1024, 512), (1536, 384), (1920, 128))
COLS = (0, 1, 2, 3)


def kb_off(c, single):
    return (2 * NC + HALF.index(c)) * DH * 8 if single else c * 2 * DH * 8


def ks_off(c, single):
    return (2 * NC + HALF.index(c)) * 8 if single else c * 16


def slots(c):
    return [('h', c) if (c in HM and x == HB) else ('b', x) for x in MXB]


def timeline(T):
    ktime = []; pvtime = {}; now = 0
    for t in range(T):
        for n, sl in enumerate(slots(t % NC)):
            if n == SPL:
                pvtime[t - SK] = now; now += 16
            ktime.append(now); now += 8 if sl[0] == 'h' else 16
    for t in range(T - SK, T):
        pvtime[t] = now + 128 * (t - T + SK) + 32
    vs = [(pvtime[t] - DLT - (3 - col) * 32, t, col, False) for t in range(T) for col in COLS]
    free = sorted(pvtime[t] - o for t in range(-SK, T) for o in SO)
    for t in range(T - 1, -1, -1):
        if t % NC in HALF:
            for col in reversed(COLS):
                tm = [x for x in free if x <= pvtime[t] - SDL][-1]
                free.remove(tm)
                vs.append((tm, t, col, True))
    vs.sort()
    return len(ktime), [(t, col, single, sum(1 for k in ktime if k < tm)) for (tm, t, col, single) in vs]


def share(x, tot, n, skip):
    if x < skip or x >= n:
        return 0
    return ((x - skip + 1) * tot) // (n - skip) - ((x - skip) * tot) // (n - skip)


def _kernel(ax, aw, ao, bx, bw, bo, out_hbm,
            x_b, w_b, wo_b, wt_s, kp_s, qt_s, vt_s, qf_s, ks_s, ot_s, ls_s, ob, bufa, bufb, bufc,
            s_s, p_c, l_c, o_c, v_c, lv_c, vm_s, kx_s, px_s, kb2, z_ref, isem, osem):
    b = pl.program_id(0)
    bufs = (bufa, bufb, bufc)

    def kbuf(ph):
        return bufs[(ph + 2) % NPH]

    def in_refs(src3, slot, j):
        x, w, wo = src3
        if j < 3:
            c0 = (D, 0, 2 * D)[j]
            return w.at[:, c0:c0 + D], w_b.at[slot, :, c0:c0 + D]
        if j < 3 + NXC:
            i = j - 3
            return x.at[0, i * PR:(i + 1) * PR, :], x_b.at[slot, i * PR:(i + 1) * PR, :]
        return wo, wo_b.at[slot]

    @pl.when(b == 0)
    def _():
        for slot, src3 in enumerate(((ax, aw, ao), (bx, bw, bo))):
            for j in (0, 3, 4, 5, 6, 1, 2, 7):
                src, dst = in_refs(src3, slot, j)
                pltpu.make_async_copy(src, dst, isem.at[slot, j]).start()
        for j in range(NZ):
            z_ref[j] = 0

    def wait_in(j):
        dst = in_refs((ax, aw, ao), b, j)[1]
        pltpu.make_async_copy(dst, dst, isem.at[b, j]).wait()

    def ldk(it, ph, row, n=8):
        return kbuf(ph)[pl.ds(pl.multiple_of(KOFF + it * (S // 2), 8) + row, n), :]

    def prep_gen(h, ph):
        for i0 in range(0, len(PITEMS), PORD):
            for d in range(DH):
                for (c, single) in PITEMS[i0:i0 + PORD]:
                    n = 8 if single else 16
                    col = ks_s[h, ks_off(c, single): ks_off(c, single) + n, :][:, d:d + 1]
                    base = kb_off(c, single) + d * n
                    bufs[ph][base: base + n, :] = pltpu.bitcast(jnp.broadcast_to(col, (n, 128)), U32)
                    yield

    nt_dims = (((1,), (1,)), ((), ()))
    stats = {}

    def upd(name, val):
        stats[name] = val if name not in stats else jnp.maximum(stats[name], val)

    def proj_k(i):
        xc = x_b[b, pl.ds(i * PR, PR), :]
        kc = jnp.dot(xc, w_b[b, :, D:2 * D], preferred_element_type=F32)
        upd("k", jnp.max(jnp.abs(kc).reshape(PR // 8, 8, D), axis=0))
        kp_s[i * (PR // 2):(i + 1) * (PR // 2), :] = pltpu.bitcast(kc.astype(BF), U32)

    def spread_k(i):
        for h in range(H):
            g, r = divmod(h, 8)
            it, ph = divmod(h, NPH)
            kr = kp_s[i * (PR // 2):(i + 1) * (PR // 2), g * 128:(g + 1) * 128]
            if r:
                kr = pltpu.roll(kr, 128 - DH * r, axis=1)
            ko = KOFF + it * (S // 2) + i * (PR // 2)
            kbuf(ph)[ko: ko + PR // 2, :] = kr
            if ph == 1 and i == 0:
                xo = XOFF + it * XC * (CH // 2)
                kbuf(0)[xo: xo + XC * (CH // 2), :] = kr[0: XC * (CH // 2)]
            for c in range(i * (PR // CH), (i + 1) * (PR // CH)):
                r0 = (c % (PR // CH)) * (CH // 2)
                ks_s[h, ks_off(c, False): ks_off(c, False) + 16, :] = (
                    pltpu.bitcast(kr[r0 + VB * 8: r0 + VB * 8 + 8], BF).astype(F32))
                if c in HM:
                    kf = pltpu.bitcast(kr[r0 + HB * 8: r0 + HB * 8 + 8], BF).astype(F32)
                    fo = FOFF + (it * HST + HM.index(c)) * 8
                    kbuf(ph)[fo: fo + 8, :] = pltpu.bitcast(kf[0:8], U32)
                    if ph == 1 and c < XC:
                        xf = XFO + (it * XC + c) * 8
                        kbuf(0)[xf: xf + 8, :] = pltpu.bitcast(kf[0:8], U32)
                    if c in HALF:
                        ks_s[h, ks_off(c, True): ks_off(c, True) + 8, :] = kf[8:16]
                    else:
                        kx_s[h] = kf[8:16]

    def proj_q(i):
        xc = x_b[b, pl.ds(i * PR, PR), :]
        q = lax.dot_general(wt_s[0:D, :], xc, nt_dims, preferred_element_type=F32) * QSCALE
        upd("q", jnp.sum((q * q).reshape(H, DH, PR), axis=1))
        qt_s[:, pl.ds(i * PR, PR)] = pltpu.bitcast(q.astype(BF), U32)
        qf_s[0:H, :, pl.ds(i * PR, PR)] = q.reshape(H, DH, PR)

    def proj_v(i):
        xc = x_b[b, pl.ds(i * PR, PR), :]
        v = lax.dot_general(wt_s[D:2 * D, :], xc, nt_dims, preferred_element_type=F32)
        va = jnp.abs(v)
        va = jnp.maximum(jnp.maximum(va[:, 0:128], va[:, 128:256]),
                         jnp.maximum(va[:, 256:384], va[:, 384:512]))
        va = jnp.max(va.reshape(H, 2, 8, 128), axis=1)
        vm_s[...] = va if i == 0 else jnp.maximum(vm_s[...], va)
        vt_s[:, pl.ds(i * PR, PR)] = v
        return v

    def pre_kb(h):
        kx = kx_s[h]
        for d in range(DH):
            kb2[(h * DH + d) * 8:(h * DH + d + 1) * 8, :] = jnp.broadcast_to(kx[:, d:d + 1], (8, 128))

    def pre_x(n, h, c0, pace):
        z = z_ref[n]
        zp = z_ref[NSTEP + n % NPAD]
        kb2[pl.ds(pl.multiple_of(H * DH * 8 + (n % NPAD) * 32 + zp, 8), 8), :] = pace
        qf_s[H + zp, 0:8, (n % NPAD) * 512:(n % NPAD) * 512 + 128] = pace
        kv = kb2[pl.ds(pl.multiple_of(h * DH * 8 + z, 8), DH * 8), :]
        accs = [None] * XW
        for d in range(DH):
            for x in range(XW):
                qs = jnp.broadcast_to(qf_s[h + z, d:d + 1, (c0 + x) * 128:(c0 + x + 1) * 128], (8, 128))
                t = kv[d * 8:(d + 1) * 8] * qs
                accs[x] = t if accs[x] is None else accs[x] + t
        px_s[h, :, c0 * 128:(c0 + XW) * 128] = jnp.exp2(jnp.concatenate(accs, axis=1))

    wait_in(0); wait_in(3)
    proj_k(0)
    wait_in(4); wait_in(5)
    proj_k(1)
    spread_k(0)
    proj_k(2)
    wait_in(6); wait_in(1); wait_in(2)
    wt_s[0:D, :] = w_b[b, :, 0:D].T
    wt_s[D:2 * D, :] = w_b[b, :, 2 * D:3 * D].T
    proj_k(3)
    spread_k(1)
    for i in range(NXC):
        proj_q(i)
        if i < 2:
            spread_k(2 + i)
        if i == 0:
            for h in range(H):
                pre_kb(h)
    per = H * (S // 128) // XW // NXC
    for i in range(NXC):
        v = proj_v(i)
        for m in range(per):
            n = i * per + m
            h, c0 = divmod(n * XW, S // 128)
            ctile, mm = divmod(m, per // 4)
            r = (mm * (D // 8) // (per // 4)) * 8
            pre_x(n, h, c0, v[r:r + 8, ctile * 128:(ctile + 1) * 128])

    km = jnp.max(stats["k"], axis=0, keepdims=True)
    km = km * km
    kseg = jnp.concatenate([km[:, g * 128:(g + 1) * 128] for g in range(4)], axis=0)
    for sh in (1, 2, 4, 8):
        kseg = kseg + pltpu.roll(kseg, sh, axis=1)
    safe_qk = jnp.max(stats["q"]) * jnp.max(kseg) <= SCORE_BOUND * SCORE_BOUND

    def vpu_col(z, ph, h, ct, c, single):
        z0 = pl.multiple_of(z, 8)
        ngrp = 1 if single else 2
        slabs = {}

        def kvreg(e):
            g = e // VG
            if g not in slabs:
                cnt = min(VG, DH * ngrp - g * VG)
                rows = pl.ds(z0 + kb_off(c, single) + g * VG * 8, cnt * 8)
                slabs[g] = pltpu.bitcast(bufs[ph][rows, :], F32)
            return slabs[g][(e % VG) * 8:(e % VG + 1) * 8]

        accs = [None] * ngrp
        for d in range(DH):
            qs = jnp.broadcast_to(qf_s[h + z, d:d + 1, ct * 128:(ct + 1) * 128], (8, 128))
            for g in range(ngrp):
                t = kvreg(d * ngrp + g) * qs
                accs[g] = t if accs[g] is None else accs[g] + t
        return accs[0] if single else jnp.concatenate(accs, axis=0)

    def pv_step(h, c, pb, oacc):
        r = pl.multiple_of(h * DH, DH)
        o = jnp.dot(vt_s[pl.ds(r, DH), c * CH:(c + 1) * CH].astype(pb.dtype), pb,
                    preferred_element_type=F32)
        return o if oacc is None else o + oacc

    def carried_p(x):
        return pltpu.bitcast(p_c[x * CH // 2:(x + 1) * CH // 2, :], BF)

    def finish(h, qb, lacc, oacc):
        ls_s[qb, pl.ds(h, 1), :] = jnp.sum(lacc, axis=0, keepdims=True)
        ot_s[h, :, qb * TQ:(qb + 1) * TQ] = oacc

    lead = [x[:3] for x in timeline(NQ * NC)[1][:RC]]

    def lead_gen(h, ph):
        lv = [jnp.zeros((8, 128), F32)] * 4
        for v, (t, col, single) in enumerate(lead):
            p = jnp.exp2(vpu_col(z_ref[v], ph, h, col, t, single))
            v_c[v * 16: v * 16 + p.shape[0], :] = p
            lv[col] = lv[col] + (p if single else p[0:8] + p[8:16])
            if v == RC - 1:
                lv_c[...] = jnp.concatenate(lv, axis=1)
            yield

    def block(it, phs):
        h0 = it * NPH + phs[0]
        hprev = (h0 + H - 1) % H
        nui = len(phs) * NQ
        T = nui * NC
        pads = [pl.multiple_of(PADOFF + 32 * x + z_ref[NSTEP + x], 8) for x in range(NPAD)]
        pbs = {t: {} for t in range(T)}
        laccs = {}; oaccs = {}
        nkt, vsteps = timeline(T)
        assert [x[:3] for x in vsteps[:RC]] == lead
        vnext = [RC]; ng = [0]; nk = [0]; pend = []; lhist = []
        pgen = [prep_gen(jnp.minimum(h0 + n + 2, H - 1), (ph + 2) % NPH) for n, ph in enumerate(phs)]
        phn = (phs[-1] + 1) % NPH
        lgen = lead_gen(jnp.minimum(h0 + len(phs), H - 1), phn)
        kph = nkt // len(phs)

        def pre_p(j):
            return px_s[h0 + j // NQ, :, (j % NQ) * TQ:(j % NQ + 1) * TQ]

        def l_init(j):
            l0 = pre_p(j)
            return [l0[:, col * 128:(col + 1) * 128] for col in COLS]

        def e_blk(j, s, cols):
            p = jnp.exp2(s)
            ll = p[0:8]
            for x in range(1, s.shape[0] // 8):
                ll = ll + p[x * 8:(x + 1) * 8]
            for n, col in enumerate(cols):
                x = ll[:, n * 128:(n + 1) * 128] if len(cols) > 1 else ll
                if j not in laccs:
                    laccs[j] = l_init(j)
                laccs[j][col] = laccs[j][col] + x
                lhist.append(laccs[j][col])
            return p, ll

        def emit_vpu(upto_k=None, upto_t=None):
            while vnext[0] < len(vsteps):
                v = vnext[0]
                t, col, single, dead = vsteps[v]
                if not ((upto_k is not None and dead <= upto_k)
                        or (upto_t is not None and min(x[0] for x in vsteps[v:]) <= upto_t)):
                    break
                j, c = divmod(t, NC)
                s = vpu_col(z_ref[v], phs[j // NQ], h0 + j // NQ, (j % NQ) * 4 + col, c, single)
                pp, ll = e_blk(j, s, [col])
                pbs[t].setdefault('s' if single else 'v', {})[col] = pp
                if v >= NG0:
                    pend.append(ll)
                vnext[0] += 1

        lv0 = lv_c[...]
        laccs[0] = [lv0[:, col * 128:(col + 1) * 128] + y for col, y in zip(COLS, l_init(0))]
        for v, (t, col, single) in enumerate(lead):
            pbs[t].setdefault('s' if single else 'v', {})[col] = v_c[v * 16: v * 16 + (8 if single else 16), :]

        def gates():
            n, kx = divmod(nk[0], kph)
            gb = kbuf(phs[n - 1]) if (n >= 1 and kx < XC * 7) else kbuf(phs[n])
            emit_vpu(upto_k=nk[0])
            if len(lhist) > LG + 4:
                pend.append(lhist[-LG])
            while pend:
                gb[pl.ds(pads[ng[0] % NPAD], 8), :] = pltpu.bitcast(pend.pop(0), U32)
                ng[0] += 1
            for _ in range(share(kx, NPREP, kph - PE, max(PS, XC * 7) if n >= 1 else PS)):
                next(pgen[n])
            for _ in range(share(nk[0], RC, nkt, nkt - LS)):
                bufs[phn][pl.ds(pads[ng[0] % NPAD], 8), :] = pltpu.bitcast(lhist[-LG - (nk[0] % 4)], U32)
                next(lgen)
            nk[0] += 1

        def qk(t, sls):
            j, c = divmod(t, NC)
            h = h0 + j // NQ; ph = phs[j // NQ]; qb = j % NQ
            dup = (j == NQ and c < XC)
            hpos = [x for x, y in enumerate(sls) if y[0] == 'h']
            if hpos and hpos[0] > 0:
                qk(t, sls[:hpos[0]]); qk(t, sls[hpos[0]:])
                return
            if hpos:
                gates()
                if dup:
                    kf = kbuf(ph - 1)[pl.ds(pl.multiple_of(XFO + it * XC * 8, 8) + c * 8, 8), :]
                else:
                    fo = pl.multiple_of(FOFF + it * HST * 8, 8) + HM.index(c) * 8
                    kf = kbuf(ph)[pl.ds(fo, 8), :]
                s = jnp.dot(pltpu.bitcast(kf, F32)[:, 0:DH], qf_s[h, :, qb * TQ:(qb + 1) * TQ],
                            preferred_element_type=F32)
                pbs[t]['h'] = e_blk(j, s, COLS)[0]
                sls = sls[1:]
            if not sls:
                return
            ks = []
            for _, bb in sls:
                gates()
                row = c * CH // 2 + bb * 8
                if dup:
                    ks.append(kbuf(ph - 1)[pl.ds(pl.multiple_of(XOFF + it * XC * (CH // 2), 8) + row, 8), :])
                else:
                    ks.append(ldk(it, ph, row))
            kk = pltpu.bitcast(jnp.concatenate(ks, axis=0) if len(ks) > 1 else ks[0], BF)[:, 0:DH]
            w = pltpu.bitcast(qt_s[pl.ds(pl.multiple_of(h * 8, 8), 8), qb * TQ:(qb + 1) * TQ], BF)
            s = jnp.dot(kk, w, preferred_element_type=F32)
            for x, (_, bb) in enumerate(sls):
                pbs[t][bb] = e_blk(j, s[x * 16:(x + 1) * 16], COLS)[0]

        def gather_p(tb):
            emit_vpu(upto_t=tb)
            pp = pbs.pop(tb)
            pv = jnp.concatenate([pp['v'][col] for col in COLS], axis=1)
            rows = []
            for bb in range(8):
                if bb == VB:
                    rows.append(pv)
                elif bb in pp:
                    rows.append(pp[bb])
                elif 's' in pp:
                    rows += [pp['h'], jnp.concatenate([pp['s'][col] for col in COLS], axis=1)]
                else:
                    rows += [pp['h'], pre_p(tb // NC)]
            return jnp.concatenate(rows, axis=0)

        def do_pv(tb):
            if tb < 0:
                if tb == -SK:
                    oaccs[-1] = o_c[...]
                oaccs[-1] = pv_step(hprev, NC + tb, carried_p(tb + SK), oaccs[-1])
                if tb == -1:
                    finish(hprev, NQ - 1, l_c[...], oaccs[-1])
                return
            j, c = divmod(tb, NC)
            oaccs[j] = pv_step(h0 + j // NQ, c, gather_p(tb), oaccs.get(j))
            if c == NC - 1:
                finish(h0 + j // NQ, j % NQ, jnp.concatenate(laccs[j], axis=1), oaccs[j])

        for t in range(T):
            sls = slots(t % NC)
            if t == 0:
                cuts = [(CP[x], x - SK) for x in range(SK)]
            else:
                cuts = [(SPL, t - SK)] if t >= SK else []
            pos = 0
            for cut, tb in cuts:
                qk(t, sls[pos:cut])
                do_pv(tb)
                pos = cut
            qk(t, sls[pos:])
        for x in range(SK):
            p_c[x * CH // 2:(x + 1) * CH // 2, :] = pltpu.bitcast(gather_p(T - SK + x).astype(BF), U32)
        l_c[...] = jnp.concatenate(laccs[nui - 1], axis=1)
        o_c[...] = oaccs[nui - 1]

    for hh in range(2):
        for _ in prep_gen(hh, hh):
            pass
    p_c[...] = jnp.zeros(p_c.shape, U32)
    l_c[...] = jnp.ones(l_c.shape, F32)
    o_c[...] = jnp.zeros(o_c.shape, F32)
    for _ in lead_gen(0, 0):
        pass

    @pl.when(safe_qk)
    def _():
        def body(i, c):
            block(i, BLOCKS[0])
            pl.when(i * NPH + BLOCKS[1][0] < H)(functools.partial(block, i, BLOCKS[1]))
            return c
        lax.fori_loop(0, NIT, body, 0)

    o = o_c[...]
    for x in range(SK):
        o = pv_step(H - 1, NC - SK + x, carried_p(x), o)
    finish(H - 1, NQ - 1, l_c[...], o)
    vh = jnp.max(jnp.max(vm_s[...], axis=1), axis=1, keepdims=True)
    safe = safe_qk & (jnp.min(vh) >= V_LO) & (jnp.max(vh) <= V_HI)

    def slow_body(it, carry):
        sc = 256
        for ph in range(NPH):
            h = it * NPH + ph

            def unit(qb, c2):
                c0 = pl.multiple_of(qb * TQ, TQ)
                w = pltpu.bitcast(qt_s[pl.ds(pl.multiple_of(h * 8, 8), 8), pl.ds(c0, TQ)], BF)

                def p1(c, m):
                    ro = pl.multiple_of(c * (sc // 2), 8)
                    kk = pltpu.bitcast(ldk(it, ph, ro, sc // 2), BF)[:, 0:DH]
                    s = jnp.dot(kk, w, preferred_element_type=F32)
                    s_s[pl.ds(pl.multiple_of(c * sc, sc), sc), :] = s
                    return jnp.maximum(m, jnp.max(s, axis=0, keepdims=True))
                m = lax.fori_loop(0, S // sc, p1, jnp.full((1, TQ), -jnp.inf, F32))

                def p2(c, lo):
                    l, o = lo
                    co = pl.multiple_of(c * sc, sc)
                    p = jnp.exp2(s_s[pl.ds(co, sc), :] - m)
                    vt = vt_s[pl.ds(pl.multiple_of(h * DH, DH), DH), pl.ds(co, sc)]
                    return (l + jnp.sum(p.reshape(sc // 8, 8, TQ), axis=0),
                            o + jnp.dot(vt, p, preferred_element_type=F32))
                l, o = lax.fori_loop(0, S // sc, p2,
                                     (jnp.zeros((8, TQ), F32), jnp.zeros((DH, TQ), F32)))
                ot_s[h, :, pl.ds(c0, TQ)] = o
                ls_s[qb, pl.ds(h, 1), :] = jnp.sum(l, axis=0, keepdims=True)
                return c2
            lax.fori_loop(0, jnp.where(h < H, NQ, 0), unit, 0)
        return carry

    @pl.when(jnp.logical_not(safe))
    def _():
        lax.fori_loop(0, NIT, slow_body, 0)

    wait_in(3 + NXC)

    def out_copy(bb, n):
        r0, nr = OCH[n]
        return pltpu.make_async_copy(
            ob.at[r0:r0 + nr, :],
            out_hbm.at[0, r0:r0 + nr, pl.ds(pl.multiple_of(bb * D, D), D)], osem.at[n])

    @pl.when(b == 1)
    def _():
        for n in range(len(OCH)):
            out_copy(0, n).wait()

    for n, (r0, nr) in enumerate(OCH):
        qb, c0 = divmod(r0, TQ)
        inv = 1.0 / ls_s[qb, :, c0:c0 + nr]
        oc = (ot_s[:, :, r0:r0 + nr] * inv.reshape(H, 1, nr)).reshape(D, nr).T.astype(BF)
        r = jnp.dot(oc, wo_b[b], preferred_element_type=F32)
        ob[r0:r0 + nr, :] = r.astype(BF)
        out_copy(b, n).start()

    @pl.when(b == 1)
    def _():
        for n in range(len(OCH)):
            out_copy(1, n).wait()


@jax.jit
def pallas_concat_heads__softmax_full_mha__softmax_full_mha__prompt_kernel(
    A_x: jax.Array,
    A_wqkv: jax.Array,
    A_wo: jax.Array,
    B_x: jax.Array,
    B_wqkv: jax.Array,
    B_wo: jax.Array,
):
    any_spec = pl.BlockSpec(memory_space=pl.ANY)
    vm = pltpu.VMEM
    return pl.pallas_call(
        _kernel,
        out_shape=jax.ShapeDtypeStruct((1, S, 2 * D), BF),
        grid=(2,),
        in_specs=[any_spec] * 6,
        out_specs=any_spec,
        scratch_shapes=[
            vm((2, S, D), BF), vm((2, D, 3 * D), BF), vm((2, D, D), BF),
            vm((2 * D, D), BF),
            vm((S // 2, D), U32), vm((D // 2, S), U32), vm((D, S), F32),
            vm((H + 1, DH, S), F32), vm((H, NGT * 8, 128), F32),
            vm((H, DH, S), F32), vm((NQ, H, TQ), F32), vm((S, D), BF),
            vm((TOTR, 128), U32), vm((TOTR, 128), U32), vm((TOTR, 128), U32),
            vm((S, TQ), F32),
            vm((SK * CH // 2, TQ), U32), vm((8, TQ), F32), vm((DH, TQ), F32),
            vm((RC * 16, 128), F32), vm((8, TQ), F32), vm((H, 8, 128), F32),
            vm((H, 8, 128), F32), vm((H, 8, S), F32), vm((H * DH * 8 + NPAD * 32, 128), F32),
            pltpu.SMEM((NZ,), jnp.int32),
            pltpu.SemaphoreType.DMA((2, NXC + 4)), pltpu.SemaphoreType.DMA((len(OCH),)),
        ],
        compiler_params=pltpu.CompilerParams(
            vmem_limit_bytes=100 * 1024 * 1024, dimension_semantics=("arbitrary",)),
    )(A_x, A_wqkv, A_wo, B_x, B_wqkv, B_wo)
```

```python
import functools
import math

import jax
import jax.numpy as jnp
from jax import lax
from jax.experimental import pallas as pl
from jax.experimental.pallas import tpu as pltpu

S = 2048; D = 512; H = 32; DH = 16
TQ = 512
CH = 128
PR = 512
NQ = S // TQ; NC = S // CH; NXC = S // PR
F32 = jnp.float32; BF = jnp.bfloat16; U32 = jnp.uint32

QSCALE = (DH ** -0.5) * math.log2(math.e)
SCORE_BOUND = 64.0
V_LO = 2.0 ** -30
V_HI = 2.0 ** 50

SK = 2
SPL = 2
LG = 50
PS = 16; PE = 12
VG_D = (5, 4, 4, 3); VG_S = (4, 4, 4, 4); PORD = 4
NG0 = 0
DLT = 24; SDL = 80; SO = (80, 16)
RC = 4; LS = 8
CP = (3, 6)
XC = 4
HALF = [c for c in range(NC) if c % 2]
XCH = 6
HM = sorted(HALF + [XCH])
HST = -(-len(HM) // 4) * 4
XW = 2
VB = 0
MXB = [x for x in range(7, -1, -1) if x != VB]
HB = MXB[SPL]
NGT = 2 * NC + len(HALF)
KBR = NGT * DH * 8
PITEMS = [(c, False) for c in range(NC)]
for _n, _c in enumerate(HALF):
    PITEMS.insert(_c + _n + 1, (_c, True))
NPREP = len(PITEMS) * DH
NPH = 3
BLOCKS = ((0, 1), (2,))
NIT = -(-H // NPH)
KOFF = KBR
FOFF = KOFF + NIT * (S // 2)
XOFF = FOFF + NIT * HST * 8
XFO = XOFF + NIT * XC * (CH // 2)
PADOFF = XFO + NIT * XC * 8
NPAD = 4
TOTR = PADOFF + 32 * NPAD
assert all(x % 32 == 0 for x in (KOFF, FOFF, XOFF, XFO, PADOFF, TOTR))
NSTEP = 2 * NQ * 4 * (NC + len(HALF))
NZ = NSTEP + NPAD
OCH = ((0, 128), (128, 384), (512, 512), (1024, 512), (1536, 384), (1920, 128))
COLS = (0, 1, 2, 3)


def kb_off(c, single):
    return (2 * NC + HALF.index(c)) * DH * 8 if single else c * 2 * DH * 8


def ks_off(c, single):
    return (2 * NC + HALF.index(c)) * 8 if single else c * 16


def slots(c):
    return [('h', c) if (c in HM and x == HB) else ('b', x) for x in MXB]


def timeline(T):
    ktime = []; pvtime = {}; now = 0
    for t in range(T):
        for n, sl in enumerate(slots(t % NC)):
            if n == SPL:
                pvtime[t - SK] = now; now += 16
            ktime.append(now); now += 8 if sl[0] == 'h' else 16
    for t in range(T - SK, T):
        pvtime[t] = now + 128 * (t - T + SK) + 32
    vs = [(pvtime[t] - DLT - (3 - col) * 32, t, col, False) for t in range(T) for col in COLS]
    free = sorted(pvtime[t] - o for t in range(-SK, T) for o in SO)
    for t in range(T - 1, -1, -1):
        if t % NC in HALF:
            for col in reversed(COLS):
                tm = [x for x in free if x <= pvtime[t] - SDL][-1]
                free.remove(tm)
                vs.append((tm, t, col, True))
    vs.sort()
    return len(ktime), [(t, col, single, sum(1 for k in ktime if k < tm)) for (tm, t, col, single) in vs]


def share(x, tot, n, skip):
    if x < skip or x >= n:
        return 0
    return ((x - skip + 1) * tot) // (n - skip) - ((x - skip) * tot) // (n - skip)


def _kernel(ax, aw, ao, bx, bw, bo, out_hbm,
            x_b, w_b, wo_b, wt_s, kp_s, qt_s, vt_s, qf_s, ks_s, ot_s, ls_s, ob, bufa, bufb, bufc,
            s_s, p_c, l_c, o_c, v_c, lv_c, vm_s, kx_s, px_s, kb2, z_ref, isem, osem):
    b = pl.program_id(0)
    bufs = (bufa, bufb, bufc)

    def kbuf(ph):
        return bufs[(ph + 2) % NPH]

    def in_refs(src3, slot, j):
        x, w, wo = src3
        if j < 3:
            c0 = (D, 0, 2 * D)[j]
            return w.at[:, c0:c0 + D], w_b.at[slot, :, c0:c0 + D]
        if j < 3 + NXC:
            i = j - 3
            return x.at[0, i * PR:(i + 1) * PR, :], x_b.at[slot, i * PR:(i + 1) * PR, :]
        return wo, wo_b.at[slot]

    @pl.when(b == 0)
    def _():
        for slot, src3 in enumerate(((ax, aw, ao), (bx, bw, bo))):
            for j in (0, 3, 4, 5, 6, 1, 2, 7):
                src, dst = in_refs(src3, slot, j)
                pltpu.make_async_copy(src, dst, isem.at[slot, j]).start()
        for j in range(NZ):
            z_ref[j] = 0

    def wait_in(j):
        dst = in_refs((ax, aw, ao), b, j)[1]
        pltpu.make_async_copy(dst, dst, isem.at[b, j]).wait()

    def ldk(it, ph, row, n):
        return kbuf(ph)[pl.ds(pl.multiple_of(KOFF + it * (S // 2), 8) + row, n), :]

    def prep_gen(h, ph):
        for i0 in range(0, len(PITEMS), PORD):
            for d in range(DH):
                for (c, single) in PITEMS[i0:i0 + PORD]:
                    n = 8 if single else 16
                    col = ks_s[h, ks_off(c, single): ks_off(c, single) + n, :][:, d:d + 1]
                    base = kb_off(c, single) + d * n
                    bufs[ph][base: base + n, :] = pltpu.bitcast(jnp.broadcast_to(col, (n, 128)), U32)
                    yield

    def mac(acc, kv, hz, ct, d0, g):
        n = kv.shape[0] // g
        qs = jnp.concatenate([jnp.broadcast_to(qf_s[hz, d:d + 1, ct * 128:(ct + 1) * 128], (n, 128))
                              for d in range(d0, d0 + g)], axis=0)
        t = (kv * qs).reshape(g, n, 128)
        if acc is not None:
            t = jnp.concatenate([acc[None], t], axis=0)
        return jnp.sum(t, axis=0)

    nt_dims = (((1,), (1,)), ((), ()))
    stats = {}

    def upd(name, val):
        stats[name] = val if name not in stats else jnp.maximum(stats[name], val)

    def proj_k(i):
        xc = x_b[b, pl.ds(i * PR, PR), :]
        kc = jnp.dot(xc, w_b[b, :, D:2 * D], preferred_element_type=F32)
        upd("k", jnp.max(jnp.abs(kc).reshape(PR // 8, 8, D), axis=0))
        kp_s[i * (PR // 2):(i + 1) * (PR // 2), :] = pltpu.bitcast(kc.astype(BF), U32)

    def spread_k(i):
        for h in range(H):
            g, r = divmod(h, 8)
            it, ph = divmod(h, NPH)
            kr = kp_s[i * (PR // 2):(i + 1) * (PR // 2), g * 128:(g + 1) * 128]
            if r:
                kr = pltpu.roll(kr, 128 - DH * r, axis=1)
            ko = KOFF + it * (S // 2) + i * (PR // 2)
            kbuf(ph)[ko: ko + PR // 2, :] = kr
            if ph == 1 and i == 0:
                xo = XOFF + it * XC * (CH // 2)
                kbuf(0)[xo: xo + XC * (CH // 2), :] = kr[0: XC * (CH // 2)]
            for c in range(i * (PR // CH), (i + 1) * (PR // CH)):
                r0 = (c % (PR // CH)) * (CH // 2)
                ks_s[h, ks_off(c, False): ks_off(c, False) + 16, :] = (
                    pltpu.bitcast(kr[r0 + VB * 8: r0 + VB * 8 + 8], BF).astype(F32))
                if c in HM:
                    kf = pltpu.bitcast(kr[r0 + HB * 8: r0 + HB * 8 + 8], BF).astype(F32)
                    fo = FOFF + (it * HST + HM.index(c)) * 8
                    kbuf(ph)[fo: fo + 8, :] = pltpu.bitcast(kf[0:8], U32)
                    if ph == 1 and c < XC:
                        xf = XFO + (it * XC + c) * 8
                        kbuf(0)[xf: xf + 8, :] = pltpu.bitcast(kf[0:8], U32)
                    if c in HALF:
                        ks_s[h, ks_off(c, True): ks_off(c, True) + 8, :] = kf[8:16]
                    else:
                        kx_s[h] = kf[8:16]

    def proj_q(i):
        xc = x_b[b, pl.ds(i * PR, PR), :]
        q = lax.dot_general(wt_s[0:D, :], xc, nt_dims, preferred_element_type=F32) * QSCALE
        upd("q", jnp.sum((q * q).reshape(H, DH, PR), axis=1))
        qt_s[:, pl.ds(i * PR, PR)] = pltpu.bitcast(q.astype(BF), U32)
        qf_s[0:H, :, pl.ds(i * PR, PR)] = q.reshape(H, DH, PR)

    def proj_v(i):
        xc = x_b[b, pl.ds(i * PR, PR), :]
        v = lax.dot_general(wt_s[D:2 * D, :], xc, nt_dims, preferred_element_type=F32)
        va = jnp.abs(v)
        va = jnp.maximum(jnp.maximum(va[:, 0:128], va[:, 128:256]),
                         jnp.maximum(va[:, 256:384], va[:, 384:512]))
        va = jnp.max(va.reshape(H, 2, 8, 128), axis=1)
        vm_s[...] = va if i == 0 else jnp.maximum(vm_s[...], va)
        vt_s[:, pl.ds(i * PR, PR)] = v
        return v

    def pre_kb(h):
        kx = kx_s[h]
        for d in range(DH):
            kb2[(h * DH + d) * 8:(h * DH + d + 1) * 8, :] = jnp.broadcast_to(kx[:, d:d + 1], (8, 128))

    def pre_x(n, h, c0, pace):
        z = z_ref[n]
        zp = z_ref[NSTEP + n % NPAD]
        kb2[pl.ds(pl.multiple_of(H * DH * 8 + (n % NPAD) * 32 + zp, 8), 8), :] = pace
        qf_s[H + zp, 0:8, (n % NPAD) * 512:(n % NPAD) * 512 + 128] = pace
        hz = h + z
        kv = kb2[pl.ds(pl.multiple_of(h * DH * 8 + z, 8), DH * 8), :]
        outs = [mac(None, kv, hz, c0 + x, 0, DH) for x in range(XW)]
        px_s[h, :, c0 * 128:(c0 + XW) * 128] = jnp.exp2(jnp.concatenate(outs, axis=1))

    wait_in(0); wait_in(3)
    proj_k(0)
    wait_in(4); wait_in(5)
    proj_k(1)
    spread_k(0)
    proj_k(2)
    wait_in(6); wait_in(1); wait_in(2)
    wt_s[0:D, :] = w_b[b, :, 0:D].T
    wt_s[D:2 * D, :] = w_b[b, :, 2 * D:3 * D].T
    proj_k(3)
    spread_k(1)
    for i in range(NXC):
        proj_q(i)
        if i < 2:
            spread_k(2 + i)
        if i == 0:
            for h in range(H):
                pre_kb(h)
    per = H * (S // 128) // XW // NXC
    for i in range(NXC):
        v = proj_v(i)
        for m in range(per):
            n = i * per + m
            h, c0 = divmod(n * XW, S // 128)
            ctile, mm = divmod(m, per // 4)
            r = (mm * (D // 8) // (per // 4)) * 8
            pre_x(n, h, c0, v[r:r + 8, ctile * 128:(ctile + 1) * 128])

    km = jnp.max(stats["k"], axis=0, keepdims=True)
    km = km * km
    kseg = jnp.concatenate([km[:, g * 128:(g + 1) * 128] for g in range(4)], axis=0)
    for sh in (1, 2, 4, 8):
        kseg = kseg + pltpu.roll(kseg, sh, axis=1)
    safe_qk = jnp.max(stats["q"]) * jnp.max(kseg) <= SCORE_BOUND * SCORE_BOUND

    def vpu_col(z, ph, h, ct, c, single):
        z0 = pl.multiple_of(z, 8)
        n = 8 if single else 16
        hz = h + z
        acc = None
        d0 = 0
        for g in (VG_S if single else VG_D):
            kv = pltpu.bitcast(bufs[ph][pl.ds(z0 + (kb_off(c, single) + d0 * n), g * n), :], F32)
            acc = mac(acc, kv, hz, ct, d0, g)
            d0 += g
        return acc

    def pv_step(h, c, pb, oacc):
        r = pl.multiple_of(h * DH, DH)
        o = jnp.dot(vt_s[pl.ds(r, DH), c * CH:(c + 1) * CH].astype(pb.dtype), pb,
                    preferred_element_type=F32)
        return o if oacc is None else o + oacc

    def carried_p(x):
        return pltpu.bitcast(p_c[x * CH // 2:(x + 1) * CH // 2, :], BF)

    def finish(h, qb, lacc, oacc):
        ls_s[qb, pl.ds(h, 1), :] = jnp.sum(lacc, axis=0, keepdims=True)
        ot_s[h, :, qb * TQ:(qb + 1) * TQ] = oacc

    lead = [x[:3] for x in timeline(NQ * NC)[1][:RC]]

    def lead_gen(h, ph):
        lv = [jnp.zeros((8, 128), F32)] * 4
        for v, (t, col, single) in enumerate(lead):
            p = jnp.exp2(vpu_col(z_ref[v], ph, h, col, t, single))
            v_c[v * 16: v * 16 + p.shape[0], :] = p
            lv[col] = lv[col] + (p if single else p[0:8] + p[8:16])
            if v == RC - 1:
                lv_c[...] = jnp.concatenate(lv, axis=1)
            yield

    def block(it, phs):
        h0 = it * NPH + phs[0]
        hprev = (h0 + H - 1) % H
        nui = len(phs) * NQ
        T = nui * NC
        pads = [pl.multiple_of(PADOFF + 32 * x + z_ref[NSTEP + x], 8) for x in range(NPAD)]
        pbs = {t: {} for t in range(T)}
        laccs = {}; oaccs = {}
        nkt, vsteps = timeline(T)
        assert [x[:3] for x in vsteps[:RC]] == lead
        vnext = [RC]; ng = [0]; nk = [0]; pend = []; lhist = []
        pgen = [prep_gen(jnp.minimum(h0 + n + 2, H - 1), (ph + 2) % NPH) for n, ph in enumerate(phs)]
        phn = (phs[-1] + 1) % NPH
        lgen = lead_gen(jnp.minimum(h0 + len(phs), H - 1), phn)
        kbase = pl.multiple_of(KOFF + it * (S // 2), 8)
        xbase = pl.multiple_of(XOFF + it * XC * (CH // 2), 8)
        fbase = pl.multiple_of(FOFF + it * HST * 8, 8)
        xfbase = pl.multiple_of(XFO + it * XC * 8, 8)
        hs = [h0 + n for n in range(len(phs))]
        wrow = [pl.multiple_of(hh * 8, 8) for hh in hs]
        kph = nkt // len(phs)

        def pre_p(j):
            return px_s[hs[j // NQ], :, (j % NQ) * TQ:(j % NQ + 1) * TQ]

        def l_init(j):
            l0 = pre_p(j)
            return [l0[:, col * 128:(col + 1) * 128] for col in COLS]

        def e_blk(j, s, cols):
            p = jnp.exp2(s)
            ll = p[0:8]
            for x in range(1, s.shape[0] // 8):
                ll = ll + p[x * 8:(x + 1) * 8]
            for n, col in enumerate(cols):
                x = ll[:, n * 128:(n + 1) * 128] if len(cols) > 1 else ll
                if j not in laccs:
                    laccs[j] = l_init(j)
                laccs[j][col] = laccs[j][col] + x
                lhist.append(laccs[j][col])
            return p, ll

        def emit_vpu(upto_k=None, upto_t=None):
            while vnext[0] < len(vsteps):
                v = vnext[0]
                t, col, single, dead = vsteps[v]
                if not ((upto_k is not None and dead <= upto_k)
                        or (upto_t is not None and min(x[0] for x in vsteps[v:]) <= upto_t)):
                    break
                j, c = divmod(t, NC)
                s = vpu_col(z_ref[v], phs[j // NQ], hs[j // NQ], (j % NQ) * 4 + col, c, single)
                pp, ll = e_blk(j, s, [col])
                pbs[t].setdefault('s' if single else 'v', {})[col] = pp
                if v >= NG0:
                    pend.append(ll)
                vnext[0] += 1

        lv0 = lv_c[...]
        laccs[0] = [lv0[:, col * 128:(col + 1) * 128] + y for col, y in zip(COLS, l_init(0))]
        for v, (t, col, single) in enumerate(lead):
            pbs[t].setdefault('s' if single else 'v', {})[col] = v_c[v * 16: v * 16 + (8 if single else 16), :]

        def gates():
            n, kx = divmod(nk[0], kph)
            gb = kbuf(phs[n - 1]) if (n >= 1 and kx < XC * 7) else kbuf(phs[n])
            emit_vpu(upto_k=nk[0])
            if len(lhist) > LG + 4:
                pend.append(lhist[-LG])
            while pend:
                gb[pl.ds(pads[ng[0] % NPAD], 8), :] = pltpu.bitcast(pend.pop(0), U32)
                ng[0] += 1
            for _ in range(share(kx, NPREP, kph - PE, max(PS, XC * 7) if n >= 1 else PS)):
                next(pgen[n])
            for _ in range(share(nk[0], RC, nkt, nkt - LS)):
                bufs[phn][pl.ds(pads[ng[0] % NPAD], 8), :] = pltpu.bitcast(lhist[-LG - (nk[0] % 4)], U32)
                next(lgen)
            nk[0] += 1

        def qk(t, sls):
            j, c = divmod(t, NC)
            h = hs[j // NQ]; ph = phs[j // NQ]; qb = j % NQ
            dup = (j == NQ and c < XC)
            hpos = [x for x, y in enumerate(sls) if y[0] == 'h']
            if hpos and hpos[0] > 0:
                qk(t, sls[:hpos[0]]); qk(t, sls[hpos[0]:])
                return
            if hpos:
                gates()
                if dup:
                    kf = kbuf(ph - 1)[pl.ds(xfbase + c * 8, 8), :]
                else:
                    kf = kbuf(ph)[pl.ds(fbase + HM.index(c) * 8, 8), :]
                s = jnp.dot(pltpu.bitcast(kf, F32)[:, 0:DH], qf_s[h, :, qb * TQ:(qb + 1) * TQ],
                            preferred_element_type=F32)
                pbs[t]['h'] = e_blk(j, s, COLS)[0]
                sls = sls[1:]
            if not sls:
                return
            ks = []
            for _, bb in sls:
                gates()
                row = c * CH // 2 + bb * 8
                if dup:
                    ks.append(kbuf(ph - 1)[pl.ds(xbase + row, 8), :])
                else:
                    ks.append(kbuf(ph)[pl.ds(kbase + row, 8), :])
            kk = pltpu.bitcast(jnp.concatenate(ks, axis=0) if len(ks) > 1 else ks[0], BF)[:, 0:DH]
            w = pltpu.bitcast(qt_s[pl.ds(wrow[j // NQ], 8), qb * TQ:(qb + 1) * TQ], BF)
            s = jnp.dot(kk, w, preferred_element_type=F32)
            for x, (_, bb) in enumerate(sls):
                pbs[t][bb] = e_blk(j, s[x * 16:(x + 1) * 16], COLS)[0]

        def gather_p(tb):
            emit_vpu(upto_t=tb)
            pp = pbs.pop(tb)
            pv = jnp.concatenate([pp['v'][col] for col in COLS], axis=1)
            rows = []
            for bb in range(8):
                if bb == VB:
                    rows.append(pv)
                elif bb in pp:
                    rows.append(pp[bb])
                elif 's' in pp:
                    rows += [pp['h'], jnp.concatenate([pp['s'][col] for col in COLS], axis=1)]
                else:
                    rows += [pp['h'], pre_p(tb // NC)]
            return jnp.concatenate(rows, axis=0)

        def do_pv(tb):
            if tb < 0:
                if tb == -SK:
                    oaccs[-1] = o_c[...]
                oaccs[-1] = pv_step(hprev, NC + tb, carried_p(tb + SK), oaccs[-1])
                if tb == -1:
                    finish(hprev, NQ - 1, l_c[...], oaccs[-1])
                return
            j, c = divmod(tb, NC)
            oaccs[j] = pv_step(hs[j // NQ], c, gather_p(tb), oaccs.get(j))
            if c == NC - 1:
                finish(hs[j // NQ], j % NQ, jnp.concatenate(laccs[j], axis=1), oaccs[j])

        for t in range(T):
            sls = slots(t % NC)
            if t == 0:
                cuts = [(CP[x], x - SK) for x in range(SK)]
            else:
                cuts = [(SPL, t - SK)] if t >= SK else []
            pos = 0
            for cut, tb in cuts:
                qk(t, sls[pos:cut])
                do_pv(tb)
                pos = cut
            qk(t, sls[pos:])
        for x in range(SK):
            p_c[x * CH // 2:(x + 1) * CH // 2, :] = pltpu.bitcast(gather_p(T - SK + x).astype(BF), U32)
        l_c[...] = jnp.concatenate(laccs[nui - 1], axis=1)
        o_c[...] = oaccs[nui - 1]

    for hh in range(2):
        for _ in prep_gen(hh, hh):
            pass
    p_c[...] = jnp.zeros(p_c.shape, U32)
    l_c[...] = jnp.ones(l_c.shape, F32)
    o_c[...] = jnp.zeros(o_c.shape, F32)
    for _ in lead_gen(0, 0):
        pass

    @pl.when(safe_qk)
    def _():
        def body(i, c):
            block(i, BLOCKS[0])
            pl.when(i * NPH + BLOCKS[1][0] < H)(functools.partial(block, i, BLOCKS[1]))
            return c
        lax.fori_loop(0, NIT, body, 0)

    o = o_c[...]
    for x in range(SK):
        o = pv_step(H - 1, NC - SK + x, carried_p(x), o)
    finish(H - 1, NQ - 1, l_c[...], o)
    vh = jnp.max(jnp.max(vm_s[...], axis=1), axis=1, keepdims=True)
    safe = safe_qk & (jnp.min(vh) >= V_LO) & (jnp.max(vh) <= V_HI)

    def slow_body(it, carry):
        sc = 256
        for ph in range(NPH):
            h = it * NPH + ph

            def unit(qb, c2):
                c0 = pl.multiple_of(qb * TQ, TQ)
                w = pltpu.bitcast(qt_s[pl.ds(pl.multiple_of(h * 8, 8), 8), pl.ds(c0, TQ)], BF)

                def p1(c, m):
                    ro = pl.multiple_of(c * (sc // 2), 8)
                    kk = pltpu.bitcast(ldk(it, ph, ro, sc // 2), BF)[:, 0:DH]
                    s = jnp.dot(kk, w, preferred_element_type=F32)
                    s_s[pl.ds(pl.multiple_of(c * sc, sc), sc), :] = s
                    return jnp.maximum(m, jnp.max(s, axis=0, keepdims=True))
                m = lax.fori_loop(0, S // sc, p1, jnp.full((1, TQ), -jnp.inf, F32))

                def p2(c, lo):
                    l, o = lo
                    co = pl.multiple_of(c * sc, sc)
                    p = jnp.exp2(s_s[pl.ds(co, sc), :] - m)
                    vt = vt_s[pl.ds(pl.multiple_of(h * DH, DH), DH), pl.ds(co, sc)]
                    return (l + jnp.sum(p.reshape(sc // 8, 8, TQ), axis=0),
                            o + jnp.dot(vt, p, preferred_element_type=F32))
                l, o = lax.fori_loop(0, S // sc, p2,
                                     (jnp.zeros((8, TQ), F32), jnp.zeros((DH, TQ), F32)))
                ot_s[h, :, pl.ds(c0, TQ)] = o
                ls_s[qb, pl.ds(h, 1), :] = jnp.sum(l, axis=0, keepdims=True)
                return c2
            lax.fori_loop(0, jnp.where(h < H, NQ, 0), unit, 0)
        return carry

    @pl.when(jnp.logical_not(safe))
    def _():
        lax.fori_loop(0, NIT, slow_body, 0)

    wait_in(3 + NXC)

    def out_copy(bb, n):
        r0, nr = OCH[n]
        return pltpu.make_async_copy(
            ob.at[r0:r0 + nr, :],
            out_hbm.at[0, r0:r0 + nr, pl.ds(pl.multiple_of(bb * D, D), D)], osem.at[n])

    @pl.when(b == 1)
    def _():
        for n in range(len(OCH)):
            out_copy(0, n).wait()

    for n, (r0, nr) in enumerate(OCH):
        qb, c0 = divmod(r0, TQ)
        inv = 1.0 / ls_s[qb, :, c0:c0 + nr]
        oc = (ot_s[:, :, r0:r0 + nr] * inv.reshape(H, 1, nr)).reshape(D, nr).T.astype(BF)
        r = jnp.dot(oc, wo_b[b], preferred_element_type=F32)
        ob[r0:r0 + nr, :] = r.astype(BF)
        out_copy(b, n).start()

    @pl.when(b == 1)
    def _():
        for n in range(len(OCH)):
            out_copy(1, n).wait()


@jax.jit
def pallas_concat_heads__softmax_full_mha__softmax_full_mha__prompt_kernel(
    A_x: jax.Array,
    A_wqkv: jax.Array,
    A_wo: jax.Array,
    B_x: jax.Array,
    B_wqkv: jax.Array,
    B_wo: jax.Array,
):
    any_spec = pl.BlockSpec(memory_space=pl.ANY)
    vm = pltpu.VMEM
    return pl.pallas_call(
        _kernel,
        out_shape=jax.ShapeDtypeStruct((1, S, 2 * D), BF),
        grid=(2,),
        in_specs=[any_spec] * 6,
        out_specs=any_spec,
        scratch_shapes=[
            vm((2, S, D), BF), vm((2, D, 3 * D), BF), vm((2, D, D), BF),
            vm((2 * D, D), BF),
            vm((S // 2, D), U32), vm((D // 2, S), U32), vm((D, S), F32),
            vm((H + 1, DH, S), F32), vm((H, NGT * 8, 128), F32),
            vm((H, DH, S), F32), vm((NQ, H, TQ), F32), vm((S, D), BF),
            vm((TOTR, 128), U32), vm((TOTR, 128), U32), vm((TOTR, 128), U32),
            vm((S, TQ), F32),
            vm((SK * CH // 2, TQ), U32), vm((8, TQ), F32), vm((DH, TQ), F32),
            vm((RC * 16, 128), F32), vm((8, TQ), F32), vm((H, 8, 128), F32),
            vm((H, 8, 128), F32), vm((H, 8, S), F32), vm((H * DH * 8 + NPAD * 32, 128), F32),
            pltpu.SMEM((NZ,), jnp.int32),
            pltpu.SemaphoreType.DMA((2, NXC + 4)), pltpu.SemaphoreType.DMA((len(OCH),)),
        ],
        compiler_params=pltpu.CompilerParams(
            vmem_limit_bytes=100 * 1024 * 1024, dimension_semantics=("arbitrary",)),
    )(A_x, A_wqkv, A_wo, B_x, B_wqkv, B_wo)
```

```python
import functools
import math

import jax
import jax.numpy as jnp
from jax import lax
from jax.experimental import pallas as pl
from jax.experimental.pallas import tpu as pltpu

S = 2048; D = 512; H = 32; DH = 16
TQ = 512
CH = 128
PR = 512
NQ = S // TQ; NC = S // CH; NXC = S // PR
F32 = jnp.float32; BF = jnp.bfloat16; U32 = jnp.uint32

QSCALE = (DH ** -0.5) * math.log2(math.e)
SCORE_BOUND = 64.0
V_LO = 2.0 ** -30
V_HI = 2.0 ** 50

SK = 2
SPL = 2
LG = 50
PS = 24; PE = 10
VGS = (3, 4, 4, 5); PORD = 4
NG0 = 0
DLT = 24; SDL = 80; SO = (80, 16)
RC = 4; LS = 10
CP = (3, 5)
XC = 4
HALF = [c for c in range(NC) if c % 2]
XCH = 6
HM = sorted(HALF + [XCH])
HST = -(-len(HM) // 4) * 4
XW = 2
VB = 0
MXB = [x for x in range(7, -1, -1) if x != VB]
HB = MXB[SPL]
NGT = 2 * NC + len(HALF)
KBR = NGT * DH * 8
PITEMS = [(c, False) for c in range(NC)]
for _n, _c in enumerate(HALF):
    PITEMS.insert(_c + _n + 1, (_c, True))
NPREP = len(PITEMS) * DH
NPH = 3
BLOCKS = ((0, 1), (2,))
NIT = -(-H // NPH)
KOFF = KBR
FOFF = KOFF + NIT * (S // 2)
XOFF = FOFF + NIT * HST * 8
XFO = XOFF + NIT * XC * (CH // 2)
PADOFF = XFO + NIT * XC * 8
NPAD = 4
TOTR = PADOFF + 32 * NPAD
assert all(x % 32 == 0 for x in (KOFF, FOFF, XOFF, XFO, PADOFF, TOTR))
NSTEP = 2 * NQ * 4 * (NC + len(HALF))
NZ = NSTEP + NPAD
OCH = ((0, 128), (128, 384), (512, 512), (1024, 512), (1536, 384), (1920, 128))
COLS = (0, 1, 2, 3)


def kb_off(c, single):
    return (2 * NC + HALF.index(c)) * DH * 8 if single else c * 2 * DH * 8


def ks_off(c, single):
    return (2 * NC + HALF.index(c)) * 8 if single else c * 16


def slots(c):
    return [('h', c) if (c in HM and x == HB) else ('b', x) for x in MXB]


def timeline(T):
    ktime = []; pvtime = {}; now = 0
    for t in range(T):
        for n, sl in enumerate(slots(t % NC)):
            if n == SPL:
                pvtime[t - SK] = now; now += 16
            ktime.append(now); now += 8 if sl[0] == 'h' else 16
    for t in range(T - SK, T):
        pvtime[t] = now + 128 * (t - T + SK) + 32
    vs = [(pvtime[t] - DLT - (3 - col) * 32, t, col, False) for t in range(T) for col in COLS]
    free = sorted(pvtime[t] - o for t in range(-SK, T) for o in SO)
    for t in range(T - 1, -1, -1):
        if t % NC in HALF:
            for col in reversed(COLS):
                tm = [x for x in free if x <= pvtime[t] - SDL][-1]
                free.remove(tm)
                vs.append((tm, t, col, True))
    vs.sort()
    return len(ktime), [(t, col, single, sum(1 for k in ktime if k < tm)) for (tm, t, col, single) in vs]


def share(x, tot, n, skip):
    if x < skip or x >= n:
        return 0
    return ((x - skip + 1) * tot) // (n - skip) - ((x - skip) * tot) // (n - skip)


def _kernel(ax, aw, ao, bx, bw, bo, out_hbm,
            x_b, w_b, wo_b, wt_s, kp_s, qt_s, vt_s, qf_s, ks_s, ot_s, ls_s, ob, bufa, bufb, bufc,
            s_s, p_c, l_c, o_c, v_c, lv_c, vm_s, kx_s, px_s, kb2, z_ref, isem, osem):
    b = pl.program_id(0)
    bufs = (bufa, bufb, bufc)

    def kbuf(ph):
        return bufs[(ph + 2) % NPH]

    def in_refs(src3, slot, j):
        x, w, wo = src3
        if j < 3:
            c0 = (D, 0, 2 * D)[j]
            return w.at[:, c0:c0 + D], w_b.at[slot, :, c0:c0 + D]
        if j < 3 + NXC:
            i = j - 3
            return x.at[0, i * PR:(i + 1) * PR, :], x_b.at[slot, i * PR:(i + 1) * PR, :]
        return wo, wo_b.at[slot]

    @pl.when(b == 0)
    def _():
        for slot, src3 in enumerate(((ax, aw, ao), (bx, bw, bo))):
            for j in (0, 3, 4, 5, 6, 1, 2, 7):
                src, dst = in_refs(src3, slot, j)
                pltpu.make_async_copy(src, dst, isem.at[slot, j]).start()
        for j in range(NZ):
            z_ref[j] = 0

    def wait_in(j):
        dst = in_refs((ax, aw, ao), b, j)[1]
        pltpu.make_async_copy(dst, dst, isem.at[b, j]).wait()

    def ldk(it, ph, row, n):
        return kbuf(ph)[pl.ds(pl.multiple_of(KOFF + it * (S // 2), 8) + row, n), :]

    def prep_gen(h, ph):
        for i0 in range(0, len(PITEMS), PORD):
            for d in range(DH):
                for (c, single) in PITEMS[i0:i0 + PORD]:
                    n = 8 if single else 16
                    col = ks_s[h, ks_off(c, single): ks_off(c, single) + n, :][:, d:d + 1]
                    base = kb_off(c, single) + d * n
                    bufs[ph][base: base + n, :] = pltpu.bitcast(jnp.broadcast_to(col, (n, 128)), U32)
                    yield

    def q_rows(hz, ct, d0, g, n):
        return jnp.concatenate([jnp.broadcast_to(qf_s[hz, d:d + 1, ct * 128:(ct + 1) * 128], (n, 128))
                                for d in range(d0, d0 + g)], axis=0)

    def mac(acc, kv, qs, g):
        t = (kv * qs).reshape(g, kv.shape[0] // g, 128)
        if acc is not None:
            t = jnp.concatenate([acc[None], t], axis=0)
        return jnp.sum(t, axis=0)

    nt_dims = (((1,), (1,)), ((), ()))
    stats = {}

    def upd(name, val):
        stats[name] = val if name not in stats else jnp.maximum(stats[name], val)

    def proj_k(i):
        xc = x_b[b, pl.ds(i * PR, PR), :]
        kc = jnp.dot(xc, w_b[b, :, D:2 * D], preferred_element_type=F32)
        upd("k", jnp.max(jnp.abs(kc).reshape(PR // 8, 8, D), axis=0))
        kp_s[i * (PR // 2):(i + 1) * (PR // 2), :] = pltpu.bitcast(kc.astype(BF), U32)

    def spread_k(i):
        for h in range(H):
            g, r = divmod(h, 8)
            it, ph = divmod(h, NPH)
            kr = kp_s[i * (PR // 2):(i + 1) * (PR // 2), g * 128:(g + 1) * 128]
            if r:
                kr = pltpu.roll(kr, 128 - DH * r, axis=1)
            ko = KOFF + it * (S // 2) + i * (PR // 2)
            kbuf(ph)[ko: ko + PR // 2, :] = kr
            if ph == 1 and i == 0:
                xo = XOFF + it * XC * (CH // 2)
                kbuf(0)[xo: xo + XC * (CH // 2), :] = kr[0: XC * (CH // 2)]
            for c in range(i * (PR // CH), (i + 1) * (PR // CH)):
                r0 = (c % (PR // CH)) * (CH // 2)
                ks_s[h, ks_off(c, False): ks_off(c, False) + 16, :] = (
                    pltpu.bitcast(kr[r0 + VB * 8: r0 + VB * 8 + 8], BF).astype(F32))
                if c in HM:
                    kf = pltpu.bitcast(kr[r0 + HB * 8: r0 + HB * 8 + 8], BF).astype(F32)
                    fo = FOFF + (it * HST + HM.index(c)) * 8
                    kbuf(ph)[fo: fo + 8, :] = pltpu.bitcast(kf[0:8], U32)
                    if ph == 1 and c < XC:
                        xf = XFO + (it * XC + c) * 8
                        kbuf(0)[xf: xf + 8, :] = pltpu.bitcast(kf[0:8], U32)
                    if c in HALF:
                        ks_s[h, ks_off(c, True): ks_off(c, True) + 8, :] = kf[8:16]
                    else:
                        kx_s[h] = kf[8:16]

    def proj_q(i):
        xc = x_b[b, pl.ds(i * PR, PR), :]
        q = lax.dot_general(wt_s[0:D, :], xc, nt_dims, preferred_element_type=F32) * QSCALE
        upd("q", jnp.sum((q * q).reshape(H, DH, PR), axis=1))
        qt_s[:, pl.ds(i * PR, PR)] = pltpu.bitcast(q.astype(BF), U32)
        qf_s[0:H, :, pl.ds(i * PR, PR)] = q.reshape(H, DH, PR)

    def proj_v(i):
        xc = x_b[b, pl.ds(i * PR, PR), :]
        v = lax.dot_general(wt_s[D:2 * D, :], xc, nt_dims, preferred_element_type=F32)
        va = jnp.abs(v)
        va = jnp.maximum(jnp.maximum(va[:, 0:128], va[:, 128:256]),
                         jnp.maximum(va[:, 256:384], va[:, 384:512]))
        va = jnp.max(va.reshape(H, 2, 8, 128), axis=1)
        vm_s[...] = va if i == 0 else jnp.maximum(vm_s[...], va)
        vt_s[:, pl.ds(i * PR, PR)] = v
        return v

    def pre_kb(h):
        kx = kx_s[h]
        for d in range(DH):
            kb2[(h * DH + d) * 8:(h * DH + d + 1) * 8, :] = jnp.broadcast_to(kx[:, d:d + 1], (8, 128))

    def pre_x(n, h, c0, pace):
        z = z_ref[n]
        zp = z_ref[NSTEP + n % NPAD]
        kb2[pl.ds(pl.multiple_of(H * DH * 8 + (n % NPAD) * 32 + zp, 8), 8), :] = pace
        qf_s[H + zp, 0:8, (n % NPAD) * 512:(n % NPAD) * 512 + 128] = pace
        hz = h + z
        kv = kb2[pl.ds(pl.multiple_of(h * DH * 8 + z, 8), DH * 8), :]
        outs = [mac(None, kv, q_rows(hz, c0 + x, 0, DH, 8), DH) for x in range(XW)]
        px_s[h, :, c0 * 128:(c0 + XW) * 128] = jnp.exp2(jnp.concatenate(outs, axis=1))

    wait_in(0); wait_in(3)
    proj_k(0)
    wait_in(4); wait_in(5)
    proj_k(1)
    spread_k(0)
    proj_k(2)
    wait_in(6); wait_in(1); wait_in(2)
    wt_s[0:D, :] = w_b[b, :, 0:D].T
    wt_s[D:2 * D, :] = w_b[b, :, 2 * D:3 * D].T
    proj_k(3)
    spread_k(1)
    for i in range(NXC):
        proj_q(i)
        if i < 2:
            spread_k(2 + i)
        if i == 0:
            for h in range(H):
                pre_kb(h)
    per = H * (S // 128) // XW // NXC
    for i in range(NXC):
        v = proj_v(i)
        for m in range(per):
            n = i * per + m
            h, c0 = divmod(n * XW, S // 128)
            ctile, mm = divmod(m, per // 4)
            r = (mm * (D // 8) // (per // 4)) * 8
            pre_x(n, h, c0, v[r:r + 8, ctile * 128:(ctile + 1) * 128])

    km = jnp.max(stats["k"], axis=0, keepdims=True)
    km = km * km
    kseg = jnp.concatenate([km[:, g * 128:(g + 1) * 128] for g in range(4)], axis=0)
    for sh in (1, 2, 4, 8):
        kseg = kseg + pltpu.roll(kseg, sh, axis=1)
    safe_qk = jnp.max(stats["q"]) * jnp.max(kseg) <= SCORE_BOUND * SCORE_BOUND

    def vpu_col(z, ph, h, ct, c, single):
        z0 = pl.multiple_of(z, 8)
        n = 8 if single else 16
        hz = h + z
        acc = None
        d0 = 0
        for g in VGS:
            qs = q_rows(hz, ct, d0, g, n)
            kv = pltpu.bitcast(bufs[ph][pl.ds(z0 + (kb_off(c, single) + d0 * n), g * n), :], F32)
            acc = mac(acc, kv, qs, g)
            d0 += g
        return acc

    def pv_step(h, c, pb, oacc):
        r = pl.multiple_of(h * DH, DH)
        o = jnp.dot(vt_s[pl.ds(r, DH), c * CH:(c + 1) * CH].astype(pb.dtype), pb,
                    preferred_element_type=F32)
        return o if oacc is None else o + oacc

    def carried_p(x):
        return pltpu.bitcast(p_c[x * CH // 2:(x + 1) * CH // 2, :], BF)

    def finish(h, qb, lacc, oacc):
        ls_s[qb, pl.ds(h, 1), :] = jnp.sum(lacc, axis=0, keepdims=True)
        ot_s[h, :, qb * TQ:(qb + 1) * TQ] = oacc

    lead = [x[:3] for x in timeline(NQ * NC)[1][:RC]]

    def lead_gen(h, ph):
        lv = [jnp.zeros((8, 128), F32)] * 4
        for v, (t, col, single) in enumerate(lead):
            p = jnp.exp2(vpu_col(z_ref[v], ph, h, col, t, single))
            v_c[v * 16: v * 16 + p.shape[0], :] = p
            lv[col] = lv[col] + (p if single else p[0:8] + p[8:16])
            if v == RC - 1:
                lv_c[...] = jnp.concatenate(lv, axis=1)
            yield

    def block(it, phs):
        h0 = it * NPH + phs[0]
        hprev = (h0 + H - 1) % H
        nui = len(phs) * NQ
        T = nui * NC
        pads = [pl.multiple_of(PADOFF + 32 * x + z_ref[NSTEP + x], 8) for x in range(NPAD)]
        pbs = {t: {} for t in range(T)}
        laccs = {}; oaccs = {}
        nkt, vsteps = timeline(T)
        assert [x[:3] for x in vsteps[:RC]] == lead
        vnext = [RC]; ng = [0]; nk = [0]; pend = []; lhist = []
        pgen = [prep_gen(jnp.minimum(h0 + n + 2, H - 1), (ph + 2) % NPH) for n, ph in enumerate(phs)]
        phn = (phs[-1] + 1) % NPH
        lgen = lead_gen(jnp.minimum(h0 + len(phs), H - 1), phn)
        kbase = pl.multiple_of(KOFF + it * (S // 2), 8)
        xbase = pl.multiple_of(XOFF + it * XC * (CH // 2), 8)
        fbase = pl.multiple_of(FOFF + it * HST * 8, 8)
        xfbase = pl.multiple_of(XFO + it * XC * 8, 8)
        hs = [h0 + n for n in range(len(phs))]
        wrow = [pl.multiple_of(hh * 8, 8) for hh in hs]
        kph = nkt // len(phs)

        def pre_p(j):
            return px_s[hs[j // NQ], :, (j % NQ) * TQ:(j % NQ + 1) * TQ]

        def l_init(j):
            l0 = pre_p(j)
            return [l0[:, col * 128:(col + 1) * 128] for col in COLS]

        def e_blk(j, s, cols):
            p = jnp.exp2(s)
            ll = p[0:8]
            for x in range(1, s.shape[0] // 8):
                ll = ll + p[x * 8:(x + 1) * 8]
            for n, col in enumerate(cols):
                x = ll[:, n * 128:(n + 1) * 128] if len(cols) > 1 else ll
                if j not in laccs:
                    laccs[j] = l_init(j)
                laccs[j][col] = laccs[j][col] + x
                lhist.append(laccs[j][col])
            return p, ll

        def emit_vpu(upto_k=None, upto_t=None):
            while vnext[0] < len(vsteps):
                v = vnext[0]
                t, col, single, dead = vsteps[v]
                if not ((upto_k is not None and dead <= upto_k)
                        or (upto_t is not None and min(x[0] for x in vsteps[v:]) <= upto_t)):
                    break
                j, c = divmod(t, NC)
                s = vpu_col(z_ref[v], phs[j // NQ], hs[j // NQ], (j % NQ) * 4 + col, c, single)
                pp, ll = e_blk(j, s, [col])
                pbs[t].setdefault('s' if single else 'v', {})[col] = pp
                if v >= NG0:
                    pend.append(ll)
                vnext[0] += 1

        lv0 = lv_c[...]
        laccs[0] = [lv0[:, col * 128:(col + 1) * 128] + y for col, y in zip(COLS, l_init(0))]
        for v, (t, col, single) in enumerate(lead):
            pbs[t].setdefault('s' if single else 'v', {})[col] = v_c[v * 16: v * 16 + (8 if single else 16), :]

        def gates():
            n, kx = divmod(nk[0], kph)
            gb = kbuf(phs[n - 1]) if (n >= 1 and kx < XC * 7) else kbuf(phs[n])
            emit_vpu(upto_k=nk[0])
            if len(lhist) > LG + 4:
                pend.append(lhist[-LG])
            while pend:
                gb[pl.ds(pads[ng[0] % NPAD], 8), :] = pltpu.bitcast(pend.pop(0), U32)
                ng[0] += 1
            for _ in range(share(kx, NPREP, kph - PE, max(PS, XC * 7) if n >= 1 else PS)):
                next(pgen[n])
            for _ in range(share(nk[0], RC, nkt, nkt - LS)):
                bufs[phn][pl.ds(pads[ng[0] % NPAD], 8), :] = pltpu.bitcast(lhist[-LG - (nk[0] % 4)], U32)
                next(lgen)
            nk[0] += 1

        def qk(t, sls):
            j, c = divmod(t, NC)
            h = hs[j // NQ]; ph = phs[j // NQ]; qb = j % NQ
            dup = (j == NQ and c < XC)
            hpos = [x for x, y in enumerate(sls) if y[0] == 'h']
            if hpos and hpos[0] > 0:
                qk(t, sls[:hpos[0]]); qk(t, sls[hpos[0]:])
                return
            if hpos:
                gates()
                if dup:
                    kf = kbuf(ph - 1)[pl.ds(xfbase + c * 8, 8), :]
                else:
                    kf = kbuf(ph)[pl.ds(fbase + HM.index(c) * 8, 8), :]
                s = jnp.dot(pltpu.bitcast(kf, F32)[:, 0:DH], qf_s[h, :, qb * TQ:(qb + 1) * TQ],
                            preferred_element_type=F32)
                pbs[t]['h'] = e_blk(j, s, COLS)[0]
                sls = sls[1:]
            if not sls:
                return
            ks = []
            for _, bb in sls:
                gates()
                row = c * CH // 2 + bb * 8
                if dup:
                    ks.append(kbuf(ph - 1)[pl.ds(xbase + row, 8), :])
                else:
                    ks.append(kbuf(ph)[pl.ds(kbase + row, 8), :])
            kk = pltpu.bitcast(jnp.concatenate(ks, axis=0) if len(ks) > 1 else ks[0], BF)[:, 0:DH]
            w = pltpu.bitcast(qt_s[pl.ds(wrow[j // NQ], 8), qb * TQ:(qb + 1) * TQ], BF)
            s = jnp.dot(kk, w, preferred_element_type=F32)
            for x, (_, bb) in enumerate(sls):
                pbs[t][bb] = e_blk(j, s[x * 16:(x + 1) * 16], COLS)[0]

        def gather_p(tb):
            emit_vpu(upto_t=tb)
            pp = pbs.pop(tb)
            pv = jnp.concatenate([pp['v'][col] for col in COLS], axis=1)
            rows = []
            for bb in range(8):
                if bb == VB:
                    rows.append(pv)
                elif bb in pp:
                    rows.append(pp[bb])
                elif 's' in pp:
                    rows += [pp['h'], jnp.concatenate([pp['s'][col] for col in COLS], axis=1)]
                else:
                    rows += [pp['h'], pre_p(tb // NC)]
            return jnp.concatenate(rows, axis=0)

        def do_pv(tb):
            if tb < 0:
                if tb == -SK:
                    oaccs[-1] = o_c[...]
                oaccs[-1] = pv_step(hprev, NC + tb, carried_p(tb + SK), oaccs[-1])
                if tb == -1:
                    finish(hprev, NQ - 1, l_c[...], oaccs[-1])
                return
            j, c = divmod(tb, NC)
            oaccs[j] = pv_step(hs[j // NQ], c, gather_p(tb), oaccs.get(j))
            if c == NC - 1:
                finish(hs[j // NQ], j % NQ, jnp.concatenate(laccs[j], axis=1), oaccs[j])

        for t in range(T):
            sls = slots(t % NC)
            if t == 0:
                cuts = [(CP[x], x - SK) for x in range(SK)]
            else:
                cuts = [(SPL, t - SK)] if t >= SK else []
            pos = 0
            for cut, tb in cuts:
                qk(t, sls[pos:cut])
                do_pv(tb)
                pos = cut
            qk(t, sls[pos:])
        for x in range(SK):
            p_c[x * CH // 2:(x + 1) * CH // 2, :] = pltpu.bitcast(gather_p(T - SK + x).astype(BF), U32)
        l_c[...] = jnp.concatenate(laccs[nui - 1], axis=1)
        o_c[...] = oaccs[nui - 1]

    for hh in range(2):
        for _ in prep_gen(hh, hh):
            pass
    p_c[...] = jnp.zeros(p_c.shape, U32)
    l_c[...] = jnp.ones(l_c.shape, F32)
    o_c[...] = jnp.zeros(o_c.shape, F32)
    for _ in lead_gen(0, 0):
        pass

    @pl.when(safe_qk)
    def _():
        def body(i, c):
            block(i, BLOCKS[0])
            pl.when(i * NPH + BLOCKS[1][0] < H)(functools.partial(block, i, BLOCKS[1]))
            return c
        lax.fori_loop(0, NIT, body, 0)

    o = o_c[...]
    for x in range(SK):
        o = pv_step(H - 1, NC - SK + x, carried_p(x), o)
    finish(H - 1, NQ - 1, l_c[...], o)
    vh = jnp.max(jnp.max(vm_s[...], axis=1), axis=1, keepdims=True)
    safe = safe_qk & (jnp.min(vh) >= V_LO) & (jnp.max(vh) <= V_HI)

    def slow_body(it, carry):
        sc = 256
        for ph in range(NPH):
            h = it * NPH + ph

            def unit(qb, c2):
                c0 = pl.multiple_of(qb * TQ, TQ)
                w = pltpu.bitcast(qt_s[pl.ds(pl.multiple_of(h * 8, 8), 8), pl.ds(c0, TQ)], BF)

                def p1(c, m):
                    ro = pl.multiple_of(c * (sc // 2), 8)
                    kk = pltpu.bitcast(ldk(it, ph, ro, sc // 2), BF)[:, 0:DH]
                    s = jnp.dot(kk, w, preferred_element_type=F32)
                    s_s[pl.ds(pl.multiple_of(c * sc, sc), sc), :] = s
                    return jnp.maximum(m, jnp.max(s, axis=0, keepdims=True))
                m = lax.fori_loop(0, S // sc, p1, jnp.full((1, TQ), -jnp.inf, F32))

                def p2(c, lo):
                    l, o = lo
                    co = pl.multiple_of(c * sc, sc)
                    p = jnp.exp2(s_s[pl.ds(co, sc), :] - m)
                    vt = vt_s[pl.ds(pl.multiple_of(h * DH, DH), DH), pl.ds(co, sc)]
                    return (l + jnp.sum(p.reshape(sc // 8, 8, TQ), axis=0),
                            o + jnp.dot(vt, p, preferred_element_type=F32))
                l, o = lax.fori_loop(0, S // sc, p2,
                                     (jnp.zeros((8, TQ), F32), jnp.zeros((DH, TQ), F32)))
                ot_s[h, :, pl.ds(c0, TQ)] = o
                ls_s[qb, pl.ds(h, 1), :] = jnp.sum(l, axis=0, keepdims=True)
                return c2
            lax.fori_loop(0, jnp.where(h < H, NQ, 0), unit, 0)
        return carry

    @pl.when(jnp.logical_not(safe))
    def _():
        lax.fori_loop(0, NIT, slow_body, 0)

    wait_in(3 + NXC)

    def out_copy(bb, n):
        r0, nr = OCH[n]
        return pltpu.make_async_copy(
            ob.at[r0:r0 + nr, :],
            out_hbm.at[0, r0:r0 + nr, pl.ds(pl.multiple_of(bb * D, D), D)], osem.at[n])

    @pl.when(b == 1)
    def _():
        for n in range(len(OCH)):
            out_copy(0, n).wait()

    for n, (r0, nr) in enumerate(OCH):
        qb, c0 = divmod(r0, TQ)
        inv = 1.0 / ls_s[qb, :, c0:c0 + nr]
        oc = (ot_s[:, :, r0:r0 + nr] * inv.reshape(H, 1, nr)).reshape(D, nr).T.astype(BF)
        r = jnp.dot(oc, wo_b[b], preferred_element_type=F32)
        ob[r0:r0 + nr, :] = r.astype(BF)
        out_copy(b, n).start()

    @pl.when(b == 1)
    def _():
        for n in range(len(OCH)):
            out_copy(1, n).wait()


@jax.jit
def pallas_concat_heads__softmax_full_mha__softmax_full_mha__prompt_kernel(
    A_x: jax.Array,
    A_wqkv: jax.Array,
    A_wo: jax.Array,
    B_x: jax.Array,
    B_wqkv: jax.Array,
    B_wo: jax.Array,
):
    any_spec = pl.BlockSpec(memory_space=pl.ANY)
    vm = pltpu.VMEM
    return pl.pallas_call(
        _kernel,
        out_shape=jax.ShapeDtypeStruct((1, S, 2 * D), BF),
        grid=(2,),
        in_specs=[any_spec] * 6,
        out_specs=any_spec,
        scratch_shapes=[
            vm((2, S, D), BF), vm((2, D, 3 * D), BF), vm((2, D, D), BF),
            vm((2 * D, D), BF),
            vm((S // 2, D), U32), vm((D // 2, S), U32), vm((D, S), F32),
            vm((H + 1, DH, S), F32), vm((H, NGT * 8, 128), F32),
            vm((H, DH, S), F32), vm((NQ, H, TQ), F32), vm((S, D), BF),
            vm((TOTR, 128), U32), vm((TOTR, 128), U32), vm((TOTR, 128), U32),
            vm((S, TQ), F32),
            vm((SK * CH // 2, TQ), U32), vm((8, TQ), F32), vm((DH, TQ), F32),
            vm((RC * 16, 128), F32), vm((8, TQ), F32), vm((H, 8, 128), F32),
            vm((H, 8, 128), F32), vm((H, 8, S), F32), vm((H * DH * 8 + NPAD * 32, 128), F32),
            pltpu.SMEM((NZ,), jnp.int32),
            pltpu.SemaphoreType.DMA((2, NXC + 4)), pltpu.SemaphoreType.DMA((len(OCH),)),
        ],
        compiler_params=pltpu.CompilerParams(
            vmem_limit_bytes=100 * 1024 * 1024, dimension_semantics=("arbitrary",)),
    )(A_x, A_wqkv, A_wo, B_x, B_wqkv, B_wo)
```

```python
import functools
import math

import jax
import jax.numpy as jnp
from jax import lax
from jax.experimental import pallas as pl
from jax.experimental.pallas import tpu as pltpu

S = 2048; D = 512; H = 32; DH = 16
TQ = 512
CH = 128
PR = 512
NQ = S // TQ; NC = S // CH; NXC = S // PR
F32 = jnp.float32; BF = jnp.bfloat16; U32 = jnp.uint32

QSCALE = (DH ** -0.5) * math.log2(math.e)
SCORE_BOUND = 64.0
V_LO = 2.0 ** -30
V_HI = 2.0 ** 50

SK = 2
SPL = 2
LG = 50
PS = 24; PE = 10
VGS = (3, 4, 4, 5); PORD = 4
NG0 = 0
DLT = 24; SDL = 80; SO = (80, 16)
RC = 4; LS = 10
CP = (3, 5)
XC = 4
HALF = [c for c in range(NC) if c % 2]
XCH = 6
HM = sorted(HALF + [XCH])
HST = -(-len(HM) // 4) * 4
XW = 2
VB = 0
MXB = [x for x in range(7, -1, -1) if x != VB]
HB = MXB[SPL]
NGT = 2 * NC + len(HALF)
KBR = NGT * DH * 8
PITEMS = [(c, False) for c in range(NC)]
for _n, _c in enumerate(HALF):
    PITEMS.insert(_c + _n + 1, (_c, True))
NPREP = len(PITEMS) * DH
NPH = 3
BLOCKS = ((0, 1), (2,))
NIT = -(-H // NPH)
KOFF = KBR
FOFF = KOFF + NIT * (S // 2)
XOFF = FOFF + NIT * HST * 8
XFO = XOFF + NIT * XC * (CH // 2)
PADOFF = XFO + NIT * XC * 8
NPAD = 4
TOTR = PADOFF + 32 * NPAD
assert all(x % 32 == 0 for x in (KOFF, FOFF, XOFF, XFO, PADOFF, TOTR))
NSTEP = 2 * NQ * 4 * (NC + len(HALF))
NZ = NSTEP + NPAD
OCH = ((0, 128), (128, 384), (512, 512), (1024, 512), (1536, 384), (1920, 128))
COLS = (0, 1, 2, 3)


def kb_off(c, single):
    return (2 * NC + HALF.index(c)) * DH * 8 if single else c * 2 * DH * 8


def ks_off(c, single):
    return (2 * NC + HALF.index(c)) * 8 if single else c * 16


def slots(c):
    return [('h', c) if (c in HM and x == HB) else ('b', x) for x in MXB]


def timeline(T):
    ktime = []; pvtime = {}; now = 0
    for t in range(T):
        for n, sl in enumerate(slots(t % NC)):
            if n == SPL:
                pvtime[t - SK] = now; now += 16
            ktime.append(now); now += 8 if sl[0] == 'h' else 16
    for t in range(T - SK, T):
        pvtime[t] = now + 128 * (t - T + SK) + 32
    vs = [(pvtime[t] - DLT - (3 - col) * 32, t, col, False) for t in range(T) for col in COLS]
    free = sorted(pvtime[t] - o for t in range(-SK, T) for o in SO)
    for t in range(T - 1, -1, -1):
        if t % NC in HALF:
            for col in reversed(COLS):
                tm = [x for x in free if x <= pvtime[t] - SDL][-1]
                free.remove(tm)
                vs.append((tm, t, col, True))
    vs.sort()
    return len(ktime), [(t, col, single, sum(1 for k in ktime if k < tm)) for (tm, t, col, single) in vs]


def share(x, tot, n, skip):
    if x < skip or x >= n:
        return 0
    return ((x - skip + 1) * tot) // (n - skip) - ((x - skip) * tot) // (n - skip)


def _kernel(ax, aw, ao, bx, bw, bo, out_hbm,
            x_b, w_b, wo_b, wt_s, kp_s, qt_s, vt_s, qf_s, ks_s, ot_s, ls_s, ob, bufa, bufb, bufc,
            s_s, p_c, l_c, o_c, v_c, lv_c, vm_s, kx_s, px_s, kb2, z_ref, isem, osem):
    b = pl.program_id(0)
    bufs = (bufa, bufb, bufc)

    def kbuf(ph):
        return bufs[(ph + 2) % NPH]

    def in_refs(src3, slot, j):
        x, w, wo = src3
        if j < 3:
            c0 = (D, 0, 2 * D)[j]
            return w.at[:, c0:c0 + D], w_b.at[slot, :, c0:c0 + D]
        if j < 3 + NXC:
            i = j - 3
            return x.at[0, i * PR:(i + 1) * PR, :], x_b.at[slot, i * PR:(i + 1) * PR, :]
        return wo, wo_b.at[slot]

    @pl.when(b == 0)
    def _():
        for slot, src3 in enumerate(((ax, aw, ao), (bx, bw, bo))):
            for j in (0, 3, 4, 5, 6, 1, 2, 7):
                src, dst = in_refs(src3, slot, j)
                pltpu.make_async_copy(src, dst, isem.at[slot, j]).start()
        for j in range(NZ):
            z_ref[j] = 0

    def wait_in(j):
        dst = in_refs((ax, aw, ao), b, j)[1]
        pltpu.make_async_copy(dst, dst, isem.at[b, j]).wait()

    def ldk(it, ph, row, n):
        return kbuf(ph)[pl.ds(pl.multiple_of(KOFF + it * (S // 2), 8) + row, n), :]

    def prep_gen(h, ph):
        for i0 in range(0, len(PITEMS), PORD):
            for d in range(DH):
                for (c, single) in PITEMS[i0:i0 + PORD]:
                    n = 8 if single else 16
                    col = ks_s[h, ks_off(c, single): ks_off(c, single) + n, :][:, d:d + 1]
                    base = kb_off(c, single) + d * n
                    bufs[ph][base: base + n, :] = jnp.broadcast_to(col, (n, 128))
                    yield

    def q_rows(hz, ct, d0, g, n):
        return jnp.concatenate([jnp.broadcast_to(qf_s[hz, d:d + 1, ct * 128:(ct + 1) * 128], (n, 128))
                                for d in range(d0, d0 + g)], axis=0)

    def mac(acc, kv, qs, g):
        t = (kv * qs).reshape(g, kv.shape[0] // g, 128)
        if acc is not None:
            t = jnp.concatenate([acc[None], t], axis=0)
        return jnp.sum(t, axis=0)

    nt_dims = (((1,), (1,)), ((), ()))
    stats = {}

    def upd(name, val):
        stats[name] = val if name not in stats else jnp.maximum(stats[name], val)

    def proj_k(i):
        xc = x_b[b, pl.ds(i * PR, PR), :]
        kc = jnp.dot(xc, w_b[b, :, D:2 * D], preferred_element_type=F32)
        upd("k", jnp.max(jnp.abs(kc).reshape(PR // 8, 8, D), axis=0))
        kp_s[i * (PR // 2):(i + 1) * (PR // 2), :] = pltpu.bitcast(kc.astype(BF), U32)

    def spread_k(i):
        for h in range(H):
            g, r = divmod(h, 8)
            it, ph = divmod(h, NPH)
            kr = kp_s[i * (PR // 2):(i + 1) * (PR // 2), g * 128:(g + 1) * 128]
            if r:
                kr = pltpu.roll(kr, 128 - DH * r, axis=1)
            ko = KOFF + it * (S // 2) + i * (PR // 2)
            kw = pltpu.bitcast(kr, F32)
            kbuf(ph)[ko: ko + PR // 2, :] = kw
            if ph == 1 and i == 0:
                xo = XOFF + it * XC * (CH // 2)
                kbuf(0)[xo: xo + XC * (CH // 2), :] = kw[0: XC * (CH // 2)]
            for c in range(i * (PR // CH), (i + 1) * (PR // CH)):
                r0 = (c % (PR // CH)) * (CH // 2)
                ks_s[h, ks_off(c, False): ks_off(c, False) + 16, :] = (
                    pltpu.bitcast(kr[r0 + VB * 8: r0 + VB * 8 + 8], BF).astype(F32))
                if c in HM:
                    kf = pltpu.bitcast(kr[r0 + HB * 8: r0 + HB * 8 + 8], BF).astype(F32)
                    fo = FOFF + (it * HST + HM.index(c)) * 8
                    kbuf(ph)[fo: fo + 8, :] = kf[0:8]
                    if ph == 1 and c < XC:
                        xf = XFO + (it * XC + c) * 8
                        kbuf(0)[xf: xf + 8, :] = kf[0:8]
                    if c in HALF:
                        ks_s[h, ks_off(c, True): ks_off(c, True) + 8, :] = kf[8:16]
                    else:
                        kx_s[h] = kf[8:16]

    def proj_q(i):
        xc = x_b[b, pl.ds(i * PR, PR), :]
        q = lax.dot_general(wt_s[0:D, :], xc, nt_dims, preferred_element_type=F32) * QSCALE
        upd("q", jnp.sum((q * q).reshape(H, DH, PR), axis=1))
        qt_s[:, pl.ds(i * PR, PR)] = pltpu.bitcast(q.astype(BF), U32)
        qf_s[0:H, :, pl.ds(i * PR, PR)] = q.reshape(H, DH, PR)

    def proj_v(i):
        xc = x_b[b, pl.ds(i * PR, PR), :]
        v = lax.dot_general(wt_s[D:2 * D, :], xc, nt_dims, preferred_element_type=F32)
        va = jnp.abs(v)
        va = jnp.maximum(jnp.maximum(va[:, 0:128], va[:, 128:256]),
                         jnp.maximum(va[:, 256:384], va[:, 384:512]))
        va = jnp.max(va.reshape(H, 2, 8, 128), axis=1)
        vm_s[...] = va if i == 0 else jnp.maximum(vm_s[...], va)
        vt_s[:, pl.ds(i * PR, PR)] = v
        return v

    def pre_kb(h):
        kx = kx_s[h]
        for d in range(DH):
            kb2[(h * DH + d) * 8:(h * DH + d + 1) * 8, :] = jnp.broadcast_to(kx[:, d:d + 1], (8, 128))

    def pre_x(n, h, c0, pace):
        z = z_ref[n]
        zp = z_ref[NSTEP + n % NPAD]
        kb2[pl.ds(pl.multiple_of(H * DH * 8 + (n % NPAD) * 32 + zp, 8), 8), :] = pace
        qf_s[H + zp, 0:8, (n % NPAD) * 512:(n % NPAD) * 512 + 128] = pace
        hz = h + z
        kv = kb2[pl.ds(pl.multiple_of(h * DH * 8 + z, 8), DH * 8), :]
        outs = [mac(None, kv, q_rows(hz, c0 + x, 0, DH, 8), DH) for x in range(XW)]
        px_s[h, :, c0 * 128:(c0 + XW) * 128] = jnp.exp2(jnp.concatenate(outs, axis=1))

    wait_in(0); wait_in(3)
    proj_k(0)
    wait_in(4); wait_in(5)
    proj_k(1)
    spread_k(0)
    proj_k(2)
    wait_in(6); wait_in(1); wait_in(2)
    wt_s[0:D, :] = w_b[b, :, 0:D].T
    wt_s[D:2 * D, :] = w_b[b, :, 2 * D:3 * D].T
    proj_k(3)
    spread_k(1)
    for i in range(NXC):
        proj_q(i)
        if i < 2:
            spread_k(2 + i)
        if i == 0:
            for h in range(H):
                pre_kb(h)
    per = H * (S // 128) // XW // NXC
    for i in range(NXC):
        v = proj_v(i)
        for m in range(per):
            n = i * per + m
            h, c0 = divmod(n * XW, S // 128)
            ctile, mm = divmod(m, per // 4)
            r = (mm * (D // 8) // (per // 4)) * 8
            pre_x(n, h, c0, v[r:r + 8, ctile * 128:(ctile + 1) * 128])

    km = jnp.max(stats["k"], axis=0, keepdims=True)
    km = km * km
    kseg = jnp.concatenate([km[:, g * 128:(g + 1) * 128] for g in range(4)], axis=0)
    for sh in (1, 2, 4, 8):
        kseg = kseg + pltpu.roll(kseg, sh, axis=1)
    safe_qk = jnp.max(stats["q"]) * jnp.max(kseg) <= SCORE_BOUND * SCORE_BOUND

    def vpu_col(z, ph, h, ct, c, single):
        z0 = pl.multiple_of(z, 8)
        n = 8 if single else 16
        hz = h + z
        acc = None
        d0 = 0
        for g in VGS:
            qs = q_rows(hz, ct, d0, g, n)
            kv = bufs[ph][pl.ds(z0 + (kb_off(c, single) + d0 * n), g * n), :]
            acc = mac(acc, kv, qs, g)
            d0 += g
        return acc

    def pv_step(h, c, pb, oacc):
        r = pl.multiple_of(h * DH, DH)
        o = jnp.dot(vt_s[pl.ds(r, DH), c * CH:(c + 1) * CH].astype(pb.dtype), pb,
                    preferred_element_type=F32)
        return o if oacc is None else o + oacc

    def carried_p(x):
        return pltpu.bitcast(p_c[x * CH // 2:(x + 1) * CH // 2, :], BF)

    def finish(h, qb, lacc, oacc):
        ls_s[qb, pl.ds(h, 1), :] = jnp.sum(lacc, axis=0, keepdims=True)
        ot_s[h, :, qb * TQ:(qb + 1) * TQ] = oacc

    lead = [x[:3] for x in timeline(NQ * NC)[1][:RC]]

    def lead_gen(h, ph):
        lv = [jnp.zeros((8, 128), F32)] * 4
        for v, (t, col, single) in enumerate(lead):
            p = jnp.exp2(vpu_col(z_ref[v], ph, h, col, t, single))
            v_c[v * 16: v * 16 + p.shape[0], :] = p
            lv[col] = lv[col] + (p if single else p[0:8] + p[8:16])
            if v == RC - 1:
                lv_c[...] = jnp.concatenate(lv, axis=1)
            yield

    def block(it, phs):
        h0 = it * NPH + phs[0]
        hprev = (h0 + H - 1) % H
        nui = len(phs) * NQ
        T = nui * NC
        pads = [pl.multiple_of(PADOFF + 32 * x + z_ref[NSTEP + x], 8) for x in range(NPAD)]
        pbs = {t: {} for t in range(T)}
        laccs = {}; oaccs = {}
        nkt, vsteps = timeline(T)
        assert [x[:3] for x in vsteps[:RC]] == lead
        vnext = [RC]; ng = [0]; nk = [0]; pend = []; lhist = []
        pgen = [prep_gen(jnp.minimum(h0 + n + 2, H - 1), (ph + 2) % NPH) for n, ph in enumerate(phs)]
        phn = (phs[-1] + 1) % NPH
        lgen = lead_gen(jnp.minimum(h0 + len(phs), H - 1), phn)
        kbase = pl.multiple_of(KOFF + it * (S // 2), 8)
        xbase = pl.multiple_of(XOFF + it * XC * (CH // 2), 8)
        fbase = pl.multiple_of(FOFF + it * HST * 8, 8)
        xfbase = pl.multiple_of(XFO + it * XC * 8, 8)
        hs = [h0 + n for n in range(len(phs))]
        wrow = [pl.multiple_of(hh * 8, 8) for hh in hs]
        kph = nkt // len(phs)

        def pre_p(j):
            return px_s[hs[j // NQ], :, (j % NQ) * TQ:(j % NQ + 1) * TQ]

        def l_init(j):
            l0 = pre_p(j)
            return [l0[:, col * 128:(col + 1) * 128] for col in COLS]

        def e_blk(j, s, cols):
            p = jnp.exp2(s)
            ll = p[0:8]
            for x in range(1, s.shape[0] // 8):
                ll = ll + p[x * 8:(x + 1) * 8]
            for n, col in enumerate(cols):
                x = ll[:, n * 128:(n + 1) * 128] if len(cols) > 1 else ll
                if j not in laccs:
                    laccs[j] = l_init(j)
                laccs[j][col] = laccs[j][col] + x
                lhist.append(laccs[j][col])
            return p, ll

        def emit_vpu(upto_k=None, upto_t=None):
            while vnext[0] < len(vsteps):
                v = vnext[0]
                t, col, single, dead = vsteps[v]
                if not ((upto_k is not None and dead <= upto_k)
                        or (upto_t is not None and min(x[0] for x in vsteps[v:]) <= upto_t)):
                    break
                j, c = divmod(t, NC)
                s = vpu_col(z_ref[v], phs[j // NQ], hs[j // NQ], (j % NQ) * 4 + col, c, single)
                pp, ll = e_blk(j, s, [col])
                pbs[t].setdefault('s' if single else 'v', {})[col] = pp
                if v >= NG0:
                    pend.append(ll)
                vnext[0] += 1

        lv0 = lv_c[...]
        laccs[0] = [lv0[:, col * 128:(col + 1) * 128] + y for col, y in zip(COLS, l_init(0))]
        for v, (t, col, single) in enumerate(lead):
            pbs[t].setdefault('s' if single else 'v', {})[col] = v_c[v * 16: v * 16 + (8 if single else 16), :]

        def gates():
            n, kx = divmod(nk[0], kph)
            gb = kbuf(phs[n - 1]) if (n >= 1 and kx < XC * 7) else kbuf(phs[n])
            emit_vpu(upto_k=nk[0])
            if len(lhist) > LG + 4:
                pend.append(lhist[-LG])
            while pend:
                gb[pl.ds(pads[ng[0] % NPAD], 8), :] = pend.pop(0)
                ng[0] += 1
            for _ in range(share(kx, NPREP, kph - PE, max(PS, XC * 7) if n >= 1 else PS)):
                next(pgen[n])
            for _ in range(share(nk[0], RC, nkt, nkt - LS)):
                bufs[phn][pl.ds(pads[ng[0] % NPAD], 8), :] = lhist[-LG - (nk[0] % 4)]
                next(lgen)
            nk[0] += 1

        def qk(t, sls):
            j, c = divmod(t, NC)
            h = hs[j // NQ]; ph = phs[j // NQ]; qb = j % NQ
            dup = (j == NQ and c < XC)
            hpos = [x for x, y in enumerate(sls) if y[0] == 'h']
            if hpos and hpos[0] > 0:
                qk(t, sls[:hpos[0]]); qk(t, sls[hpos[0]:])
                return
            if hpos:
                gates()
                if dup:
                    kf = kbuf(ph - 1)[pl.ds(xfbase + c * 8, 8), :]
                else:
                    kf = kbuf(ph)[pl.ds(fbase + HM.index(c) * 8, 8), :]
                s = jnp.dot(kf[:, 0:DH], qf_s[h, :, qb * TQ:(qb + 1) * TQ],
                            preferred_element_type=F32)
                pbs[t]['h'] = e_blk(j, s, COLS)[0]
                sls = sls[1:]
            if not sls:
                return
            ks = []
            for _, bb in sls:
                gates()
                row = c * CH // 2 + bb * 8
                if dup:
                    ks.append(kbuf(ph - 1)[pl.ds(xbase + row, 8), :])
                else:
                    ks.append(kbuf(ph)[pl.ds(kbase + row, 8), :])
            kk = pltpu.bitcast(jnp.concatenate(ks, axis=0) if len(ks) > 1 else ks[0], BF)[:, 0:DH]
            w = pltpu.bitcast(qt_s[pl.ds(wrow[j // NQ], 8), qb * TQ:(qb + 1) * TQ], BF)
            s = jnp.dot(kk, w, preferred_element_type=F32)
            for x, (_, bb) in enumerate(sls):
                pbs[t][bb] = e_blk(j, s[x * 16:(x + 1) * 16], COLS)[0]

        def gather_p(tb):
            emit_vpu(upto_t=tb)
            pp = pbs.pop(tb)
            pv = jnp.concatenate([pp['v'][col] for col in COLS], axis=1)
            rows = []
            for bb in range(8):
                if bb == VB:
                    rows.append(pv)
                elif bb in pp:
                    rows.append(pp[bb])
                elif 's' in pp:
                    rows += [pp['h'], jnp.concatenate([pp['s'][col] for col in COLS], axis=1)]
                else:
                    rows += [pp['h'], pre_p(tb // NC)]
            return jnp.concatenate(rows, axis=0)

        def do_pv(tb):
            if tb < 0:
                if tb == -SK:
                    oaccs[-1] = o_c[...]
                oaccs[-1] = pv_step(hprev, NC + tb, carried_p(tb + SK), oaccs[-1])
                if tb == -1:
                    finish(hprev, NQ - 1, l_c[...], oaccs[-1])
                return
            j, c = divmod(tb, NC)
            oaccs[j] = pv_step(hs[j // NQ], c, gather_p(tb), oaccs.get(j))
            if c == NC - 1:
                finish(hs[j // NQ], j % NQ, jnp.concatenate(laccs[j], axis=1), oaccs[j])

        for t in range(T):
            sls = slots(t % NC)
            if t == 0:
                cuts = [(CP[x], x - SK) for x in range(SK)]
            else:
                cuts = [(SPL, t - SK)] if t >= SK else []
            pos = 0
            for cut, tb in cuts:
                qk(t, sls[pos:cut])
                do_pv(tb)
                pos = cut
            qk(t, sls[pos:])
        for x in range(SK):
            p_c[x * CH // 2:(x + 1) * CH // 2, :] = pltpu.bitcast(gather_p(T - SK + x).astype(BF), U32)
        l_c[...] = jnp.concatenate(laccs[nui - 1], axis=1)
        o_c[...] = oaccs[nui - 1]

    for hh in range(2):
        for _ in prep_gen(hh, hh):
            pass
    p_c[...] = jnp.zeros(p_c.shape, U32)
    l_c[...] = jnp.ones(l_c.shape, F32)
    o_c[...] = jnp.zeros(o_c.shape, F32)
    for _ in lead_gen(0, 0):
        pass

    @pl.when(safe_qk)
    def _():
        def body(i, c):
            block(i, BLOCKS[0])
            pl.when(i * NPH + BLOCKS[1][0] < H)(functools.partial(block, i, BLOCKS[1]))
            return c
        lax.fori_loop(0, NIT, body, 0)

    o = o_c[...]
    for x in range(SK):
        o = pv_step(H - 1, NC - SK + x, carried_p(x), o)
    finish(H - 1, NQ - 1, l_c[...], o)
    vh = jnp.max(jnp.max(vm_s[...], axis=1), axis=1, keepdims=True)
    safe = safe_qk & (jnp.min(vh) >= V_LO) & (jnp.max(vh) <= V_HI)

    def slow_body(it, carry):
        sc = 256
        for ph in range(NPH):
            h = it * NPH + ph

            def unit(qb, c2):
                c0 = pl.multiple_of(qb * TQ, TQ)
                w = pltpu.bitcast(qt_s[pl.ds(pl.multiple_of(h * 8, 8), 8), pl.ds(c0, TQ)], BF)

                def p1(c, m):
                    ro = pl.multiple_of(c * (sc // 2), 8)
                    kk = pltpu.bitcast(ldk(it, ph, ro, sc // 2), BF)[:, 0:DH]
                    s = jnp.dot(kk, w, preferred_element_type=F32)
                    s_s[pl.ds(pl.multiple_of(c * sc, sc), sc), :] = s
                    return jnp.maximum(m, jnp.max(s, axis=0, keepdims=True))
                m = lax.fori_loop(0, S // sc, p1, jnp.full((1, TQ), -jnp.inf, F32))

                def p2(c, lo):
                    l, o = lo
                    co = pl.multiple_of(c * sc, sc)
                    p = jnp.exp2(s_s[pl.ds(co, sc), :] - m)
                    vt = vt_s[pl.ds(pl.multiple_of(h * DH, DH), DH), pl.ds(co, sc)]
                    return (l + jnp.sum(p.reshape(sc // 8, 8, TQ), axis=0),
                            o + jnp.dot(vt, p, preferred_element_type=F32))
                l, o = lax.fori_loop(0, S // sc, p2,
                                     (jnp.zeros((8, TQ), F32), jnp.zeros((DH, TQ), F32)))
                ot_s[h, :, pl.ds(c0, TQ)] = o
                ls_s[qb, pl.ds(h, 1), :] = jnp.sum(l, axis=0, keepdims=True)
                return c2
            lax.fori_loop(0, jnp.where(h < H, NQ, 0), unit, 0)
        return carry

    @pl.when(jnp.logical_not(safe))
    def _():
        lax.fori_loop(0, NIT, slow_body, 0)

    wait_in(3 + NXC)

    def out_copy(bb, n):
        r0, nr = OCH[n]
        return pltpu.make_async_copy(
            ob.at[r0:r0 + nr, :],
            out_hbm.at[0, r0:r0 + nr, pl.ds(pl.multiple_of(bb * D, D), D)], osem.at[n])

    @pl.when(b == 1)
    def _():
        for n in range(len(OCH)):
            out_copy(0, n).wait()

    for n, (r0, nr) in enumerate(OCH):
        qb, c0 = divmod(r0, TQ)
        inv = 1.0 / ls_s[qb, :, c0:c0 + nr]
        oc = (ot_s[:, :, r0:r0 + nr] * inv.reshape(H, 1, nr)).reshape(D, nr).T.astype(BF)
        r = jnp.dot(oc, wo_b[b], preferred_element_type=F32)
        ob[r0:r0 + nr, :] = r.astype(BF)
        out_copy(b, n).start()

    @pl.when(b == 1)
    def _():
        for n in range(len(OCH)):
            out_copy(1, n).wait()


@jax.jit
def pallas_concat_heads__softmax_full_mha__softmax_full_mha__prompt_kernel(
    A_x: jax.Array,
    A_wqkv: jax.Array,
    A_wo: jax.Array,
    B_x: jax.Array,
    B_wqkv: jax.Array,
    B_wo: jax.Array,
):
    any_spec = pl.BlockSpec(memory_space=pl.ANY)
    vm = pltpu.VMEM
    return pl.pallas_call(
        _kernel,
        out_shape=jax.ShapeDtypeStruct((1, S, 2 * D), BF),
        grid=(2,),
        in_specs=[any_spec] * 6,
        out_specs=any_spec,
        scratch_shapes=[
            vm((2, S, D), BF), vm((2, D, 3 * D), BF), vm((2, D, D), BF),
            vm((2 * D, D), BF),
            vm((S // 2, D), U32), vm((D // 2, S), U32), vm((D, S), F32),
            vm((H + 1, DH, S), F32), vm((H, NGT * 8, 128), F32),
            vm((H, DH, S), F32), vm((NQ, H, TQ), F32), vm((S, D), BF),
            vm((TOTR, 128), F32), vm((TOTR, 128), F32), vm((TOTR, 128), F32),
            vm((S, TQ), F32),
            vm((SK * CH // 2, TQ), U32), vm((8, TQ), F32), vm((DH, TQ), F32),
            vm((RC * 16, 128), F32), vm((8, TQ), F32), vm((H, 8, 128), F32),
            vm((H, 8, 128), F32), vm((H, 8, S), F32), vm((H * DH * 8 + NPAD * 32, 128), F32),
            pltpu.SMEM((NZ,), jnp.int32),
            pltpu.SemaphoreType.DMA((2, NXC + 4)), pltpu.SemaphoreType.DMA((len(OCH),)),
        ],
        compiler_params=pltpu.CompilerParams(
            vmem_limit_bytes=100 * 1024 * 1024, dimension_semantics=("arbitrary",)),
    )(A_x, A_wqkv, A_wo, B_x, B_wqkv, B_wo)
```
